```python
import jax
import jax.numpy as jnp

def _softmax(x, axis=-1):
    return jax.nn.softmax(x, axis=axis)

def _gelu(x):
    return jax.nn.gelu(x, approximate=True)

def _silu(x):
    return jax.nn.silu(x)

def _sigmoid(x):
    return jax.nn.sigmoid(x)

def _layernorm(x, axis=-1, eps=1e-05):
    m = jnp.mean(x, axis=axis, keepdims=True)
    v = jnp.var(x, axis=axis, keepdims=True)
    return (x - m) / jnp.sqrt(v + eps)

def _scatter_add(tgt, idx, src, axis=0):
    return tgt.at[idx].add(src)

def _segment_sum(src, seg, n):
    return jax.ops.segment_sum(src, seg, n)

class _Rng:

    def __init__(self, key):
        self._k = key

    def _next(self):
        self._k, sub = jax.random.split(self._k)
        return sub

    def normal(self, shape):
        return jax.random.normal(self._next(), shape, dtype=jnp.bfloat16)

    def randint(self, lo, hi, shape):
        return jax.random.randint(self._next(), shape, lo, hi, dtype=jnp.int32)

    def uniform(self, shape, lo=0.0, hi=1.0):
        return jax.random.uniform(self._next(), shape, jnp.bfloat16, lo, hi)

    def permutation(self, n):
        return jax.random.permutation(self._next(), n)
kernel_name = 'sequential_preLN__memory_aug_infini_attn__moe_arch_mod__prompt'

def setup_inputs():
    _rng = _Rng(jax.random.key(int.from_bytes(__import__("os").urandom(4), "little")))
    _w = lambda a: (lambda t: t.astype(jnp.bfloat16) if jnp.issubdtype(t.dtype, jnp.floating) else t)(jnp.asarray(a))

    def _A_setup():
        B, S, D, H = (1, 2048, 576, 32)
        N = 4
        L = max(1, S // N)
        sc = D ** (-0.5)
        return {'x': _w((lambda *s: _rng.normal(s) * 0.05)(B, N * L, D)), 'wq': _w((lambda *s: _rng.normal(s) * 0.05)(D, D) * sc), 'wk': _w((lambda *s: _rng.normal(s) * 0.05)(D, D) * sc), 'wv': _w((lambda *s: _rng.normal(s) * 0.05)(D, D) * sc), 'wo': _w((lambda *s: _rng.normal(s) * 0.05)(D, D) * sc), 'beta': _w((lambda *s: _rng.normal(s) * 0.05)(H))}
    _A_in = _A_setup()

    def _B_setup():
        B, S, D, F, C = (1, 2048, 576, 4608, 1)
        return {'x': _w((lambda *s: _rng.normal(s) * 0.05)(B, S, D)), 'w_r': _w((lambda *s: _rng.normal(s) * 0.05)(D)), 'w_gate': _w((lambda *s: _rng.normal(s) * 0.05)(D, F)), 'w_up': _w((lambda *s: _rng.normal(s) * 0.05)(D, F)), 'w_down': _w((lambda *s: _rng.normal(s) * 0.05)(F, D))}
    _B_in = _B_setup()
    return {'A_x': _A_in['x'], 'A_wq': _A_in['wq'], 'A_wk': _A_in['wk'], 'A_wv': _A_in['wv'], 'A_wo': _A_in['wo'], 'A_beta': _A_in['beta'], 'B_x': _B_in['x'], 'B_w_r': _B_in['w_r'], 'B_w_gate': _B_in['w_gate'], 'B_w_up': _B_in['w_up'], 'B_w_down': _B_in['w_down']}

def reference(A_x, A_wq, A_wk, A_wv, A_wo, A_beta, B_x, B_w_r, B_w_gate, B_w_up, B_w_down):

    def _A_ref(x, wq, wk, wv, wo, beta):
        B, S, D = x.shape
        H = 32
        Dh = D // H
        N = 4
        L = S // N
        q = (lambda x, *d: x.transpose(*d))((x @ wq).reshape(B, S, H, Dh), 0, 2, 1, 3).reshape(B, H, N, L, Dh)
        k = (lambda x, *d: x.transpose(*d))((x @ wk).reshape(B, S, H, Dh), 0, 2, 1, 3).reshape(B, H, N, L, Dh)
        v = (lambda x, *d: x.transpose(*d))((x @ wv).reshape(B, S, H, Dh), 0, 2, 1, 3).reshape(B, H, N, L, Dh)
        phi = lambda t: jnp.where(t > 0, t + 1.0, jnp.exp(t))
        scale = Dh ** (-0.5)
        ar = jnp.arange(L)
        mask = (lambda x, dt: x.astype(dt))(ar[:, None] < ar[None, :], x.dtype) * -1000000000.0
        g = _sigmoid(beta).reshape(1, H, 1, 1)
        M = jnp.einsum('bhd,bhe->bhde', q[:, :, 0, 0, :] * 0.0, q[:, :, 0, 0, :] * 0.0)
        z = q[:, :, 0, 0, :] * 0.0
        outs = []
        for s in range(N):
            qs, ks, vs = (q[:, :, s].copy(), k[:, :, s].copy(), v[:, :, s].copy())
            logits = jnp.einsum('bhqd,bhkd->bhqk', qs, ks) * scale + mask
            p = _softmax(logits, axis=-1)
            a_dot = jnp.einsum('bhqk,bhkd->bhqd', p, vs)
            pq = phi(qs)
            num = jnp.einsum('bhld,bhde->bhle', pq, M)
            den = jnp.einsum('bhld,bhd->bhl', pq, z)[..., None] + 1e-06
            a_mem = num / den
            o = g * a_mem + (1.0 - g) * a_dot
            outs.append(o)
            pk = phi(ks)
            M = M + jnp.einsum('bhld,bhle->bhde', pk, vs)
            z = z + jnp.einsum('bhld->bhd', pk)
        o = (lambda x, *d: x.transpose(*d))(jnp.stack(outs, 2).reshape(B, H, S, Dh), 0, 2, 1, 3).reshape(B, S, D)
        return o @ wo

    def _B_ref(x, w_r, w_gate, w_up, w_down):
        B, S, D = x.shape
        C = 1
        r = x @ w_r
        idx = jnp.argsort(-r, axis=-1)[:, :C]
        idx_e = jnp.repeat(idx.reshape(B, C, 1), D, axis=2)
        x_sel = jnp.take_along_axis(x, idx_e, axis=1)
        g = _silu(x_sel @ w_gate)
        u = x_sel @ w_up
        y = g * u @ w_down
        r_sel = _sigmoid(jnp.take_along_axis(r, idx, axis=1))
        y = y * r_sel.reshape(B, C, 1)
        b_off = (jnp.arange(B) * S).reshape(B, 1)
        flat_idx = (idx + b_off).reshape(B * C)
        zero = (x * 0.0).reshape(B * S, D)
        upd = _scatter_add(zero, flat_idx, y.reshape(B * C, D), axis=0)
        return x + upd.reshape(B, S, D)
    x = A_x
    h = x + _A_ref(_layernorm(x, axis=-1), A_wq, A_wk, A_wv, A_wo, A_beta)
    h2 = h + _B_ref(_layernorm(h, axis=-1), B_w_r, B_w_gate, B_w_up, B_w_down)
    return h2
```

```python
import jax
import jax.numpy as jnp
from jax import lax
import jax.experimental.pallas as pl
import jax.experimental.pallas.tpu as pltpu

S = 2048
D = 576
H = 32
DH = 18
NSEG = 4
L = 512
F = 4608
G = 4
NG = H // G
GD = G * DH
WIN = 128
VW = 80
LOG2E = 1.4426950408889634
SCALE = 0.2353515625
QSCALE = SCALE * LOG2E
MASKV = -1e9 * LOG2E
EPS = 1e-5
SOFF = (0, 128, 384, 768)
CHUNKS = [(j, i) for j in (3, 2, 1, 0) for i in range(j + 1)]
f32 = jnp.float32
bf16 = jnp.bfloat16
u32 = jnp.uint32
NT = (((1,), (1,)), ((), ()))
ONES2 = 0x3F803F80


def _fdiv18(i):
    return jnp.floor((i.astype(f32) + 0.5) * (1.0 / DH)).astype(jnp.int32)


def _phi(t):
    return jnp.where(t > 0, t + 1.0, jnp.exp(t))


def _layernorm_t(x):
    m = jnp.mean(x, axis=0, keepdims=True)
    xc = x - m
    v = jnp.mean(xc * xc, axis=0, keepdims=True)
    return xc * lax.rsqrt(v + EPS)


def _gstart(g):
    return 16 * ((GD * g) // 16)


def _free0(par):
    return GD if par == 0 else 0


def _kernel(x_hbm, wq_hbm, wk_hbm, wv_hbm, wo_hbm, beta_hbm, wr_hbm, wg_hbm, wu_hbm, wd_hbm,
            out_hbm,
            x_v, wraw, wT, woT, wg_v, wu_v, wd_v,
            xn_s, qt_s, pqt_s, k_s, pkt_s, vt_s, stA, stB, mxA, mxB, nd_s, mext_s, mmask_s, oT_s, at_s,
            g_s, wr_s, h_v, hn_v, out_v, xs_s, y_s, beta_ref, wr_ref, best_s,
            sem_x, sem_w, sem_moe, sem_o, sem_s, sem_f):
    def cols(s):
        return pl.ds(pl.multiple_of(s * L, L), L)

    def x_copy(s):
        return pltpu.make_async_copy(x_hbm.at[:, cols(s)], x_v.at[:, cols(s)], sem_x.at[s])

    def w_copy(i):
        src = (wq_hbm, wk_hbm, wv_hbm, wo_hbm)[i]
        return pltpu.make_async_copy(src, wraw.at[i], sem_w.at[i])

    def moe_copy(i):
        src, dst = ((wg_hbm, wg_v), (wu_hbm, wu_v), (wd_hbm, wd_v))[i]
        return pltpu.make_async_copy(src, dst, sem_moe.at[i])

    def out_copy(s):
        return pltpu.make_async_copy(out_v.at[:, cols(s)], out_hbm.at[:, cols(s)], sem_o.at[s])

    def small_copy(i):
        src, dst = ((beta_hbm, beta_ref), (wr_hbm, wr_ref))[i]
        return pltpu.make_async_copy(src, dst, sem_s.at[i])

    def fence():
        pl.semaphore_signal(sem_f, 1)
        pl.semaphore_wait(sem_f, 1)

    x_copy(0).start()
    fence()
    w_copy(0).start()
    fence()
    w_copy(1).start()
    fence()
    w_copy(2).start()

    qt_s[...] = jnp.zeros_like(qt_s)
    pqt_s[...] = jnp.zeros_like(pqt_s)
    pkt_s[...] = jnp.zeros_like(pkt_s)
    mext_s[...] = jnp.zeros_like(mext_s)
    nd_s[...] = jnp.zeros_like(nd_s)
    for par in range(2):
        r = lax.broadcasted_iota(jnp.int32, (VW, WIN), 0)
        l = lax.broadcasted_iota(jnp.int32, (VW, WIN), 1)
        free0 = _free0(par)
        is_free = (r >= free0) & (r < free0 + 8)
        he = jnp.where(is_free, r - free0, _fdiv18(r - 8 * par + DH) - 1)
        mmask_s[par] = jnp.where((he == _fdiv18(l)) & (l < GD), 1.0, 0.0).astype(f32)

    def small_setup():
        beta = beta_ref[...].astype(f32)
        gsig = 1.0 / (1.0 + jnp.exp(-beta))
        fi = lax.broadcasted_iota(jnp.int32, (D, H), 0)
        hi = lax.broadcasted_iota(jnp.int32, (D, H), 1)
        gcol = jnp.sum(jnp.where(_fdiv18(fi) == hi, gsig, 0.0), axis=1, keepdims=True)
        g_s[...] = jnp.broadcast_to(gcol, (D, WIN))
        wr_s[...] = jnp.broadcast_to(wr_ref[...].astype(f32).reshape(1, D), (WIN, D)).T

    best_s[0] = jnp.float32(-jnp.inf)
    best_s[1] = jnp.float32(0.0)

    kq_r = lax.broadcasted_iota(jnp.int32, (WIN, G * WIN), 0)
    kq_c = lax.broadcasted_iota(jnp.int32, (WIN, G * WIN), 1) & (WIN - 1)
    r64 = lax.broadcasted_iota(jnp.int32, (WIN // 2, WIN), 0)

    def ln1(s):
        xn_s[...] = _layernorm_t(x_v[:, cols(s)].astype(f32)).astype(bf16)

    def pad_rows(a, n):
        return jnp.concatenate([a, jnp.zeros((n - a.shape[0], a.shape[1]), a.dtype)], axis=0)

    def proj_q(g0=0, g1=NG):
        q = jnp.dot(wT[pl.ds(g0 * GD, (g1 - g0) * GD), :], xn_s[...], preferred_element_type=f32)
        for g in range(g0, g1):
            qg = q[(g - g0) * GD:(g - g0 + 1) * GD]
            qt_s[g, 0:VW, :] = pad_rows(qg * QSCALE, VW).astype(bf16)
            pqt_s[g, 0:VW, :] = pad_rows(_phi(qg), VW).astype(bf16)

    def proj_k():
        k = jnp.dot(wT[pl.ds(D, D), :], xn_s[...], preferred_element_type=f32)
        for g in range(NG):
            kg = k[g * GD:(g + 1) * GD]
            k_s[g] = pad_rows(kg, WIN).astype(bf16).T
            pkt_s[g, 0:VW, :] = pad_rows(_phi(kg), VW).astype(bf16)

    def proj_v():
        v = jnp.dot(wT[pl.ds(2 * D, D), :], xn_s[...], preferred_element_type=f32)
        vt_s[...] = v.astype(bf16)

    def mem_read():
        for g in range(NG):
            nd_s[g] = jnp.dot(mext_s[g].astype(bf16), pqt_s[g], preferred_element_type=f32)

    def mem_update(g):
        free0 = _free0(g % 2) // 2
        r40 = lax.broadcasted_iota(jnp.int32, (VW // 2, L), 0)
        lhs = pltpu.bitcast(vt_s[pl.ds(_gstart(g), VW), :], u32)
        lhs = pltpu.bitcast(jnp.where((r40 >= free0) & (r40 < free0 + 4), u32(ONES2), lhs), bf16)
        upd = lax.dot_general(lhs, pkt_s[g], NT, preferred_element_type=f32)
        mext_s[g] += jnp.where(mmask_s[g % 2] > 0.5, upd, 0.0)

    def b_chunk(g, st, mx, state, j, i):
        if i == 0:
            q = pltpu.bitcast(qt_s[g, :, j * WIN:(j + 1) * WIN], u32)
            state["rhs"] = jnp.concatenate(
                [pltpu.bitcast(jnp.where((r64 >= 9 * a) & (r64 < 9 * a + 9), q, u32(0)), bf16) for a in range(G)],
                axis=1)
        s = jnp.dot(k_s[g, i * WIN:(i + 1) * WIN, :], state["rhs"], preferred_element_type=f32)
        if i == j:
            s = s + jnp.where(kq_r > kq_c, MASKV, 0.0)
        m = jnp.max(s, axis=0, keepdims=True)
        state["m"] = m if i == 0 else jnp.maximum(state["m"], m)
        st[SOFF[j] + i * WIN:SOFF[j] + (i + 1) * WIN, :] = s
        if i == j:
            mx[j] = jnp.broadcast_to(state["m"], (8, G * WIN))

    def c_chunk(pr, par, st, mx, state, j, i):
        g = 2 * pr + par
        m = mx[j][0:1, :]
        p = jnp.exp2(st[SOFF[j] + i * WIN:SOFF[j] + (i + 1) * WIN, :] - m).astype(bf16)
        for a in range(G):
            row = par * GD + a * DH
            start = (row // 16) * 16
            off = row - start
            rows = pl.ds(pl.multiple_of(pr * (2 * GD) + start, 16), 32)
            one_row = ((off + DH) % 32) // 2
            r16 = lax.broadcasted_iota(jnp.int32, (16, WIN), 0)
            vt = pltpu.bitcast(vt_s[rows, i * WIN:(i + 1) * WIN], u32)
            vt = pltpu.bitcast(jnp.where(r16 == one_row, u32(ONES2), vt), bf16)
            d = jnp.dot(vt, p[:, a * WIN:(a + 1) * WIN], preferred_element_type=f32)
            acc = d if i == 0 else state[a] + d
            state[a] = acc
            if i == j:
                qs = slice(j * WIN, (j + 1) * WIN)
                lsum = acc[2 * one_row:2 * one_row + 1, :]
                ls = start - _gstart(par)
                num = nd_s[g, ls:ls + 32, qs]
                den = nd_s[g, _free0(par) + a:_free0(par) + a + 1, qs] + 1e-6
                gate = g_s[rows, :]
                o = gate * (num * (1.0 / den)) + (1.0 - gate) * (acc * (1.0 / lsum))
                r32 = lax.broadcasted_iota(jnp.int32, (32, WIN), 0)
                keep = (r32 >= off) & (r32 < off + DH)
                pltpu.store(oT_s.at[rows, qs], o, mask=keep)

    bufs = ((stA, mxA), (stB, mxB))

    def b_all0():
        sb = {}
        for (j, i) in CHUNKS:
            b_chunk(0, *bufs[0], sb, j, i)

    def step(pr, par, gnext):
        sb, sc = {}, {}
        for (j, i) in CHUNKS:
            b_chunk(gnext, *bufs[1 - par], sb, j, i)
            c_chunk(pr, par, *bufs[par], sc, j, i)

    def attention():
        def body(t, c):
            step(t, 0, 2 * t + 1)
            step(t, 1, 2 * t + 2)
            return c
        lax.fori_loop(0, NG // 2 - 1, body, 0)
        step(NG // 2 - 1, 0, NG - 1)
        sc = {}
        for n, (j, i) in enumerate(CHUNKS):
            if n < NG:
                mem_update(n)
            c_chunk(NG // 2 - 1, 1, *bufs[1], sc, j, i)

    def out_proj():
        at_s[...] = jnp.dot(woT[...], oT_s[...].astype(bf16), preferred_element_type=f32).astype(bf16)

    def ln2(s):
        hb = (x_v[:, cols(s)].astype(f32) + at_s[...].astype(f32)).astype(bf16)
        h_v[:, cols(s)] = hb
        hf = hb.astype(f32)
        hn = _layernorm_t(hf).astype(bf16)
        hn_v[:, cols(s)] = hn
        hnf = hn.astype(f32)
        out_v[:, cols(s)] = (hf + hnf).astype(bf16)
        out_copy(s).start()
        wr = wr_s[...]
        r = jnp.sum(jnp.concatenate([hnf[:, t * WIN:(t + 1) * WIN] * wr for t in range(L // WIN)], axis=1),
                    axis=0, keepdims=True)
        r = r.astype(bf16).astype(f32)
        rmax = jnp.max(r)
        ridx = lax.broadcasted_iota(jnp.int32, (1, L), 1)
        amax = jnp.min(jnp.where(r == rmax, ridx, L)) + s * L

        @pl.when(rmax > best_s[0])
        def _():
            best_s[0] = rmax
            best_s[1] = amax.astype(f32)

    x_copy(0).wait()
    small_copy(0).start()
    small_copy(1).start()
    ln1(0)
    w_copy(0).wait()
    w_copy(3).start()
    x_copy(1).start()
    wT[pl.ds(0, D), :] = wraw[0].T
    proj_q(0, 2)
    w_copy(1).wait()
    wT[pl.ds(D, D), :] = wraw[1].T
    proj_q(2, NG)
    w_copy(2).wait()
    x_copy(2).start()
    x_copy(3).start()
    wT[pl.ds(2 * D, D), :] = wraw[2].T
    proj_k()
    w_copy(3).wait()
    small_copy(0).wait()
    small_copy(1).wait()
    for i in range(3):
        moe_copy(i).start()
    woT[...] = wraw[3].T
    small_setup()
    proj_v()
    b_all0()

    def segment(s, carry):
        attention()

        @pl.when(s + 1 < NSEG)
        def _():
            x_copy(s + 1).wait()
            out_proj()
            ln1(s + 1)
            proj_q()
            proj_k()
            proj_v()
            mem_read()
            b_all0()
            ln2(s)

        @pl.when(s + 1 == NSEG)
        def _():
            out_proj()
            ln2(s)

        return carry

    lax.fori_loop(0, NSEG, segment, 0)

    idx = best_s[1].astype(jnp.int32)
    tile = pl.ds(pl.multiple_of((idx >> 7) << 7, WIN), WIN)
    lane = idx & (WIN - 1)
    base = pl.multiple_of((lane >> 4) << 4, 16)
    for i in range(3):
        moe_copy(i).wait()
    hn_t = hn_v[:, tile]
    xs_s[...] = hn_t.T
    xs = xs_s[pl.ds(base, 16), :]
    gt = jnp.dot(xs, wg_v[...], preferred_element_type=f32).astype(bf16).astype(f32)
    up = jnp.dot(xs, wu_v[...], preferred_element_type=f32).astype(bf16).astype(f32)
    act = (gt * (1.0 / (1.0 + jnp.exp(-gt)))).astype(bf16).astype(f32) * up
    y = lax.dot_general(act.astype(bf16), wd_v[...], NT, preferred_element_type=f32)
    rsel = jnp.full((1, 1), best_s[0], f32)
    y = y.astype(bf16).astype(f32) * (1.0 / (1.0 + jnp.exp(-rsel)))
    r16 = lax.broadcasted_iota(jnp.int32, (16, D), 0)
    y_s[...] = jnp.zeros_like(y_s)
    y_s[pl.ds(base, 16), :] = jnp.where(r16 == lane - base, y, 0.0).astype(bf16)
    yt = y_s[...].T.astype(f32)
    t = (hn_t.astype(f32) + yt).astype(bf16).astype(f32)
    for s in range(NSEG):
        out_copy(s).wait()
    out_v[:, tile] = (h_v[:, tile].astype(f32) + t).astype(bf16)
    fix = pltpu.make_async_copy(out_v.at[:, tile], out_hbm.at[:, tile], sem_o.at[0])
    fix.start()
    fix.wait()


@jax.jit
def pallas_sequential_preLN__memory_aug_infini_attn__moe_arch_mod__prompt_kernel(
    A_x: jax.Array,
    A_wq: jax.Array,
    A_wk: jax.Array,
    A_wv: jax.Array,
    A_wo: jax.Array,
    A_beta: jax.Array,
    B_x: jax.Array,
    B_w_r: jax.Array,
    B_w_gate: jax.Array,
    B_w_up: jax.Array,
    B_w_down: jax.Array,
):
    del B_x
    hbm = pl.BlockSpec(memory_space=pltpu.HBM)
    out_t = pl.pallas_call(
        _kernel,
        out_shape=jax.ShapeDtypeStruct((D, S), bf16),
        in_specs=[hbm] * 10,
        out_specs=hbm,
        scratch_shapes=[
            pltpu.VMEM((D, S), bf16),
            pltpu.VMEM((4, D, D), bf16),
            pltpu.VMEM((3 * D, D), bf16),
            pltpu.VMEM((D, D), bf16),
            pltpu.VMEM((D, F), bf16),
            pltpu.VMEM((D, F), bf16),
            pltpu.VMEM((D, F), bf16),
            pltpu.VMEM((D, L), bf16),
            pltpu.VMEM((NG, WIN, L), bf16),
            pltpu.VMEM((NG, WIN, L), bf16),
            pltpu.VMEM((NG, L, WIN), bf16),
            pltpu.VMEM((NG, WIN, L), bf16),
            pltpu.VMEM((D, L), bf16),
            pltpu.VMEM((1280, G * WIN), f32),
            pltpu.VMEM((1280, G * WIN), f32),
            pltpu.VMEM((4, 8, G * WIN), f32),
            pltpu.VMEM((4, 8, G * WIN), f32),
            pltpu.VMEM((NG, VW, L), f32),
            pltpu.VMEM((NG, VW, WIN), f32),
            pltpu.VMEM((2, VW, WIN), f32),
            pltpu.VMEM((D, L), f32),
            pltpu.VMEM((D, L), bf16),
            pltpu.VMEM((D, WIN), f32),
            pltpu.VMEM((D, WIN), f32),
            pltpu.VMEM((D, S), bf16),
            pltpu.VMEM((D, S), bf16),
            pltpu.VMEM((D, S), bf16),
            pltpu.VMEM((WIN, D), bf16),
            pltpu.VMEM((WIN, D), bf16),
            pltpu.VMEM((1, H), bf16),
            pltpu.VMEM((D,), bf16),
            pltpu.SMEM((2,), f32),
            pltpu.SemaphoreType.DMA((NSEG,)),
            pltpu.SemaphoreType.DMA((4,)),
            pltpu.SemaphoreType.DMA((3,)),
            pltpu.SemaphoreType.DMA((NSEG,)),
            pltpu.SemaphoreType.DMA((2,)),
            pltpu.SemaphoreType.REGULAR,
        ],
        compiler_params=pltpu.CompilerParams(vmem_limit_bytes=100 * 1024 * 1024),
    )(A_x.reshape(S, D).T, A_wq, A_wk, A_wv, A_wo, A_beta.reshape(1, H), B_w_r,
      B_w_gate, B_w_up, B_w_down.T)
    return out_t.T.reshape(1, S, D)
```

```python
import jax
import jax.numpy as jnp
from jax import lax
import jax.experimental.pallas as pl
import jax.experimental.pallas.tpu as pltpu

S = 2048
D = 576
H = 32
DH = 18
NSEG = 4
L = 512
F = 4608
G = 4
NG = H // G
GD = G * DH
WIN = 128
VW = 80
MC = 96
LOG2E = 1.4426950408889634
SCALE = 0.2353515625
QSCALE = SCALE * LOG2E
MASKV = -1e9 * LOG2E
EPS = 1e-5
SOFF = (0, 128, 384, 768)
CHUNKS = [(j, i) for j in (3, 2, 1, 0) for i in range(j + 1)]
f32 = jnp.float32
bf16 = jnp.bfloat16
u32 = jnp.uint32
NT = (((1,), (1,)), ((), ()))
ONES2 = 0x3F803F80


def _fdiv18(i):
    return jnp.floor((i.astype(f32) + 0.5) * (1.0 / DH)).astype(jnp.int32)


def _phi(t):
    return jnp.where(t > 0, t + 1.0, jnp.exp(t))


def _fold8(x):
    parts = [x[i:i + 8] for i in range(0, x.shape[0], 8)]
    while len(parts) > 1:
        parts = [parts[i] + parts[i + 1] if i + 1 < len(parts) else parts[i] for i in range(0, len(parts), 2)]
    return parts[0]


def _colsum(load, rb):
    acc = _fold8(load(0, rb))
    for r0 in range(rb, D, rb):
        acc = acc + _fold8(load(r0, rb))
    return jnp.sum(acc, axis=0, keepdims=True)


def _ln_stats(load):
    m = _colsum(load, 64) * (1.0 / D)

    def sq(r0, n):
        xc = load(r0, n) - m
        return xc * xc

    v = _colsum(sq, 96) * (1.0 / D)
    return m, lax.rsqrt(v + EPS)


def _recip(x):
    r = pl.reciprocal(x, approx=True)
    return r * (2.0 - x * r)


def _woff(par):
    return 16 * ((GD * par) // 16)


def _free0(par):
    return GD if par == 0 else 0


def _as_bf16(x):
    return pltpu.bitcast(x, bf16)


def _as_u32(x):
    return pltpu.bitcast(x, u32)


def _pad_rows(a, n):
    return jnp.concatenate([a, jnp.zeros((n - a.shape[0], a.shape[1]), a.dtype)], axis=0)


def _kernel(x_hbm, wq_hbm, wk_hbm, wv_hbm, wo_hbm, beta_hbm, wr_hbm, wg_hbm, wu_hbm, wd_hbm,
            out_hbm,
            xl_s, xr_s, wraw, wT, woT, wg_v, wu_v, wd_v,
            xn_s, xnp_s, qt_s, pqt_s, kt_s, k_s, pkt_s, vt_s, stA, stB, mxA, mxB, nd_s, mext_s, mmask_s,
            oT_s, otp_s, at_s, g_s, wr_s, h_s, hn_s, out_s, bh_s, bhn_s, fix_s, acc_s, beta_ref, wr_ref, best_s,
            sem_x, sem_w, sem_moe, sem_o, sem_s, sem_f):
    def cols(s):
        return pl.ds(pl.multiple_of(s * L, L), L)

    def window(pr, par):
        return pl.ds(pl.multiple_of(pr * (2 * GD) + _woff(par), 16), VW)

    def xl_copy(s):
        return pltpu.make_async_copy(x_hbm.at[:, cols(s)], xl_s, sem_x.at[0])

    def xr_copy(s):
        return pltpu.make_async_copy(x_hbm.at[:, cols(s)], xr_s, sem_x.at[1])

    def w_copy(i):
        src = (wq_hbm, wk_hbm, wv_hbm, wo_hbm)[i]
        return pltpu.make_async_copy(src, wraw.at[i], sem_w.at[i])

    WQA = 2 * WIN

    def wq_copy(part):
        cs = pl.ds(0, WQA) if part == 0 else pl.ds(WQA, D - WQA)
        return pltpu.make_async_copy(wq_hbm.at[:, cs], wraw.at[0, :, cs], sem_w.at[0 if part else 4])

    def moe_copy(i):
        src, dst = ((wg_hbm, wg_v), (wu_hbm, wu_v), (wd_hbm, wd_v))[i]
        return pltpu.make_async_copy(src, dst, sem_moe.at[i])

    def out_copy(s):
        return pltpu.make_async_copy(out_s, out_hbm.at[:, cols(s)], sem_o.at[0])

    def small_copy(i):
        src, dst = ((beta_hbm, beta_ref), (wr_hbm, wr_ref))[i]
        return pltpu.make_async_copy(src, dst, sem_s.at[i])

    def fence():
        pl.semaphore_signal(sem_f, 1)
        pl.semaphore_wait(sem_f, 1)

    xl_copy(0).start()
    fence()
    wq_copy(0).start()
    fence()
    wq_copy(1).start()
    fence()
    w_copy(1).start()
    fence()
    w_copy(2).start()

    mext_s[...] = jnp.zeros_like(mext_s)
    k_s[...] = jnp.zeros_like(k_s)
    nd_s[...] = jnp.zeros_like(nd_s)
    acc_s[...] = jnp.zeros_like(acc_s)
    for par in range(2):
        r = lax.broadcasted_iota(jnp.int32, (VW, WIN), 0)
        l = lax.broadcasted_iota(jnp.int32, (VW, WIN), 1)
        free0 = _free0(par)
        hl = _fdiv18(l - 8 * par + DH) - 1
        he = jnp.where((r >= free0) & (r < free0 + 8), r - free0, _fdiv18(r - 8 * par + DH) - 1)
        ok = (he == hl) & (l >= 8 * par) & (l < 8 * par + GD)
        mmask_s[par] = jnp.where(ok, 1.0, 0.0).astype(f32)
    best_s[0] = jnp.float32(-jnp.inf)
    best_s[1] = jnp.float32(0.0)

    def small_setup():
        beta = beta_ref[...].astype(f32)
        gsig = 1.0 / (1.0 + jnp.exp(-beta))
        fi = lax.broadcasted_iota(jnp.int32, (D, H), 0)
        hi = lax.broadcasted_iota(jnp.int32, (D, H), 1)
        gcol = jnp.sum(jnp.where(_fdiv18(fi) == hi, gsig, 0.0), axis=1, keepdims=True)
        g_s[...] = jnp.broadcast_to(gcol, (D, WIN))
        wr_s[...] = jnp.broadcast_to(wr_ref[...].astype(f32).reshape(1, D), (WIN, D)).T

    kq_r = lax.broadcasted_iota(jnp.int32, (WIN, G * WIN), 0)
    kq_c = lax.broadcasted_iota(jnp.int32, (WIN, G * WIN), 1) & (WIN - 1)
    r40 = lax.broadcasted_iota(jnp.int32, (VW // 2, WIN), 0)

    def ln1_tile(t):
        cs = pl.ds(pl.multiple_of(t * WIN, WIN), WIN)
        m, rstd = _ln_stats(lambda r0, n: xl_s[r0:r0 + n, cs].astype(f32))
        for r0 in range(0, D, 48):
            xn_s[r0:r0 + 48, :] = ((xl_s[r0:r0 + 48, cs].astype(f32) - m) * rstd).astype(bf16)
        xnp_s[:, cs] = _as_u32(xn_s[...])

    def proj(base, c):
        return jnp.dot(wT[pl.ds(base + c * MC, MC), :], _as_bf16(xnp_s[...]), preferred_element_type=f32)

    def proj_q(c0=0, c1=D // MC):
        for c in range(c0, c1):
            q = proj(0, c)
            qt_s[pl.ds(c * MC, MC), :] = (q * QSCALE).astype(bf16)
            pqt_s[pl.ds(c * MC, MC), :] = _phi(q).astype(bf16)

    def proj_k():
        for c in range(D // MC):
            k = proj(D, c)
            kt_s[pl.ds(c * MC, MC), :] = k.astype(bf16)
            pkt_s[pl.ds(c * MC, MC), :] = _phi(k).astype(bf16)

    def transpose_k():
        for g in range(NG):
            k_s[g, :, 0:VW] = kt_s[window(g // 2, g % 2), :].T

    def proj_v():
        for c in range(D // MC):
            vt_s[pl.ds(c * MC, MC), :] = proj(2 * D, c).astype(bf16)

    def mem_read():
        r80 = lax.broadcasted_iota(jnp.int32, (VW, L), 0)
        for g in range(NG):
            par = g % 2
            rows = window(g // 2, par)
            nd = jnp.dot(mext_s[g].astype(bf16), _pad_rows(pqt_s[rows, :], WIN), preferred_element_type=f32)
            rden = 1.0 / (nd[_free0(par):_free0(par) + 8] + 1e-6)
            scale = jnp.broadcast_to(rden[0:1], (VW, L))
            for a in range(1, G):
                scale = jnp.where(r80 >= 8 * par + a * DH, rden[a:a + 1], scale)
            nd_s[g] = nd * scale * jnp.concatenate([g_s[rows, :]] * (L // WIN), axis=1)

    def mem_update(g):
        free0 = _free0(g % 2) // 2
        rows = window(g // 2, g % 2)
        r = lax.broadcasted_iota(jnp.int32, (VW // 2, L), 0)
        lhs = _as_u32(vt_s[rows, :])
        lhs = _as_bf16(jnp.where((r >= free0) & (r < free0 + 4), u32(ONES2), lhs))
        upd = lax.dot_general(lhs, _pad_rows(pkt_s[rows, :], WIN), NT, preferred_element_type=f32)
        mext_s[g] += jnp.where(mmask_s[g % 2] > 0.5, upd, 0.0)

    def b_chunk(pr, par, st, mx, state, j, i):
        if i == 0:
            q = _as_u32(qt_s[window(pr, par), j * WIN:(j + 1) * WIN])
            lo = 4 * par
            state["rhs"] = jnp.concatenate(
                [_as_bf16(_pad_rows(jnp.where((r40 >= lo + 9 * a) & (r40 < lo + 9 * a + 9), q, u32(0)), WIN // 2))
                 for a in range(G)], axis=1)
        s = jnp.dot(k_s[2 * pr + par, i * WIN:(i + 1) * WIN, :], state["rhs"], preferred_element_type=f32)
        if i == j:
            s = s + jnp.where(kq_r > kq_c, MASKV, 0.0)
        m = jnp.max(s, axis=0, keepdims=True)
        state["m"] = m if i == 0 else jnp.maximum(state["m"], m)
        st[SOFF[j] + i * WIN:SOFF[j] + (i + 1) * WIN, :] = s
        if i == j:
            mx[j] = jnp.broadcast_to(state["m"], (8, G * WIN))

    def c_chunk(pr, par, st, mx, state, j, i):
        g = 2 * pr + par
        for a in range(G):
            row = par * GD + a * DH
            start = (row // 16) * 16
            off = row - start
            rows = pl.ds(pl.multiple_of(pr * (2 * GD) + start, 16), 32)
            one_row = ((off + DH) % 32) // 2
            r16 = lax.broadcasted_iota(jnp.int32, (16, WIN), 0)
            vt = _as_u32(vt_s[rows, i * WIN:(i + 1) * WIN])
            vt = _as_bf16(jnp.where(r16 == one_row, u32(ONES2), vt))
            hs = slice(a * WIN, (a + 1) * WIN)
            p = jnp.exp2(st[SOFF[j] + i * WIN:SOFF[j] + (i + 1) * WIN, hs] - mx[j, 0:1, hs]).astype(bf16)
            d = jnp.dot(vt, p, preferred_element_type=f32)
            acc = d if i == 0 else state[a] + d
            state[a] = acc
            if i == j:
                qs = slice(j * WIN, (j + 1) * WIN)
                lsum = acc[2 * one_row:2 * one_row + 1, :]
                ls = start - _woff(par)
                o = nd_s[g, ls:ls + 32, qs] + ((1.0 - g_s[rows, :]) * _recip(lsum)) * acc
                r32 = lax.broadcasted_iota(jnp.int32, (32, WIN), 0)
                keep = (r32 >= off) & (r32 < off + DH)
                pltpu.store(oT_s.at[rows, qs], o, mask=keep)

    bufs = ((stA, mxA), (stB, mxB))

    def b_all0():
        sb = {}
        for (j, i) in CHUNKS:
            b_chunk(0, 0, *bufs[0], sb, j, i)

    def step(pr, par):
        npr, npar = (pr, 1) if par == 0 else (pr + 1, 0)
        sb, sc = {}, {}
        for (j, i) in CHUNKS:
            b_chunk(npr, npar, *bufs[1 - par], sb, j, i)
            c_chunk(pr, par, *bufs[par], sc, j, i)

    def attention():
        def body(t, c):
            step(t, 0)
            step(t, 1)
            ln1_tile(t)
            return c
        lax.fori_loop(0, NG // 2 - 1, body, 0)
        ln1_tile(L // WIN - 1)
        step(NG // 2 - 1, 0)
        sc = {}
        for n, (j, i) in enumerate(CHUNKS):
            if n < NG:
                mem_update(n)
            c_chunk(NG // 2 - 1, 1, *bufs[1], sc, j, i)

    def pack_ot():
        at_s[...] = oT_s[...].astype(bf16)
        otp_s[...] = _as_u32(at_s[...])

    def out_proj(nsplit=1):
        pack_ot()
        w = L // nsplit
        for p in range(nsplit):
            cs = slice(p * w, (p + 1) * w)
            for c in range(D // MC):
                at_s[pl.ds(c * MC, MC), cs] = jnp.dot(woT[pl.ds(c * MC, MC), :], _as_bf16(otp_s[:, cs]),
                                                      preferred_element_type=f32).astype(bf16)

    LW = 2 * WIN

    def ln2_strip(t):
        cs = slice(t * LW, (t + 1) * LW)
        for r0 in range(0, D, 32):
            h_s[r0:r0 + 32, cs] = (xr_s[r0:r0 + 32, cs].astype(f32) + at_s[r0:r0 + 32, cs].astype(f32)).astype(bf16)
        m, rstd = _ln_stats(lambda r0, n: h_s[r0:r0 + n, cs].astype(f32))
        racc = None
        for r0 in range(0, D, 48):
            hf = h_s[r0:r0 + 48, cs].astype(f32)
            hn = ((hf - m) * rstd).astype(bf16)
            hn_s[r0:r0 + 48, cs] = hn
            hnf = hn.astype(f32)
            out_s[r0:r0 + 48, cs] = (hf + hnf).astype(bf16)
            wr = wr_s[r0:r0 + 48, :]
            p = _fold8(hnf * jnp.concatenate([wr] * (LW // WIN), axis=1))
            racc = p if racc is None else racc + p
        return jnp.sum(racc, axis=0, keepdims=True)

    def ln2(s):
        rs = [ln2_strip(t) for t in range(L // LW)]
        out_copy(s).start()
        r = jnp.concatenate(rs, axis=1).astype(bf16).astype(f32)
        rmax = jnp.max(r)
        ridx = lax.broadcasted_iota(jnp.int32, (1, L), 1)
        amax = jnp.min(jnp.where(r == rmax, ridx, L))

        @pl.when(rmax > best_s[0])
        def _():
            best_s[0] = rmax
            best_s[1] = (amax + s * L).astype(f32)
            ts = pl.ds(pl.multiple_of((amax >> 7) << 7, WIN), WIN)
            bh_s[...] = h_s[:, ts]
            bhn_s[...] = hn_s[:, ts]

    xl_copy(0).wait()
    small_copy(0).start()
    small_copy(1).start()
    for t in range(L // WIN):
        ln1_tile(t)
    wq_copy(0).wait()
    w_copy(3).start()
    fence()
    xl_copy(1).start()
    fence()
    xr_copy(0).start()
    wT[pl.ds(0, WQA), :] = wraw[0, :, 0:WQA].T
    proj_q(0, 2)
    wq_copy(1).wait()
    wT[pl.ds(WQA, D - WQA), :] = wraw[0, :, WQA:D].T
    proj_q(2, 4)
    w_copy(1).wait()
    wT[pl.ds(D, D), :] = wraw[1].T
    proj_q(4, D // MC)
    w_copy(2).wait()
    wT[pl.ds(2 * D, D), :] = wraw[2].T
    proj_k()
    w_copy(3).wait()
    small_copy(0).wait()
    small_copy(1).wait()
    transpose_k()
    woT[...] = wraw[3].T
    small_setup()
    proj_v()
    b_all0()

    def segment(s, carry):
        @pl.when(s + 1 < NSEG)
        def _():
            xl_copy(s + 1).wait()

        attention()

        @pl.when(s > 0)
        def _():
            out_copy(s - 1).wait()

        xr_copy(s).wait()

        @pl.when(s + 2 < NSEG)
        def _():
            xl_copy(s + 2).start()

        fence()
        for i in range(3):
            @pl.when(s == i)
            def _():
                moe_copy(i).start()

        @pl.when(s + 1 < NSEG)
        def _():
            out_proj()
            proj_v()
            proj_k()
            transpose_k()
            proj_q()
            mem_read()
            b_all0()
            ln2(s)
            xr_copy(s + 1).start()

        @pl.when(s + 1 == NSEG)
        def _():
            out_proj(2)
            ln2(s)

        return carry

    lax.fori_loop(0, NSEG, segment, 0)

    idx = best_s[1].astype(jnp.int32)
    tile = pl.ds(pl.multiple_of((idx >> 7) << 7, WIN), WIN)
    lane = idx & (WIN - 1)
    for i in range(3):
        moe_copy(i).wait()
    hn_t = bhn_s[...]
    onehot = (lax.broadcasted_iota(jnp.int32, (16, WIN), 1) == lane).astype(f32).astype(bf16)
    xs = lax.dot_general(onehot, hn_t, NT, preferred_element_type=f32).astype(bf16)
    FC = 4 * WIN
    RB = 64
    for c in range(F // FC):
        cs = slice(c * FC, (c + 1) * FC)
        gt = jnp.dot(xs, wg_v[:, cs], preferred_element_type=f32)[0:8].astype(bf16).astype(f32)
        up = jnp.dot(xs, wu_v[:, cs], preferred_element_type=f32)[0:8].astype(bf16).astype(f32)
        act = (gt * (1.0 / (1.0 + jnp.exp(-gt)))).astype(bf16).astype(f32) * up
        act = act.astype(bf16).astype(f32)
        for rb in range(D // RB):
            p = acc_s[rb * RB:(rb + 1) * RB, :]
            for t in range(0, FC // WIN, 2):
                w2 = wd_v[rb * RB:(rb + 1) * RB, c * FC + t * WIN:c * FC + (t + 2) * WIN].astype(f32)
                w2 = w2 * act[0:1, t * WIN:(t + 2) * WIN]
                p = p + w2[:, 0:WIN] + w2[:, WIN:2 * WIN]
            acc_s[rb * RB:(rb + 1) * RB, :] = p
    y = jnp.sum(acc_s[...], axis=1, keepdims=True)
    rsel = jnp.full((1, 1), best_s[0], f32)
    y = y.astype(bf16).astype(f32) * (1.0 / (1.0 + jnp.exp(-rsel)))
    lanes = lax.broadcasted_iota(jnp.int32, (D, WIN), 1)
    yt = jnp.where(lanes == lane, y.astype(bf16).astype(f32), 0.0)
    t = (hn_t.astype(f32) + yt).astype(bf16).astype(f32)
    out_copy(NSEG - 1).wait()
    fix_s[...] = (bh_s[...].astype(f32) + t).astype(bf16)
    fix = pltpu.make_async_copy(fix_s, out_hbm.at[:, tile], sem_o.at[0])
    fix.start()
    fix.wait()


@jax.jit
def pallas_sequential_preLN__memory_aug_infini_attn__moe_arch_mod__prompt_kernel(
    A_x: jax.Array,
    A_wq: jax.Array,
    A_wk: jax.Array,
    A_wv: jax.Array,
    A_wo: jax.Array,
    A_beta: jax.Array,
    B_x: jax.Array,
    B_w_r: jax.Array,
    B_w_gate: jax.Array,
    B_w_up: jax.Array,
    B_w_down: jax.Array,
):
    del B_x
    hbm = pl.BlockSpec(memory_space=pltpu.HBM)
    out_t = pl.pallas_call(
        _kernel,
        out_shape=jax.ShapeDtypeStruct((D, S), bf16),
        in_specs=[hbm] * 10,
        out_specs=hbm,
        scratch_shapes=[
            pltpu.VMEM((D, L), bf16),
            pltpu.VMEM((D, L), bf16),
            pltpu.VMEM((4, D, D), bf16),
            pltpu.VMEM((3 * D, D), bf16),
            pltpu.VMEM((D, D), bf16),
            pltpu.VMEM((D, F), bf16),
            pltpu.VMEM((D, F), bf16),
            pltpu.VMEM((D, F), bf16),
            pltpu.VMEM((D, WIN), bf16),
            pltpu.VMEM((D // 2, L), u32),
            pltpu.VMEM((D, L), bf16),
            pltpu.VMEM((D, L), bf16),
            pltpu.VMEM((D, L), bf16),
            pltpu.VMEM((NG, L, WIN), bf16),
            pltpu.VMEM((D, L), bf16),
            pltpu.VMEM((D, L), bf16),
            pltpu.VMEM((1280, G * WIN), f32),
            pltpu.VMEM((1280, G * WIN), f32),
            pltpu.VMEM((4, 8, G * WIN), f32),
            pltpu.VMEM((4, 8, G * WIN), f32),
            pltpu.VMEM((NG, VW, L), f32),
            pltpu.VMEM((NG, VW, WIN), f32),
            pltpu.VMEM((2, VW, WIN), f32),
            pltpu.VMEM((D, L), f32),
            pltpu.VMEM((D // 2, L), u32),
            pltpu.VMEM((D, L), bf16),
            pltpu.VMEM((D, WIN), f32),
            pltpu.VMEM((D, WIN), f32),
            pltpu.VMEM((D, L), bf16),
            pltpu.VMEM((D, L), bf16),
            pltpu.VMEM((D, L), bf16),
            pltpu.VMEM((D, WIN), bf16),
            pltpu.VMEM((D, WIN), bf16),
            pltpu.VMEM((D, WIN), bf16),
            pltpu.VMEM((D, WIN), f32),
            pltpu.VMEM((1, H), bf16),
            pltpu.VMEM((D,), bf16),
            pltpu.SMEM((2,), f32),
            pltpu.SemaphoreType.DMA((2,)),
            pltpu.SemaphoreType.DMA((5,)),
            pltpu.SemaphoreType.DMA((3,)),
            pltpu.SemaphoreType.DMA((1,)),
            pltpu.SemaphoreType.DMA((2,)),
            pltpu.SemaphoreType.REGULAR,
        ],
        compiler_params=pltpu.CompilerParams(vmem_limit_bytes=100 * 1024 * 1024),
    )(A_x.reshape(S, D).T, A_wq, A_wk, A_wv, A_wo, A_beta.reshape(1, H), B_w_r,
      B_w_gate, B_w_up, B_w_down.T)
    return out_t.T.reshape(1, S, D)
```

```python
import os
import jax
import jax.numpy as jnp
from jax import lax
import jax.experimental.pallas as pl
import jax.experimental.pallas.tpu as pltpu

S = 2048
D = 576
H = 32
DH = 18
NSEG = 4
L = 512
F = 4608
G = 4
NG = H // G
GD = G * DH
WIN = 128
VW = 80
MC = 96
LOG2E = 1.4426950408889634
SCALE = 0.2353515625
QSCALE = SCALE * LOG2E
MASKV = -1e9 * LOG2E
EPS = 1e-5
SOFF = (0, 128, 384, 768)
CHUNKS = [(j, i) for j in (3, 2, 1, 0) for i in range(j + 1)]
f32 = jnp.float32
bf16 = jnp.bfloat16
u32 = jnp.uint32
NT = (((1,), (1,)), ((), ()))
ONES2 = 0x3F803F80


def _fdiv18(i):
    return jnp.floor((i.astype(f32) + 0.5) * (1.0 / DH)).astype(jnp.int32)


def _phi(t):
    return jnp.where(t > 0, t + 1.0, jnp.exp(t))


def _fold8(x):
    parts = [x[i:i + 8] for i in range(0, x.shape[0], 8)]
    while len(parts) > 1:
        parts = [parts[i] + parts[i + 1] if i + 1 < len(parts) else parts[i] for i in range(0, len(parts), 2)]
    return parts[0]


def _colsum(load, rb):
    acc = _fold8(load(0, rb))
    for r0 in range(rb, D, rb):
        acc = acc + _fold8(load(r0, rb))
    return jnp.sum(acc, axis=0, keepdims=True)


def _ln_stats(load):
    m = _colsum(load, 64) * (1.0 / D)

    def sq(r0, n):
        xc = load(r0, n) - m
        return xc * xc

    v = _colsum(sq, 96) * (1.0 / D)
    return m, lax.rsqrt(v + EPS)


def _recip(x):
    r = pl.reciprocal(x, approx=True)
    return r * (2.0 - x * r)


def _woff(par):
    return 16 * ((GD * par) // 16)


def _free0(par):
    return GD if par == 0 else 0


def _as_bf16(x):
    return pltpu.bitcast(x, bf16)


def _as_u32(x):
    return pltpu.bitcast(x, u32)


def _pad_rows(a, n):
    return jnp.concatenate([a, jnp.zeros((n - a.shape[0], a.shape[1]), a.dtype)], axis=0)


def _kernel(x_hbm, wq_hbm, wk_hbm, wv_hbm, wo_hbm, beta_hbm, wr_hbm, wg_hbm, wu_hbm, wd_hbm,
            out_hbm,
            xl_s, xr_s, wraw, wT, woT, wg_v, wu_v, wd_v,
            xn_s, xnp_s, qt_s, pqt_s, kt_s, k_s, pkt_s, vt_s, stA, stB, mxA, mxB, nd_s, mext_s, mmask_s,
            oT_s, otp_s, at_s, g_s, wr_s, h_s, hn_s, out_s, bh_s, bhn_s, fix_s, acc_s, beta_ref, wr_ref, best_s,
            sem_x, sem_w, sem_moe, sem_o, sem_s, sem_f):
    def cols(s):
        return pl.ds(pl.multiple_of(s * L, L), L)

    def window(pr, par):
        return pl.ds(pl.multiple_of(pr * (2 * GD) + _woff(par), 16), VW)

    def xl_copy(s):
        return pltpu.make_async_copy(x_hbm.at[:, cols(s)], xl_s, sem_x.at[0])

    def xr_copy(s):
        return pltpu.make_async_copy(x_hbm.at[:, cols(s)], xr_s, sem_x.at[1])

    def w_copy(i):
        src = (wq_hbm, wk_hbm, wv_hbm, wo_hbm)[i]
        return pltpu.make_async_copy(src, wraw.at[i], sem_w.at[i])

    WQA = 3 * WIN

    def wq_copy(part):
        cs = pl.ds(0, WQA) if part == 0 else pl.ds(WQA, D - WQA)
        return pltpu.make_async_copy(wq_hbm.at[:, cs], wraw.at[0, :, cs], sem_w.at[0 if part else 4])

    def moe_copy(i):
        src, dst = ((wg_hbm, wg_v), (wu_hbm, wu_v), (wd_hbm, wd_v))[i]
        return pltpu.make_async_copy(src, dst, sem_moe.at[i])

    def out_copy(s):
        return pltpu.make_async_copy(out_s, out_hbm.at[:, cols(s)], sem_o.at[0])

    def small_copy(i):
        src, dst = ((beta_hbm, beta_ref), (wr_hbm, wr_ref))[i]
        return pltpu.make_async_copy(src, dst, sem_s.at[i])

    def fence():
        pl.semaphore_signal(sem_f, 1)
        pl.semaphore_wait(sem_f, 1)

    xl_copy(0).start()
    fence()
    wq_copy(0).start()
    fence()
    wq_copy(1).start()
    fence()
    w_copy(1).start()
    fence()
    w_copy(2).start()

    mext_s[...] = jnp.zeros_like(mext_s)
    k_s[...] = jnp.zeros_like(k_s)
    nd_s[...] = jnp.zeros_like(nd_s)
    acc_s[...] = jnp.zeros_like(acc_s)
    for par in range(2):
        r = lax.broadcasted_iota(jnp.int32, (VW, WIN), 0)
        l = lax.broadcasted_iota(jnp.int32, (VW, WIN), 1)
        free0 = _free0(par)
        hl = _fdiv18(l - 8 * par + DH) - 1
        he = jnp.where((r >= free0) & (r < free0 + 8), r - free0, _fdiv18(r - 8 * par + DH) - 1)
        ok = (he == hl) & (l >= 8 * par) & (l < 8 * par + GD)
        mmask_s[par] = jnp.where(ok, 1.0, 0.0).astype(f32)
    best_s[0] = jnp.float32(-jnp.inf)
    best_s[1] = jnp.float32(0.0)

    def small_setup():
        beta = beta_ref[...].astype(f32)
        gsig = 1.0 / (1.0 + jnp.exp(-beta))
        fi = lax.broadcasted_iota(jnp.int32, (D, H), 0)
        hi = lax.broadcasted_iota(jnp.int32, (D, H), 1)
        gcol = jnp.sum(jnp.where(_fdiv18(fi) == hi, gsig, 0.0), axis=1, keepdims=True)
        g_s[...] = jnp.broadcast_to(gcol, (D, WIN))
        wr_s[...] = jnp.broadcast_to(wr_ref[...].astype(f32).reshape(1, D), (WIN, D)).T

    kq_r = lax.broadcasted_iota(jnp.int32, (WIN, G * WIN), 0)
    kq_c = lax.broadcasted_iota(jnp.int32, (WIN, G * WIN), 1) & (WIN - 1)
    r40 = lax.broadcasted_iota(jnp.int32, (VW // 2, WIN), 0)

    def ln1_tile(t, tie=None):
        cs = pl.ds(pl.multiple_of(t * WIN, WIN), WIN) if not isinstance(t, int) else slice(t * WIN, (t + 1) * WIN)
        first = (lambda r0, n: xl_s[r0:r0 + n, cs].astype(f32)) if tie is None else (
            lambda r0, n: xl_s[r0:r0 + n, cs].astype(f32) + tie)
        m = _colsum(first, 64) * (1.0 / D)

        def sq(r0, n):
            xc = xl_s[r0:r0 + n, cs].astype(f32) - m
            return xc * xc

        rstd = lax.rsqrt(_colsum(sq, 96) * (1.0 / D) + EPS)
        for r0 in range(0, D, 48):
            xn_s[t if isinstance(t, int) else 0, r0:r0 + 48, :] = ((xl_s[r0:r0 + 48, cs].astype(f32) - m) * rstd).astype(bf16)
        xnp_s[:, cs] = _as_u32(xn_s[t if isinstance(t, int) else 0])

    def proj(base, c):
        return jnp.dot(wT[pl.ds(base + c * MC, MC), :], _as_bf16(xnp_s[...]), preferred_element_type=f32)

    def proj_q(c0=0, c1=D // MC):
        for c in range(c0, c1):
            q = proj(0, c)
            qt_s[pl.ds(c * MC, MC), :] = (q * QSCALE).astype(bf16)
            pqt_s[pl.ds(c * MC, MC), :] = _phi(q).astype(bf16)

    def proj_k(c0=0, c1=D // MC):
        for c in range(c0, c1):
            k = proj(D, c)
            kt_s[pl.ds(c * MC, MC), :] = k.astype(bf16)
            pkt_s[pl.ds(c * MC, MC), :] = _phi(k).astype(bf16)

    def transpose_k():
        for g in range(NG):
            k_s[g, :, 0:VW] = kt_s[window(g // 2, g % 2), :].T

    def proj_v():
        for c in range(D // MC):
            vt_s[pl.ds(c * MC, MC), :] = proj(2 * D, c).astype(bf16)

    def mem_read():
        r80 = lax.broadcasted_iota(jnp.int32, (VW, L), 0)
        for g in range(NG):
            par = g % 2
            rows = window(g // 2, par)
            nd = jnp.dot(mext_s[g].astype(bf16), _pad_rows(pqt_s[rows, :], WIN), preferred_element_type=f32)
            rden = 1.0 / (nd[_free0(par):_free0(par) + 8] + 1e-6)
            scale = jnp.broadcast_to(rden[0:1], (VW, L))
            for a in range(1, G):
                scale = jnp.where(r80 >= 8 * par + a * DH, rden[a:a + 1], scale)
            nd_s[g] = nd * scale * jnp.concatenate([g_s[rows, :]] * (L // WIN), axis=1)

    def mem_update(g):
        free0 = _free0(g % 2) // 2
        rows = window(g // 2, g % 2)
        r = lax.broadcasted_iota(jnp.int32, (VW // 2, L), 0)
        lhs = _as_u32(vt_s[rows, :])
        lhs = _as_bf16(jnp.where((r >= free0) & (r < free0 + 4), u32(ONES2), lhs))
        upd = lax.dot_general(lhs, _pad_rows(pkt_s[rows, :], WIN), NT, preferred_element_type=f32)
        mext_s[g] += jnp.where(mmask_s[g % 2] > 0.5, upd, 0.0)

    def b_chunk(pr, par, st, mx, state, j, i):
        if i == 0:
            q = _as_u32(qt_s[window(pr, par), j * WIN:(j + 1) * WIN])
            lo = 4 * par
            state["rhs"] = jnp.concatenate(
                [_as_bf16(_pad_rows(jnp.where((r40 >= lo + 9 * a) & (r40 < lo + 9 * a + 9), q, u32(0)), WIN // 2))
                 for a in range(G)], axis=1)
        s = jnp.dot(k_s[2 * pr + par, i * WIN:(i + 1) * WIN, :], state["rhs"], preferred_element_type=f32)
        if i == j:
            s = s + jnp.where(kq_r > kq_c, MASKV, 0.0)
        m = jnp.max(s, axis=0, keepdims=True)
        state["m"] = m if i == 0 else jnp.maximum(state["m"], m)
        st[SOFF[j] + i * WIN:SOFF[j] + (i + 1) * WIN, :] = s
        if i == j:
            mx[j] = jnp.broadcast_to(state["m"], (8, G * WIN))

    def c_chunk(pr, par, st, mx, state, j, i):
        g = 2 * pr + par
        for a in range(G):
            row = par * GD + a * DH
            start = (row // 16) * 16
            off = row - start
            rows = pl.ds(pl.multiple_of(pr * (2 * GD) + start, 16), 32)
            one_row = ((off + DH) % 32) // 2
            r16 = lax.broadcasted_iota(jnp.int32, (16, WIN), 0)
            vt = _as_u32(vt_s[rows, i * WIN:(i + 1) * WIN])
            vt = _as_bf16(jnp.where(r16 == one_row, u32(ONES2), vt))
            hs = slice(a * WIN, (a + 1) * WIN)
            p = jnp.exp2(st[SOFF[j] + i * WIN:SOFF[j] + (i + 1) * WIN, hs] - mx[j, 0:1, hs]).astype(bf16)
            d = jnp.dot(vt, p, preferred_element_type=f32)
            acc = d if i == 0 else state[a] + d
            state[a] = acc
            if i == j:
                qs = slice(j * WIN, (j + 1) * WIN)
                lsum = acc[2 * one_row:2 * one_row + 1, :]
                ls = start - _woff(par)
                o = nd_s[g, ls:ls + 32, qs] + ((1.0 - g_s[rows, :]) * _recip(lsum)) * acc
                r32 = lax.broadcasted_iota(jnp.int32, (32, WIN), 0)
                keep = (r32 >= off) & (r32 < off + DH)
                pltpu.store(oT_s.at[rows, qs], o, mask=keep)

    bufs = ((stA, mxA), (stB, mxB))

    def b_all0():
        sb = {}
        for (j, i) in CHUNKS:
            b_chunk(0, 0, *bufs[0], sb, j, i)

    def step(pr, par):
        npr, npar = (pr, 1) if par == 0 else (pr + 1, 0)
        sb, sc = {}, {}
        for (j, i) in CHUNKS:
            b_chunk(npr, npar, *bufs[1 - par], sb, j, i)
            c_chunk(pr, par, *bufs[par], sc, j, i)

    def attention():
        def body(t, c):
            step(t, 0)
            step(t, 1)
            return c
        lax.fori_loop(0, NG // 2 - 1, body, 0)
        step(NG // 2 - 1, 0)
        sc = {}
        for n, (j, i) in enumerate(CHUNKS):
            if n < NG:
                mem_update(n)
            c_chunk(NG // 2 - 1, 1, *bufs[1], sc, j, i)

    def pack_ot():
        at_s[...] = oT_s[...].astype(bf16)
        otp_s[...] = _as_u32(at_s[...])

    def out_proj(nsplit=1, with_ln1=False):
        pack_ot()
        w = L // nsplit
        for p in range(nsplit):
            cs = slice(p * w, (p + 1) * w)
            for c in range(D // MC):
                a = jnp.dot(woT[pl.ds(c * MC, MC), :], _as_bf16(otp_s[:, cs]), preferred_element_type=f32)
                at_s[pl.ds(c * MC, MC), cs] = a.astype(bf16)
                if with_ln1 and c < L // WIN:
                    bits = pltpu.bitcast(a[0:8, c * WIN:(c + 1) * WIN], u32)
                    zero = pltpu.bitcast(lax.shift_right_logical(lax.shift_right_logical(bits, u32(16)), u32(16)), f32)
                    ln1_tile(c, zero[0:1, :])

    LW = 2 * WIN

    def ln2_strip(t):
        cs = slice(t * LW, (t + 1) * LW)
        for r0 in range(0, D, 32):
            h_s[r0:r0 + 32, cs] = (xr_s[r0:r0 + 32, cs].astype(f32) + at_s[r0:r0 + 32, cs].astype(f32)).astype(bf16)
        m, rstd = _ln_stats(lambda r0, n: h_s[r0:r0 + n, cs].astype(f32))
        racc = None
        for r0 in range(0, D, 48):
            hf = h_s[r0:r0 + 48, cs].astype(f32)
            hn = ((hf - m) * rstd).astype(bf16)
            hn_s[r0:r0 + 48, cs] = hn
            hnf = hn.astype(f32)
            out_s[r0:r0 + 48, cs] = (hf + hnf).astype(bf16)
            wr = wr_s[r0:r0 + 48, :]
            p = _fold8(hnf * jnp.concatenate([wr] * (LW // WIN), axis=1))
            racc = p if racc is None else racc + p
        return jnp.sum(racc, axis=0, keepdims=True)

    def ln2(s):
        rs = [ln2_strip(t) for t in range(L // LW)]
        out_copy(s).start()
        r = jnp.concatenate(rs, axis=1).astype(bf16).astype(f32)
        rmax = jnp.max(r)
        ridx = lax.broadcasted_iota(jnp.int32, (1, L), 1)
        amax = jnp.min(jnp.where(r == rmax, ridx, L))

        @pl.when(rmax > best_s[0])
        def _():
            best_s[0] = rmax
            best_s[1] = (amax + s * L).astype(f32)
            ts = pl.ds(pl.multiple_of((amax >> 7) << 7, WIN), WIN)
            bh_s[...] = h_s[:, ts]
            bhn_s[...] = hn_s[:, ts]

    xl_copy(0).wait()
    small_copy(0).start()
    small_copy(1).start()
    for t in range(L // WIN):
        ln1_tile(t)
    wq_copy(0).wait()
    w_copy(3).start()
    fence()
    xl_copy(1).start()
    fence()
    xr_copy(0).start()
    wT[pl.ds(0, WQA), :] = wraw[0, :, 0:WQA].T
    proj_q(0, 4)
    wq_copy(1).wait()
    w_copy(1).wait()
    wT[pl.ds(WQA, D - WQA), :] = wraw[0, :, WQA:D].T
    wT[pl.ds(D, D), :] = wraw[1].T
    proj_q(4, D // MC)
    proj_k(0, 4)
    w_copy(2).wait()
    w_copy(3).wait()
    small_copy(0).wait()
    small_copy(1).wait()
    wT[pl.ds(2 * D, D), :] = wraw[2].T
    woT[...] = wraw[3].T
    small_setup()
    proj_k(4, D // MC)
    transpose_k()
    proj_v()
    b_all0()

    def segment(s, carry):
        attention()

        @pl.when(s > 0)
        def _():
            out_copy(s - 1).wait()

        xr_copy(s).wait()

        @pl.when(s + 1 < NSEG)
        def _():
            xl_copy(s + 1).wait()

        fence()
        for i in range(3):
            @pl.when(s == i)
            def _():
                moe_copy(i).start()

        @pl.when(s + 1 < NSEG)
        def _():
            out_proj(1, True)
            proj_v()
            proj_k()
            transpose_k()
            proj_q()
            mem_read()
            b_all0()
            ln2(s)
            xr_copy(s + 1).start()

            @pl.when(s + 2 < NSEG)
            def _():
                xl_copy(s + 2).start()

        @pl.when(s + 1 == NSEG)
        def _():
            out_proj(2)
            ln2(s)

        return carry

    lax.fori_loop(0, NSEG, segment, 0)

    idx = best_s[1].astype(jnp.int32)
    tile = pl.ds(pl.multiple_of((idx >> 7) << 7, WIN), WIN)
    lane = idx & (WIN - 1)
    for i in range(3):
        moe_copy(i).wait()
    hn_t = bhn_s[...]
    onehot = (lax.broadcasted_iota(jnp.int32, (16, WIN), 1) == lane).astype(f32).astype(bf16)
    xs = lax.dot_general(onehot, hn_t, NT, preferred_element_type=f32).astype(bf16)
    FC = 4 * WIN
    RB = 64
    for c in range(F // FC):
        cs = slice(c * FC, (c + 1) * FC)
        gt = jnp.dot(xs, wg_v[:, cs], preferred_element_type=f32)[0:8].astype(bf16).astype(f32)
        up = jnp.dot(xs, wu_v[:, cs], preferred_element_type=f32)[0:8].astype(bf16).astype(f32)
        act = (gt * (1.0 / (1.0 + jnp.exp(-gt)))).astype(bf16).astype(f32) * up
        act = act.astype(bf16).astype(f32)
        for rb in range(D // RB):
            p = acc_s[rb * RB:(rb + 1) * RB, :]
            for t in range(0, FC // WIN, 2):
                w2 = wd_v[rb * RB:(rb + 1) * RB, c * FC + t * WIN:c * FC + (t + 2) * WIN].astype(f32)
                w2 = w2 * act[0:1, t * WIN:(t + 2) * WIN]
                p = p + w2[:, 0:WIN] + w2[:, WIN:2 * WIN]
            acc_s[rb * RB:(rb + 1) * RB, :] = p
    y = jnp.sum(acc_s[...], axis=1, keepdims=True)
    rsel = jnp.full((1, 1), best_s[0], f32)
    y = y.astype(bf16).astype(f32) * (1.0 / (1.0 + jnp.exp(-rsel)))
    lanes = lax.broadcasted_iota(jnp.int32, (D, WIN), 1)
    yt = jnp.where(lanes == lane, y.astype(bf16).astype(f32), 0.0)
    t = (hn_t.astype(f32) + yt).astype(bf16).astype(f32)
    out_copy(NSEG - 1).wait()
    fix_s[...] = (bh_s[...].astype(f32) + t).astype(bf16)
    fix = pltpu.make_async_copy(fix_s, out_hbm.at[:, tile], sem_o.at[0])
    fix.start()
    fix.wait()


@jax.jit
def pallas_sequential_preLN__memory_aug_infini_attn__moe_arch_mod__prompt_kernel(
    A_x: jax.Array,
    A_wq: jax.Array,
    A_wk: jax.Array,
    A_wv: jax.Array,
    A_wo: jax.Array,
    A_beta: jax.Array,
    B_x: jax.Array,
    B_w_r: jax.Array,
    B_w_gate: jax.Array,
    B_w_up: jax.Array,
    B_w_down: jax.Array,
):
    del B_x
    hbm = pl.BlockSpec(memory_space=pltpu.HBM)
    out_t = pl.pallas_call(
        _kernel,
        out_shape=jax.ShapeDtypeStruct((D, S), bf16),
        in_specs=[hbm] * 10,
        out_specs=hbm,
        scratch_shapes=[
            pltpu.VMEM((D, L), bf16),
            pltpu.VMEM((D, L), bf16),
            pltpu.VMEM((4, D, D), bf16),
            pltpu.VMEM((3 * D, D), bf16),
            pltpu.VMEM((D, D), bf16),
            pltpu.VMEM((D, F), bf16),
            pltpu.VMEM((D, F), bf16),
            pltpu.VMEM((D, F), bf16),
            pltpu.VMEM((4, D, WIN), bf16),
            pltpu.VMEM((D // 2, L), u32),
            pltpu.VMEM((D, L), bf16),
            pltpu.VMEM((D, L), bf16),
            pltpu.VMEM((D, L), bf16),
            pltpu.VMEM((NG, L, WIN), bf16),
            pltpu.VMEM((D, L), bf16),
            pltpu.VMEM((D, L), bf16),
            pltpu.VMEM((1280, G * WIN), f32),
            pltpu.VMEM((1280, G * WIN), f32),
            pltpu.VMEM((4, 8, G * WIN), f32),
            pltpu.VMEM((4, 8, G * WIN), f32),
            pltpu.VMEM((NG, VW, L), f32),
            pltpu.VMEM((NG, VW, WIN), f32),
            pltpu.VMEM((2, VW, WIN), f32),
            pltpu.VMEM((D, L), f32),
            pltpu.VMEM((D // 2, L), u32),
            pltpu.VMEM((D, L), bf16),
            pltpu.VMEM((D, WIN), f32),
            pltpu.VMEM((D, WIN), f32),
            pltpu.VMEM((D, L), bf16),
            pltpu.VMEM((D, L), bf16),
            pltpu.VMEM((D, L), bf16),
            pltpu.VMEM((D, WIN), bf16),
            pltpu.VMEM((D, WIN), bf16),
            pltpu.VMEM((D, WIN), bf16),
            pltpu.VMEM((D, WIN), f32),
            pltpu.VMEM((1, H), bf16),
            pltpu.VMEM((D,), bf16),
            pltpu.SMEM((2,), f32),
            pltpu.SemaphoreType.DMA((2,)),
            pltpu.SemaphoreType.DMA((5,)),
            pltpu.SemaphoreType.DMA((3,)),
            pltpu.SemaphoreType.DMA((1,)),
            pltpu.SemaphoreType.DMA((2,)),
            pltpu.SemaphoreType.REGULAR,
        ],
        compiler_params=pltpu.CompilerParams(vmem_limit_bytes=100 * 1024 * 1024),
    )(A_x.reshape(S, D).T, A_wq, A_wk, A_wv, A_wo, A_beta.reshape(1, H), B_w_r,
      B_w_gate, B_w_up, B_w_down.T)
    return out_t.T.reshape(1, S, D)
```

```python
import os
import jax
import jax.numpy as jnp
from jax import lax
import jax.experimental.pallas as pl
import jax.experimental.pallas.tpu as pltpu

S = 2048
D = 576
H = 32
DH = 18
NSEG = 4
L = 512
F = 4608
G = 4
NG = H // G
GD = G * DH
WIN = 128
VW = 80
MC = 96
LOG2E = 1.4426950408889634
SCALE = 0.2353515625
QSCALE = SCALE * LOG2E
MASKV = -1e9 * LOG2E
EPS = 1e-5
SOFF = (0, 128, 384, 768)
CHUNKS = [(j, i) for j in (3, 2, 1, 0) for i in range(j + 1)]
f32 = jnp.float32
bf16 = jnp.bfloat16
u32 = jnp.uint32
NT = (((1,), (1,)), ((), ()))
ONES2 = 0x3F803F80


def _fdiv18(i):
    return jnp.floor((i.astype(f32) + 0.5) * (1.0 / DH)).astype(jnp.int32)


def _phi(t):
    return jnp.where(t > 0, t + 1.0, jnp.exp(t))


def _fold8(x):
    parts = [x[i:i + 8] for i in range(0, x.shape[0], 8)]
    while len(parts) > 1:
        parts = [parts[i] + parts[i + 1] if i + 1 < len(parts) else parts[i] for i in range(0, len(parts), 2)]
    return parts[0]


def _colsum(load, rb):
    acc = _fold8(load(0, rb))
    for r0 in range(rb, D, rb):
        acc = acc + _fold8(load(r0, rb))
    return jnp.sum(acc, axis=0, keepdims=True)


def _ln_stats(load):
    m = _colsum(load, 64) * (1.0 / D)

    def sq(r0, n):
        xc = load(r0, n) - m
        return xc * xc

    v = _colsum(sq, 96) * (1.0 / D)
    return m, lax.rsqrt(v + EPS)


def _recip(x):
    r = pl.reciprocal(x, approx=True)
    return r * (2.0 - x * r)


def _woff(par):
    return 16 * ((GD * par) // 16)


def _free0(par):
    return GD if par == 0 else 0


def _as_bf16(x):
    return pltpu.bitcast(x, bf16)


def _as_u32(x):
    return pltpu.bitcast(x, u32)


def _pad_rows(a, n):
    return jnp.concatenate([a, jnp.zeros((n - a.shape[0], a.shape[1]), a.dtype)], axis=0)


def _kernel(x_hbm, wq_hbm, wk_hbm, wv_hbm, wo_hbm, beta_hbm, wr_hbm, wg_hbm, wu_hbm, wd_hbm,
            out_hbm,
            xl_s, xr_s, wraw, wT, woT, wg_v, wu_v, wd_v,
            xn_s, xnp_s, qt_s, pqt_s, kt_s, k_s, pkt_s, vt_s, stA, stB, mxA, mxB, nd_s, mext_s, mmask_s,
            oT_s, otp_s, at_s, g_s, wr_s, h_s, hn_s, out_s, bh_s, bhn_s, fix_s, acc_s, beta_ref, wr_ref, best_s,
            sem_x, sem_w, sem_moe, sem_o, sem_s, sem_f):
    def cols(s):
        return pl.ds(pl.multiple_of(s * L, L), L)

    def window(pr, par):
        return pl.ds(pl.multiple_of(pr * (2 * GD) + _woff(par), 16), VW)

    def xl_copy(s):
        return pltpu.make_async_copy(x_hbm.at[:, cols(s)], xl_s, sem_x.at[0])

    def xr_copy(s):
        return pltpu.make_async_copy(x_hbm.at[:, cols(s)], xr_s, sem_x.at[1])

    def w_copy(i):
        src = (wq_hbm, wk_hbm, wv_hbm, wo_hbm)[i]
        return pltpu.make_async_copy(src, wraw.at[i], sem_w.at[i])

    WQA = 3 * WIN

    def wq_copy(part):
        cs = pl.ds(0, WQA) if part == 0 else pl.ds(WQA, D - WQA)
        return pltpu.make_async_copy(wq_hbm.at[:, cs], wraw.at[0, :, cs], sem_w.at[0 if part else 4])

    def moe_copy(i):
        src, dst = ((wg_hbm, wg_v), (wu_hbm, wu_v), (wd_hbm, wd_v))[i]
        return pltpu.make_async_copy(src, dst, sem_moe.at[i])

    def out_copy(s):
        return pltpu.make_async_copy(out_s, out_hbm.at[:, cols(s)], sem_o.at[0])

    def small_copy(i):
        src, dst = ((beta_hbm, beta_ref), (wr_hbm, wr_ref))[i]
        return pltpu.make_async_copy(src, dst, sem_s.at[i])

    def fence():
        pl.semaphore_signal(sem_f, 1)
        pl.semaphore_wait(sem_f, 1)

    xl_copy(0).start()
    fence()
    wq_copy(0).start()
    fence()
    wq_copy(1).start()
    fence()
    w_copy(1).start()
    fence()
    w_copy(2).start()

    mext_s[...] = jnp.zeros_like(mext_s)
    k_s[...] = jnp.zeros_like(k_s)
    nd_s[...] = jnp.zeros_like(nd_s)
    acc_s[...] = jnp.zeros_like(acc_s)
    for par in range(2):
        r = lax.broadcasted_iota(jnp.int32, (VW, WIN), 0)
        l = lax.broadcasted_iota(jnp.int32, (VW, WIN), 1)
        free0 = _free0(par)
        hl = _fdiv18(l - 8 * par + DH) - 1
        he = jnp.where((r >= free0) & (r < free0 + 8), r - free0, _fdiv18(r - 8 * par + DH) - 1)
        ok = (he == hl) & (l >= 8 * par) & (l < 8 * par + GD)
        mmask_s[par] = jnp.where(ok, 1.0, 0.0).astype(f32)
    best_s[0] = jnp.float32(-jnp.inf)
    best_s[1] = jnp.float32(0.0)

    def small_setup():
        beta = beta_ref[...].astype(f32)
        gsig = 1.0 / (1.0 + jnp.exp(-beta))
        fi = lax.broadcasted_iota(jnp.int32, (D, H), 0)
        hi = lax.broadcasted_iota(jnp.int32, (D, H), 1)
        gcol = jnp.sum(jnp.where(_fdiv18(fi) == hi, gsig, 0.0), axis=1, keepdims=True)
        g_s[...] = jnp.broadcast_to(gcol, (D, WIN))
        wr_s[...] = jnp.broadcast_to(wr_ref[...].astype(f32).reshape(1, D), (WIN, D)).T

    kq_r = lax.broadcasted_iota(jnp.int32, (WIN, G * WIN), 0)
    kq_c = lax.broadcasted_iota(jnp.int32, (WIN, G * WIN), 1) & (WIN - 1)
    r40 = lax.broadcasted_iota(jnp.int32, (VW // 2, WIN), 0)

    def ln1_tile(t, tie=None):
        cs = pl.ds(pl.multiple_of(t * WIN, WIN), WIN) if not isinstance(t, int) else slice(t * WIN, (t + 1) * WIN)
        first = (lambda r0, n: xl_s[r0:r0 + n, cs].astype(f32)) if tie is None else (
            lambda r0, n: xl_s[r0:r0 + n, cs].astype(f32) + tie)
        m = _colsum(first, 64) * (1.0 / D)

        def sq(r0, n):
            xc = xl_s[r0:r0 + n, cs].astype(f32) - m
            return xc * xc

        rstd = lax.rsqrt(_colsum(sq, 96) * (1.0 / D) + EPS)
        for r0 in range(0, D, 48):
            xn_s[t if isinstance(t, int) else 0, r0:r0 + 48, :] = ((xl_s[r0:r0 + 48, cs].astype(f32) - m) * rstd).astype(bf16)
        xnp_s[:, cs] = _as_u32(xn_s[t if isinstance(t, int) else 0])

    def proj(base, c):
        return jnp.dot(wT[pl.ds(base + c * MC, MC), :], _as_bf16(xnp_s[...]), preferred_element_type=f32)

    def proj_q(c0=0, c1=D // MC):
        for c in range(c0, c1):
            q = proj(0, c)
            qt_s[pl.ds(c * MC, MC), :] = (q * QSCALE).astype(bf16)
            pqt_s[pl.ds(c * MC, MC), :] = _phi(q).astype(bf16)

    def proj_k(c0=0, c1=D // MC):
        for c in range(c0, c1):
            k = proj(D, c)
            kt_s[pl.ds(c * MC, MC), :] = k.astype(bf16)
            pkt_s[pl.ds(c * MC, MC), :] = _phi(k).astype(bf16)

    def transpose_k():
        for g in range(NG):
            k_s[g, :, 0:VW] = kt_s[window(g // 2, g % 2), :].T

    def proj_v():
        for c in range(D // MC):
            vt_s[pl.ds(c * MC, MC), :] = proj(2 * D, c).astype(bf16)

    def mem_read():
        r80 = lax.broadcasted_iota(jnp.int32, (VW, L), 0)
        for g in range(NG):
            par = g % 2
            rows = window(g // 2, par)
            nd = jnp.dot(mext_s[g].astype(bf16), _pad_rows(pqt_s[rows, :], WIN), preferred_element_type=f32)
            rden = 1.0 / (nd[_free0(par):_free0(par) + 8] + 1e-6)
            scale = jnp.broadcast_to(rden[0:1], (VW, L))
            for a in range(1, G):
                scale = jnp.where(r80 >= 8 * par + a * DH, rden[a:a + 1], scale)
            nd_s[g] = nd * scale * jnp.concatenate([g_s[rows, :]] * (L // WIN), axis=1)

    def mem_update(g):
        free0 = _free0(g % 2) // 2
        rows = window(g // 2, g % 2)
        r = lax.broadcasted_iota(jnp.int32, (VW // 2, L), 0)
        lhs = _as_u32(vt_s[rows, :])
        lhs = _as_bf16(jnp.where((r >= free0) & (r < free0 + 4), u32(ONES2), lhs))
        upd = lax.dot_general(lhs, _pad_rows(pkt_s[rows, :], WIN), NT, preferred_element_type=f32)
        mext_s[g] += jnp.where(mmask_s[g % 2] > 0.5, upd, 0.0)

    def b_chunk(pr, par, st, mx, state, j, i):
        if i == 0:
            q = _as_u32(qt_s[window(pr, par), j * WIN:(j + 1) * WIN])
            lo = 4 * par
            state["rhs"] = jnp.concatenate(
                [_as_bf16(_pad_rows(jnp.where((r40 >= lo + 9 * a) & (r40 < lo + 9 * a + 9), q, u32(0)), WIN // 2))
                 for a in range(G)], axis=1)
        s = jnp.dot(k_s[2 * pr + par, i * WIN:(i + 1) * WIN, :], state["rhs"], preferred_element_type=f32)
        if i == j:
            s = s + jnp.where(kq_r > kq_c, MASKV, 0.0)
        m = jnp.max(s, axis=0, keepdims=True)
        state["m"] = m if i == 0 else jnp.maximum(state["m"], m)
        st[SOFF[j] + i * WIN:SOFF[j] + (i + 1) * WIN, :] = s
        if i == j:
            mx[j] = jnp.broadcast_to(state["m"], (8, G * WIN))

    def c_chunk(pr, par, st, mx, state, j, i):
        g = 2 * pr + par
        for a in range(G):
            row = par * GD + a * DH
            start = (row // 16) * 16
            off = row - start
            rows = pl.ds(pl.multiple_of(pr * (2 * GD) + start, 16), 32)
            one_row = ((off + DH) % 32) // 2
            r16 = lax.broadcasted_iota(jnp.int32, (16, WIN), 0)
            vt = _as_u32(vt_s[rows, i * WIN:(i + 1) * WIN])
            vt = _as_bf16(jnp.where(r16 == one_row, u32(ONES2), vt))
            hs = slice(a * WIN, (a + 1) * WIN)
            p = jnp.exp2(st[SOFF[j] + i * WIN:SOFF[j] + (i + 1) * WIN, hs] - mx[j, 0:1, hs]).astype(bf16)
            d = jnp.dot(vt, p, preferred_element_type=f32)
            acc = d if i == 0 else state[a] + d
            state[a] = acc
            if i == j:
                qs = slice(j * WIN, (j + 1) * WIN)
                lsum = acc[2 * one_row:2 * one_row + 1, :]
                ls = start - _woff(par)
                o = nd_s[g, ls:ls + 32, qs] + ((1.0 - g_s[rows, :]) * _recip(lsum)) * acc
                r32 = lax.broadcasted_iota(jnp.int32, (32, WIN), 0)
                keep = (r32 >= off) & (r32 < off + DH)
                pltpu.store(oT_s.at[rows, qs], o, mask=keep)

    bufs = ((stA, mxA), (stB, mxB))

    def b_all0():
        sb = {}
        for (j, i) in CHUNKS:
            b_chunk(0, 0, *bufs[0], sb, j, i)

    def step(pr, par):
        npr, npar = (pr, 1) if par == 0 else (pr + 1, 0)
        sb, sc = {}, {}
        for (j, i) in CHUNKS:
            b_chunk(npr, npar, *bufs[1 - par], sb, j, i)
            c_chunk(pr, par, *bufs[par], sc, j, i)

    def attention_loop():
        def body(t, c):
            step(t, 0)
            step(t, 1)
            return c
        lax.fori_loop(0, NG // 2 - 1, body, 0)

    def attention_tail(last):
        step(NG // 2 - 1, 0)
        sc = {}
        for n, (j, i) in enumerate(CHUNKS):
            if n < NG and not last:
                mem_update(n)
            c_chunk(NG // 2 - 1, 1, *bufs[1], sc, j, i)

    def pack_ot():
        at_s[...] = oT_s[...].astype(bf16)
        otp_s[...] = _as_u32(at_s[...])

    def out_proj(nsplit=1, with_ln1=False):
        pack_ot()
        w = L // nsplit
        for p in range(nsplit):
            cs = slice(p * w, (p + 1) * w)
            for c in range(D // MC):
                a = jnp.dot(woT[pl.ds(c * MC, MC), :], _as_bf16(otp_s[:, cs]), preferred_element_type=f32)
                at_s[pl.ds(c * MC, MC), cs] = a.astype(bf16)
                if with_ln1 and c < L // WIN:
                    bits = pltpu.bitcast(a[0:8, c * WIN:(c + 1) * WIN], u32)
                    zero = pltpu.bitcast(lax.shift_right_logical(lax.shift_right_logical(bits, u32(16)), u32(16)), f32)
                    ln1_tile(c, zero[0:1, :])

    LW = 2 * WIN

    def ln2_strip(t):
        cs = slice(t * LW, (t + 1) * LW)
        for r0 in range(0, D, 32):
            h_s[r0:r0 + 32, cs] = (xr_s[r0:r0 + 32, cs].astype(f32) + at_s[r0:r0 + 32, cs].astype(f32)).astype(bf16)
        m, rstd = _ln_stats(lambda r0, n: h_s[r0:r0 + n, cs].astype(f32))
        racc = None
        for r0 in range(0, D, 48):
            hf = h_s[r0:r0 + 48, cs].astype(f32)
            hn = ((hf - m) * rstd).astype(bf16)
            hn_s[r0:r0 + 48, cs] = hn
            hnf = hn.astype(f32)
            out_s[r0:r0 + 48, cs] = (hf + hnf).astype(bf16)
            wr = wr_s[r0:r0 + 48, :]
            p = _fold8(hnf * jnp.concatenate([wr] * (LW // WIN), axis=1))
            racc = p if racc is None else racc + p
        return jnp.sum(racc, axis=0, keepdims=True)

    def ln2(s):
        rs = [ln2_strip(t) for t in range(L // LW)]
        out_copy(s).start()
        r = jnp.concatenate(rs, axis=1).astype(bf16).astype(f32)
        rmax = jnp.max(r)
        ridx = lax.broadcasted_iota(jnp.int32, (1, L), 1)
        amax = jnp.min(jnp.where(r == rmax, ridx, L))

        @pl.when(rmax > best_s[0])
        def _():
            best_s[0] = rmax
            best_s[1] = (amax + s * L).astype(f32)
            ts = pl.ds(pl.multiple_of((amax >> 7) << 7, WIN), WIN)
            bh_s[...] = h_s[:, ts]
            bhn_s[...] = hn_s[:, ts]

    xl_copy(0).wait()
    small_copy(0).start()
    small_copy(1).start()
    for t in range(L // WIN):
        ln1_tile(t)
    wq_copy(0).wait()
    w_copy(3).start()
    fence()
    xl_copy(1).start()
    fence()
    xr_copy(0).start()
    wT[pl.ds(0, WQA), :] = wraw[0, :, 0:WQA].T
    proj_q(0, 4)
    wq_copy(1).wait()
    w_copy(1).wait()
    wT[pl.ds(WQA, D - WQA), :] = wraw[0, :, WQA:D].T
    wT[pl.ds(D, D), :] = wraw[1].T
    proj_q(4, D // MC)
    proj_k(0, 4)
    w_copy(2).wait()
    w_copy(3).wait()
    small_copy(0).wait()
    small_copy(1).wait()
    wT[pl.ds(2 * D, D), :] = wraw[2].T
    woT[...] = wraw[3].T
    small_setup()
    proj_k(4, D // MC)
    transpose_k()
    proj_v()
    b_all0()

    def segment(s, carry):
        attention_loop()

        @pl.when(s + 1 < NSEG)
        def _():
            attention_tail(False)

        @pl.when(s > 0)
        def _():
            out_copy(s - 1).wait()

        xr_copy(s).wait()

        @pl.when(s + 1 < NSEG)
        def _():
            xl_copy(s + 1).wait()

        fence()
        for i in range(3):
            @pl.when(s == i)
            def _():
                moe_copy(i).start()

        @pl.when(s + 1 < NSEG)
        def _():
            out_proj(1, True)
            proj_v()
            proj_k()
            transpose_k()
            proj_q()
            mem_read()
            b_all0()
            ln2(s)
            xr_copy(s + 1).start()

            @pl.when(s + 2 < NSEG)
            def _():
                xl_copy(s + 2).start()

        @pl.when(s + 1 == NSEG)
        def _():
            attention_tail(True)
            out_proj(2)
            ln2(s)

        return carry

    lax.fori_loop(0, NSEG, segment, 0)

    idx = best_s[1].astype(jnp.int32)
    tile = pl.ds(pl.multiple_of((idx >> 7) << 7, WIN), WIN)
    lane = idx & (WIN - 1)
    for i in range(3):
        moe_copy(i).wait()
    hn_t = bhn_s[...]
    onehot = (lax.broadcasted_iota(jnp.int32, (16, WIN), 1) == lane).astype(f32).astype(bf16)
    xs = lax.dot_general(onehot, hn_t, NT, preferred_element_type=f32).astype(bf16)
    FC = 4 * WIN
    RB = 64
    for c in range(F // FC):
        cs = slice(c * FC, (c + 1) * FC)
        gt = jnp.dot(xs, wg_v[:, cs], preferred_element_type=f32)[0:8].astype(bf16).astype(f32)
        up = jnp.dot(xs, wu_v[:, cs], preferred_element_type=f32)[0:8].astype(bf16).astype(f32)
        act = (gt * (1.0 / (1.0 + jnp.exp(-gt)))).astype(bf16).astype(f32) * up
        act = act.astype(bf16).astype(f32)
        for rb in range(D // RB):
            p = acc_s[rb * RB:(rb + 1) * RB, :]
            for t in range(0, FC // WIN, 2):
                w2 = wd_v[rb * RB:(rb + 1) * RB, c * FC + t * WIN:c * FC + (t + 2) * WIN].astype(f32)
                w2 = w2 * act[0:1, t * WIN:(t + 2) * WIN]
                p = p + w2[:, 0:WIN] + w2[:, WIN:2 * WIN]
            acc_s[rb * RB:(rb + 1) * RB, :] = p
    y = jnp.sum(acc_s[...], axis=1, keepdims=True)
    rsel = jnp.full((1, 1), best_s[0], f32)
    y = y.astype(bf16).astype(f32) * (1.0 / (1.0 + jnp.exp(-rsel)))
    lanes = lax.broadcasted_iota(jnp.int32, (D, WIN), 1)
    yt = jnp.where(lanes == lane, y.astype(bf16).astype(f32), 0.0)
    t = (hn_t.astype(f32) + yt).astype(bf16).astype(f32)
    out_copy(NSEG - 1).wait()
    fix_s[...] = (bh_s[...].astype(f32) + t).astype(bf16)
    fix = pltpu.make_async_copy(fix_s, out_hbm.at[:, tile], sem_o.at[0])
    fix.start()
    fix.wait()


@jax.jit
def pallas_sequential_preLN__memory_aug_infini_attn__moe_arch_mod__prompt_kernel(
    A_x: jax.Array,
    A_wq: jax.Array,
    A_wk: jax.Array,
    A_wv: jax.Array,
    A_wo: jax.Array,
    A_beta: jax.Array,
    B_x: jax.Array,
    B_w_r: jax.Array,
    B_w_gate: jax.Array,
    B_w_up: jax.Array,
    B_w_down: jax.Array,
):
    del B_x
    hbm = pl.BlockSpec(memory_space=pltpu.HBM)
    out_t = pl.pallas_call(
        _kernel,
        out_shape=jax.ShapeDtypeStruct((D, S), bf16),
        in_specs=[hbm] * 10,
        out_specs=hbm,
        scratch_shapes=[
            pltpu.VMEM((D, L), bf16),
            pltpu.VMEM((D, L), bf16),
            pltpu.VMEM((4, D, D), bf16),
            pltpu.VMEM((3 * D, D), bf16),
            pltpu.VMEM((D, D), bf16),
            pltpu.VMEM((D, F), bf16),
            pltpu.VMEM((D, F), bf16),
            pltpu.VMEM((D, F), bf16),
            pltpu.VMEM((4, D, WIN), bf16),
            pltpu.VMEM((D // 2, L), u32),
            pltpu.VMEM((D, L), bf16),
            pltpu.VMEM((D, L), bf16),
            pltpu.VMEM((D, L), bf16),
            pltpu.VMEM((NG, L, WIN), bf16),
            pltpu.VMEM((D, L), bf16),
            pltpu.VMEM((D, L), bf16),
            pltpu.VMEM((1280, G * WIN), f32),
            pltpu.VMEM((1280, G * WIN), f32),
            pltpu.VMEM((4, 8, G * WIN), f32),
            pltpu.VMEM((4, 8, G * WIN), f32),
            pltpu.VMEM((NG, VW, L), f32),
            pltpu.VMEM((NG, VW, WIN), f32),
            pltpu.VMEM((2, VW, WIN), f32),
            pltpu.VMEM((D, L), f32),
            pltpu.VMEM((D // 2, L), u32),
            pltpu.VMEM((D, L), bf16),
            pltpu.VMEM((D, WIN), f32),
            pltpu.VMEM((D, WIN), f32),
            pltpu.VMEM((D, L), bf16),
            pltpu.VMEM((D, L), bf16),
            pltpu.VMEM((D, L), bf16),
            pltpu.VMEM((D, WIN), bf16),
            pltpu.VMEM((D, WIN), bf16),
            pltpu.VMEM((D, WIN), bf16),
            pltpu.VMEM((D, WIN), f32),
            pltpu.VMEM((1, H), bf16),
            pltpu.VMEM((D,), bf16),
            pltpu.SMEM((2,), f32),
            pltpu.SemaphoreType.DMA((2,)),
            pltpu.SemaphoreType.DMA((5,)),
            pltpu.SemaphoreType.DMA((3,)),
            pltpu.SemaphoreType.DMA((1,)),
            pltpu.SemaphoreType.DMA((2,)),
            pltpu.SemaphoreType.REGULAR,
        ],
        compiler_params=pltpu.CompilerParams(vmem_limit_bytes=100 * 1024 * 1024),
    )(A_x.reshape(S, D).T, A_wq, A_wk, A_wv, A_wo, A_beta.reshape(1, H), B_w_r,
      B_w_gate, B_w_up, B_w_down.T)
    return out_t.T.reshape(1, S, D)
```

```python
import os
import jax
import jax.numpy as jnp
from jax import lax
import jax.experimental.pallas as pl
import jax.experimental.pallas.tpu as pltpu

S = 2048
D = 576
H = 32
DH = 18
NSEG = 4
L = 512
F = 4608
G = 4
NG = H // G
GD = G * DH
WIN = 128
VW = 80
MC = 96
LOG2E = 1.4426950408889634
SCALE = 0.2353515625
QSCALE = SCALE * LOG2E
MASKV = -1e9 * LOG2E
EPS = 1e-5
SOFF = (0, 128, 384, 768)
CHUNKS = [(j, i) for j in (3, 2, 1, 0) for i in range(j + 1)]
f32 = jnp.float32
bf16 = jnp.bfloat16
u32 = jnp.uint32
NT = (((1,), (1,)), ((), ()))
ONES2 = 0x3F803F80


def _fdiv18(i):
    return jnp.floor((i.astype(f32) + 0.5) * (1.0 / DH)).astype(jnp.int32)


def _phi(t):
    return jnp.where(t > 0, t + 1.0, jnp.exp(t))


def _fold8(x):
    parts = [x[i:i + 8] for i in range(0, x.shape[0], 8)]
    while len(parts) > 1:
        parts = [parts[i] + parts[i + 1] if i + 1 < len(parts) else parts[i] for i in range(0, len(parts), 2)]
    return parts[0]


def _colsum(load, rb):
    acc = _fold8(load(0, rb))
    for r0 in range(rb, D, rb):
        acc = acc + _fold8(load(r0, rb))
    return jnp.sum(acc, axis=0, keepdims=True)


def _ln_stats(load):
    m = _colsum(load, 64) * (1.0 / D)

    def sq(r0, n):
        xc = load(r0, n) - m
        return xc * xc

    v = _colsum(sq, 96) * (1.0 / D)
    return m, lax.rsqrt(v + EPS)


def _recip(x):
    r = pl.reciprocal(x, approx=True)
    return r * (2.0 - x * r)


def _woff(par):
    return 16 * ((GD * par) // 16)


def _free0(par):
    return GD if par == 0 else 0


def _as_bf16(x):
    return pltpu.bitcast(x, bf16)


def _as_u32(x):
    return pltpu.bitcast(x, u32)


def _pad_rows(a, n):
    return jnp.concatenate([a, jnp.zeros((n - a.shape[0], a.shape[1]), a.dtype)], axis=0)


def _kernel(x_hbm, wq_hbm, wk_hbm, wv_hbm, wo_hbm, beta_hbm, wr_hbm, wg_hbm, wu_hbm, wd_hbm,
            out_hbm,
            xl_s, xr_s, wraw, wT, woT, wg_v, wu_v, wd_v,
            xn_s, xnp_s, qt_s, pqt_s, kt_s, k_s, pkt_s, vt_s, stA, stB, mxA, mxB, nd_s, mext_s, mmask_s,
            oT_s, otp_s, at_s, g_s, wr_s, h_s, hn_s, out_s, bh_s, bhn_s, fix_s, acc_s, beta_ref, wr_ref, best_s, zero_s,
            sem_x, sem_w, sem_moe, sem_o, sem_s, sem_f):
    def cols(s):
        return pl.ds(pl.multiple_of(s * L, L), L)

    def window(pr, par):
        return pl.ds(pl.multiple_of(pr * (2 * GD) + _woff(par), 16), VW)

    def xl_copy(s):
        return pltpu.make_async_copy(x_hbm.at[:, cols(s)], xl_s, sem_x.at[0])

    def xr_copy(s):
        return pltpu.make_async_copy(x_hbm.at[:, cols(s)], xr_s, sem_x.at[1])

    def w_copy(i):
        src = (wq_hbm, wk_hbm, wv_hbm, wo_hbm)[i]
        return pltpu.make_async_copy(src, wraw.at[i], sem_w.at[i])

    WQA = 3 * WIN

    def wq_copy(part):
        cs = pl.ds(0, WQA) if part == 0 else pl.ds(WQA, D - WQA)
        return pltpu.make_async_copy(wq_hbm.at[:, cs], wraw.at[0, :, cs], sem_w.at[0 if part else 4])

    def moe_copy(i):
        src, dst = ((wg_hbm, wg_v), (wu_hbm, wu_v), (wd_hbm, wd_v))[i]
        return pltpu.make_async_copy(src, dst, sem_moe.at[i])

    def out_copy(s):
        return pltpu.make_async_copy(out_s, out_hbm.at[:, cols(s)], sem_o.at[0])

    def small_copy(i):
        src, dst = ((beta_hbm, beta_ref), (wr_hbm, wr_ref))[i]
        return pltpu.make_async_copy(src, dst, sem_s.at[i])

    def fence():
        pl.semaphore_signal(sem_f, 1)
        pl.semaphore_wait(sem_f, 1)

    xl_copy(0).start()
    fence()
    wq_copy(0).start()
    fence()
    wq_copy(1).start()
    fence()
    w_copy(1).start()
    fence()
    w_copy(2).start()

    mext_s[...] = jnp.zeros_like(mext_s)
    k_s[...] = jnp.zeros_like(k_s)
    nd_s[...] = jnp.zeros_like(nd_s)
    acc_s[...] = jnp.zeros_like(acc_s)
    for par in range(2):
        r = lax.broadcasted_iota(jnp.int32, (VW, WIN), 0)
        l = lax.broadcasted_iota(jnp.int32, (VW, WIN), 1)
        free0 = _free0(par)
        hl = _fdiv18(l - 8 * par + DH) - 1
        he = jnp.where((r >= free0) & (r < free0 + 8), r - free0, _fdiv18(r - 8 * par + DH) - 1)
        ok = (he == hl) & (l >= 8 * par) & (l < 8 * par + GD)
        mmask_s[par] = jnp.where(ok, 1.0, 0.0).astype(f32)
    best_s[0] = jnp.float32(-jnp.inf)
    zero_s[0] = jnp.int32(0)
    best_s[1] = jnp.float32(0.0)

    def small_setup():
        beta = beta_ref[...].astype(f32)
        gsig = 1.0 / (1.0 + jnp.exp(-beta))
        fi = lax.broadcasted_iota(jnp.int32, (D, H), 0)
        hi = lax.broadcasted_iota(jnp.int32, (D, H), 1)
        gcol = jnp.sum(jnp.where(_fdiv18(fi) == hi, gsig, 0.0), axis=1, keepdims=True)
        g_s[...] = jnp.broadcast_to(gcol, (D, WIN))
        wr_s[...] = jnp.broadcast_to(wr_ref[...].astype(f32).reshape(1, D), (WIN, D)).T

    kq_r = lax.broadcasted_iota(jnp.int32, (WIN, G * WIN), 0)
    kq_c = lax.broadcasted_iota(jnp.int32, (WIN, G * WIN), 1) & (WIN - 1)
    r40 = lax.broadcasted_iota(jnp.int32, (VW // 2, WIN), 0)

    def ln1_tile(t, tie=None):
        cs = pl.ds(pl.multiple_of(t * WIN, WIN), WIN) if not isinstance(t, int) else slice(t * WIN, (t + 1) * WIN)
        first = (lambda r0, n: xl_s[r0:r0 + n, cs].astype(f32)) if tie is None else (
            lambda r0, n: xl_s[r0:r0 + n, cs].astype(f32) + tie)
        m = _colsum(first, 64) * (1.0 / D)

        def sq(r0, n):
            xc = xl_s[r0:r0 + n, cs].astype(f32) - m
            return xc * xc

        rstd = lax.rsqrt(_colsum(sq, 96) * (1.0 / D) + EPS)
        for r0 in range(0, D, 48):
            xn_s[t if isinstance(t, int) else 0, r0:r0 + 48, :] = ((xl_s[r0:r0 + 48, cs].astype(f32) - m) * rstd).astype(bf16)
        xnp_s[:, cs] = _as_u32(xn_s[t if isinstance(t, int) else 0])

    def proj(base, c):
        return jnp.dot(wT[pl.ds(base + c * MC, MC), :], _as_bf16(xnp_s[...]), preferred_element_type=f32)

    def proj_q(c0=0, c1=D // MC):
        for c in range(c0, c1):
            q = proj(0, c)
            qt_s[pl.ds(c * MC, MC), :] = (q * QSCALE).astype(bf16)
            pqt_s[pl.ds(c * MC, MC), :] = _phi(q).astype(bf16)

    def proj_k(c0=0, c1=D // MC):
        for c in range(c0, c1):
            k = proj(D, c)
            kt_s[pl.ds(c * MC, MC), :] = k.astype(bf16)
            pkt_s[pl.ds(c * MC, MC), :] = _phi(k).astype(bf16)

    def transpose_k():
        for g in range(NG):
            k_s[g, :, 0:VW] = kt_s[window(g // 2, g % 2), :].T

    def proj_v():
        for c in range(D // MC):
            vt_s[pl.ds(c * MC, MC), :] = proj(2 * D, c).astype(bf16)

    def mem_read():
        r80 = lax.broadcasted_iota(jnp.int32, (VW, L), 0)
        for g in range(NG):
            par = g % 2
            rows = window(g // 2, par)
            nd = jnp.dot(mext_s[g].astype(bf16), _pad_rows(pqt_s[rows, :], WIN), preferred_element_type=f32)
            rden = 1.0 / (nd[_free0(par):_free0(par) + 8] + 1e-6)
            scale = jnp.broadcast_to(rden[0:1], (VW, L))
            for a in range(1, G):
                scale = jnp.where(r80 >= 8 * par + a * DH, rden[a:a + 1], scale)
            nd_s[g] = nd * scale * jnp.concatenate([g_s[rows, :]] * (L // WIN), axis=1)

    def mem_update(g):
        free0 = _free0(g % 2) // 2
        rows = window(g // 2, g % 2)
        r = lax.broadcasted_iota(jnp.int32, (VW // 2, L), 0)
        lhs = _as_u32(vt_s[rows, :])
        lhs = _as_bf16(jnp.where((r >= free0) & (r < free0 + 4), u32(ONES2), lhs))
        upd = lax.dot_general(lhs, _pad_rows(pkt_s[rows, :], WIN), NT, preferred_element_type=f32)
        mext_s[g] += jnp.where(mmask_s[g % 2] > 0.5, upd, 0.0)

    def b_chunk(pr, par, st, mx, state, j, i):
        if i == 0:
            q = _as_u32(qt_s[window(pr, par), j * WIN:(j + 1) * WIN])
            lo = 4 * par
            state["rhs"] = jnp.concatenate(
                [_as_bf16(_pad_rows(jnp.where((r40 >= lo + 9 * a) & (r40 < lo + 9 * a + 9), q, u32(0)), WIN // 2))
                 for a in range(G)], axis=1)
        s = jnp.dot(k_s[2 * pr + par, i * WIN:(i + 1) * WIN, :], state["rhs"], preferred_element_type=f32)
        if i == j:
            s = s + jnp.where(kq_r > kq_c, MASKV, 0.0)
        m = jnp.max(s, axis=0, keepdims=True)
        state["m"] = m if i == 0 else jnp.maximum(state["m"], m)
        st[SOFF[j] + i * WIN:SOFF[j] + (i + 1) * WIN, :] = s
        if i == j:
            mx[j] = jnp.broadcast_to(state["m"], (8, G * WIN))

    def c_chunk(pr, par, st, mx, state, j, i):
        g = 2 * pr + par
        for a in range(G):
            row = par * GD + a * DH
            start = (row // 16) * 16
            off = row - start
            rows = pl.ds(pl.multiple_of(pr * (2 * GD) + start, 16), 32)
            one_row = ((off + DH) % 32) // 2
            r16 = lax.broadcasted_iota(jnp.int32, (16, WIN), 0)
            vt = _as_u32(vt_s[rows, i * WIN:(i + 1) * WIN])
            vt = _as_bf16(jnp.where(r16 == one_row, u32(ONES2), vt))
            hs = slice(a * WIN, (a + 1) * WIN)
            p = jnp.exp2(st[SOFF[j] + i * WIN:SOFF[j] + (i + 1) * WIN, hs] - mx[j, 0:1, hs]).astype(bf16)
            d = jnp.dot(vt, p, preferred_element_type=f32)
            acc = d if i == 0 else state[a] + d
            state[a] = acc
            if i == j:
                qs = slice(j * WIN, (j + 1) * WIN)
                lsum = acc[2 * one_row:2 * one_row + 1, :]
                ls = start - _woff(par)
                o = nd_s[g, ls:ls + 32, qs] + ((1.0 - g_s[rows, :]) * _recip(lsum)) * acc
                r32 = lax.broadcasted_iota(jnp.int32, (32, WIN), 0)
                keep = (r32 >= off) & (r32 < off + DH)
                pltpu.store(oT_s.at[rows, qs], o, mask=keep)

    bufs = ((stA, mxA), (stB, mxB))

    def b_all0():
        sb = {}
        for (j, i) in CHUNKS:
            b_chunk(0, 0, *bufs[0], sb, j, i)

    def step(pr, par):
        npr, npar = (pr, 1) if par == 0 else (pr + 1, 0)
        sb, sc = {}, {}
        for (j, i) in CHUNKS:
            b_chunk(npr, npar, *bufs[1 - par], sb, j, i)
            c_chunk(pr, par, *bufs[par], sc, j, i)

    def attention():
        z = zero_s[0]
        for g in range(NG - 1):
            step(z + g // 2, g % 2)
        sc = {}
        for n, (j, i) in enumerate(CHUNKS):
            if n < NG:
                mem_update(n)
            c_chunk(z + NG // 2 - 1, 1, *bufs[1], sc, j, i)

    def pack_ot():
        at_s[...] = oT_s[...].astype(bf16)
        otp_s[...] = _as_u32(at_s[...])

    def out_proj(nsplit=1, with_ln1=False):
        pack_ot()
        w = L // nsplit
        for p in range(nsplit):
            cs = slice(p * w, (p + 1) * w)
            for c in range(D // MC):
                a = jnp.dot(woT[pl.ds(c * MC, MC), :], _as_bf16(otp_s[:, cs]), preferred_element_type=f32)
                at_s[pl.ds(c * MC, MC), cs] = a.astype(bf16)
                if with_ln1 and c < L // WIN:
                    bits = pltpu.bitcast(a[0:8, c * WIN:(c + 1) * WIN], u32)
                    zero = pltpu.bitcast(lax.shift_right_logical(lax.shift_right_logical(bits, u32(16)), u32(16)), f32)
                    ln1_tile(c, zero[0:1, :])

    LW = 2 * WIN

    def ln2_strip(t):
        cs = slice(t * LW, (t + 1) * LW)
        for r0 in range(0, D, 32):
            h_s[r0:r0 + 32, cs] = (xr_s[r0:r0 + 32, cs].astype(f32) + at_s[r0:r0 + 32, cs].astype(f32)).astype(bf16)
        m, rstd = _ln_stats(lambda r0, n: h_s[r0:r0 + n, cs].astype(f32))
        racc = None
        for r0 in range(0, D, 48):
            hf = h_s[r0:r0 + 48, cs].astype(f32)
            hn = ((hf - m) * rstd).astype(bf16)
            hn_s[r0:r0 + 48, cs] = hn
            hnf = hn.astype(f32)
            out_s[r0:r0 + 48, cs] = (hf + hnf).astype(bf16)
            wr = wr_s[r0:r0 + 48, :]
            p = _fold8(hnf * jnp.concatenate([wr] * (LW // WIN), axis=1))
            racc = p if racc is None else racc + p
        return jnp.sum(racc, axis=0, keepdims=True)

    def ln2(s):
        rs = [ln2_strip(t) for t in range(L // LW)]
        out_copy(s).start()
        r = jnp.concatenate(rs, axis=1).astype(bf16).astype(f32)
        rmax = jnp.max(r)
        ridx = lax.broadcasted_iota(jnp.int32, (1, L), 1)
        amax = jnp.min(jnp.where(r == rmax, ridx, L))

        @pl.when(rmax > best_s[0])
        def _():
            best_s[0] = rmax
            best_s[1] = (amax + s * L).astype(f32)
            ts = pl.ds(pl.multiple_of((amax >> 7) << 7, WIN), WIN)
            bh_s[...] = h_s[:, ts]
            bhn_s[...] = hn_s[:, ts]

    xl_copy(0).wait()
    small_copy(0).start()
    small_copy(1).start()
    for t in range(L // WIN):
        ln1_tile(t)
    wq_copy(0).wait()
    w_copy(3).start()
    fence()
    xl_copy(1).start()
    fence()
    xr_copy(0).start()
    wT[pl.ds(0, WQA), :] = wraw[0, :, 0:WQA].T
    proj_q(0, 4)
    wq_copy(1).wait()
    w_copy(1).wait()
    wT[pl.ds(WQA, D - WQA), :] = wraw[0, :, WQA:D].T
    wT[pl.ds(D, D), :] = wraw[1].T
    proj_q(4, D // MC)
    proj_k(0, 4)
    w_copy(2).wait()
    w_copy(3).wait()
    small_copy(0).wait()
    small_copy(1).wait()
    wT[pl.ds(2 * D, D), :] = wraw[2].T
    woT[...] = wraw[3].T
    small_setup()
    proj_k(4, D // MC)
    transpose_k()
    proj_v()
    b_all0()

    def segment(s, carry):
        attention()

        @pl.when(s > 0)
        def _():
            out_copy(s - 1).wait()

        xr_copy(s).wait()

        @pl.when(s + 1 < NSEG)
        def _():
            xl_copy(s + 1).wait()

        fence()
        for i in range(3):
            @pl.when(s == i)
            def _():
                moe_copy(i).start()

        @pl.when(s + 1 < NSEG)
        def _():
            out_proj(1, True)
            proj_v()
            proj_k()
            transpose_k()
            proj_q()
            mem_read()
            b_all0()
            ln2(s)
            xr_copy(s + 1).start()

            @pl.when(s + 2 < NSEG)
            def _():
                xl_copy(s + 2).start()

        @pl.when(s + 1 == NSEG)
        def _():
            out_proj(2)
            ln2(s)

        return carry

    lax.fori_loop(0, NSEG, segment, 0)

    idx = best_s[1].astype(jnp.int32)
    tile = pl.ds(pl.multiple_of((idx >> 7) << 7, WIN), WIN)
    lane = idx & (WIN - 1)
    for i in range(3):
        moe_copy(i).wait()
    hn_t = bhn_s[...]
    onehot = (lax.broadcasted_iota(jnp.int32, (16, WIN), 1) == lane).astype(f32).astype(bf16)
    xs = lax.dot_general(onehot, hn_t, NT, preferred_element_type=f32).astype(bf16)
    FC = 4 * WIN
    RB = 64
    for c in range(F // FC):
        cs = slice(c * FC, (c + 1) * FC)
        gt = jnp.dot(xs, wg_v[:, cs], preferred_element_type=f32)[0:8].astype(bf16).astype(f32)
        up = jnp.dot(xs, wu_v[:, cs], preferred_element_type=f32)[0:8].astype(bf16).astype(f32)
        act = (gt * (1.0 / (1.0 + jnp.exp(-gt)))).astype(bf16).astype(f32) * up
        act = act.astype(bf16).astype(f32)
        for rb in range(D // RB):
            p = acc_s[rb * RB:(rb + 1) * RB, :]
            for t in range(0, FC // WIN, 2):
                w2 = wd_v[rb * RB:(rb + 1) * RB, c * FC + t * WIN:c * FC + (t + 2) * WIN].astype(f32)
                w2 = w2 * act[0:1, t * WIN:(t + 2) * WIN]
                p = p + w2[:, 0:WIN] + w2[:, WIN:2 * WIN]
            acc_s[rb * RB:(rb + 1) * RB, :] = p
    y = jnp.sum(acc_s[...], axis=1, keepdims=True)
    rsel = jnp.full((1, 1), best_s[0], f32)
    y = y.astype(bf16).astype(f32) * (1.0 / (1.0 + jnp.exp(-rsel)))
    lanes = lax.broadcasted_iota(jnp.int32, (D, WIN), 1)
    yt = jnp.where(lanes == lane, y.astype(bf16).astype(f32), 0.0)
    t = (hn_t.astype(f32) + yt).astype(bf16).astype(f32)
    out_copy(NSEG - 1).wait()
    fix_s[...] = (bh_s[...].astype(f32) + t).astype(bf16)
    fix = pltpu.make_async_copy(fix_s, out_hbm.at[:, tile], sem_o.at[0])
    fix.start()
    fix.wait()


@jax.jit
def pallas_sequential_preLN__memory_aug_infini_attn__moe_arch_mod__prompt_kernel(
    A_x: jax.Array,
    A_wq: jax.Array,
    A_wk: jax.Array,
    A_wv: jax.Array,
    A_wo: jax.Array,
    A_beta: jax.Array,
    B_x: jax.Array,
    B_w_r: jax.Array,
    B_w_gate: jax.Array,
    B_w_up: jax.Array,
    B_w_down: jax.Array,
):
    del B_x
    hbm = pl.BlockSpec(memory_space=pltpu.HBM)
    out_t = pl.pallas_call(
        _kernel,
        out_shape=jax.ShapeDtypeStruct((D, S), bf16),
        in_specs=[hbm] * 10,
        out_specs=hbm,
        scratch_shapes=[
            pltpu.VMEM((D, L), bf16),
            pltpu.VMEM((D, L), bf16),
            pltpu.VMEM((4, D, D), bf16),
            pltpu.VMEM((3 * D, D), bf16),
            pltpu.VMEM((D, D), bf16),
            pltpu.VMEM((D, F), bf16),
            pltpu.VMEM((D, F), bf16),
            pltpu.VMEM((D, F), bf16),
            pltpu.VMEM((4, D, WIN), bf16),
            pltpu.VMEM((D // 2, L), u32),
            pltpu.VMEM((D, L), bf16),
            pltpu.VMEM((D, L), bf16),
            pltpu.VMEM((D, L), bf16),
            pltpu.VMEM((NG, L, WIN), bf16),
            pltpu.VMEM((D, L), bf16),
            pltpu.VMEM((D, L), bf16),
            pltpu.VMEM((1280, G * WIN), f32),
            pltpu.VMEM((1280, G * WIN), f32),
            pltpu.VMEM((4, 8, G * WIN), f32),
            pltpu.VMEM((4, 8, G * WIN), f32),
            pltpu.VMEM((NG, VW, L), f32),
            pltpu.VMEM((NG, VW, WIN), f32),
            pltpu.VMEM((2, VW, WIN), f32),
            pltpu.VMEM((D, L), f32),
            pltpu.VMEM((D // 2, L), u32),
            pltpu.VMEM((D, L), bf16),
            pltpu.VMEM((D, WIN), f32),
            pltpu.VMEM((D, WIN), f32),
            pltpu.VMEM((D, L), bf16),
            pltpu.VMEM((D, L), bf16),
            pltpu.VMEM((D, L), bf16),
            pltpu.VMEM((D, WIN), bf16),
            pltpu.VMEM((D, WIN), bf16),
            pltpu.VMEM((D, WIN), bf16),
            pltpu.VMEM((D, WIN), f32),
            pltpu.VMEM((1, H), bf16),
            pltpu.VMEM((D,), bf16),
            pltpu.SMEM((2,), f32),
            pltpu.SMEM((1,), jnp.int32),
            pltpu.SemaphoreType.DMA((2,)),
            pltpu.SemaphoreType.DMA((5,)),
            pltpu.SemaphoreType.DMA((3,)),
            pltpu.SemaphoreType.DMA((1,)),
            pltpu.SemaphoreType.DMA((2,)),
            pltpu.SemaphoreType.REGULAR,
        ],
        compiler_params=pltpu.CompilerParams(vmem_limit_bytes=100 * 1024 * 1024),
    )(A_x.reshape(S, D).T, A_wq, A_wk, A_wv, A_wo, A_beta.reshape(1, H), B_w_r,
      B_w_gate, B_w_up, B_w_down.T)
    return out_t.T.reshape(1, S, D)
```

```python
import os
import jax
import jax.numpy as jnp
from jax import lax
import jax.experimental.pallas as pl
import jax.experimental.pallas.tpu as pltpu

S = 2048
D = 576
H = 32
DH = 18
NSEG = 4
L = 512
F = 4608
G = 4
NG = H // G
GD = G * DH
WIN = 128
VW = 80
MC = 96
LOG2E = 1.4426950408889634
SCALE = 0.2353515625
QSCALE = SCALE * LOG2E
MASKV = -1e9 * LOG2E
EPS = 1e-5
SOFF = (0, 128, 384, 768)
CHUNKS = [(j, i) for j in (3, 2, 1, 0) for i in range(j + 1)]
f32 = jnp.float32
bf16 = jnp.bfloat16
u32 = jnp.uint32
NT = (((1,), (1,)), ((), ()))
ONES2 = 0x3F803F80


def _fdiv18(i):
    return jnp.floor((i.astype(f32) + 0.5) * (1.0 / DH)).astype(jnp.int32)


def _phi(t):
    return jnp.where(t > 0, t + 1.0, jnp.exp(t))


def _fold8(x):
    parts = [x[i:i + 8] for i in range(0, x.shape[0], 8)]
    while len(parts) > 1:
        parts = [parts[i] + parts[i + 1] if i + 1 < len(parts) else parts[i] for i in range(0, len(parts), 2)]
    return parts[0]


def _colsum(load, rb):
    acc = _fold8(load(0, rb))
    for r0 in range(rb, D, rb):
        acc = acc + _fold8(load(r0, rb))
    return jnp.sum(acc, axis=0, keepdims=True)


def _ln_stats(load):
    m = _colsum(load, 64) * (1.0 / D)

    def sq(r0, n):
        xc = load(r0, n) - m
        return xc * xc

    v = _colsum(sq, 96) * (1.0 / D)
    return m, lax.rsqrt(v + EPS)


def _recip(x):
    r = pl.reciprocal(x, approx=True)
    return r * (2.0 - x * r)


def _woff(par):
    return 16 * ((GD * par) // 16)


def _free0(par):
    return GD if par == 0 else 0


def _as_bf16(x):
    return pltpu.bitcast(x, bf16)


def _as_u32(x):
    return pltpu.bitcast(x, u32)


def _pad_rows(a, n):
    return jnp.concatenate([a, jnp.zeros((n - a.shape[0], a.shape[1]), a.dtype)], axis=0)


def _kernel(x_hbm, wq_hbm, wk_hbm, wv_hbm, wo_hbm, beta_hbm, wr_hbm, wg_hbm, wu_hbm, wd_hbm,
            out_hbm,
            xl_s, xr_s, wraw, wT, woT, wg_v, wu_v, wd_v,
            xn_s, xnp_s, qt_s, pqt_s, kt_s, k_s, pkt_s, vt_s, stA, stB, mxA, mxB, nd_s, mext_s, mmask_s,
            oT_s, otp_s, at_s, g_s, wr_s, h_s, hn_s, out_s, out2_s, bh_s, bhn_s, fix_s, acc_s, beta_ref, wr_ref, best_s, zero_s,
            sem_x, sem_w, sem_moe, sem_o, sem_s, sem_f):
    def cols(s):
        return pl.ds(pl.multiple_of(s * L, L), L)

    def window(pr, par):
        return pl.ds(pl.multiple_of(pr * (2 * GD) + _woff(par), 16), VW)

    def xl_copy(s):
        return pltpu.make_async_copy(x_hbm.at[:, cols(s)], xl_s, sem_x.at[0])

    def xr_copy(s):
        return pltpu.make_async_copy(x_hbm.at[:, cols(s)], xr_s, sem_x.at[1])

    def w_copy(i):
        src = (wq_hbm, wk_hbm, wv_hbm, wo_hbm)[i]
        return pltpu.make_async_copy(src, wraw.at[i], sem_w.at[i])

    WQA = 3 * WIN

    def wq_copy(part):
        cs = pl.ds(0, WQA) if part == 0 else pl.ds(WQA, D - WQA)
        return pltpu.make_async_copy(wq_hbm.at[:, cs], wraw.at[0, :, cs], sem_w.at[0 if part else 4])

    def moe_copy(i):
        src, dst = ((wg_hbm, wg_v), (wu_hbm, wu_v), (wd_hbm, wd_v))[i]
        return pltpu.make_async_copy(src, dst, sem_moe.at[i])

    def out_copy(s):
        return pltpu.make_async_copy(out_s, out_hbm.at[:, cols(s)], sem_o.at[0])

    def small_copy(i):
        src, dst = ((beta_hbm, beta_ref), (wr_hbm, wr_ref))[i]
        return pltpu.make_async_copy(src, dst, sem_s.at[i])

    def fence():
        pl.semaphore_signal(sem_f, 1)
        pl.semaphore_wait(sem_f, 1)

    xl_copy(0).start()
    fence()
    wq_copy(0).start()
    fence()
    wq_copy(1).start()
    fence()
    w_copy(1).start()
    fence()
    w_copy(2).start()

    mext_s[...] = jnp.zeros_like(mext_s)
    k_s[...] = jnp.zeros_like(k_s)
    nd_s[...] = jnp.zeros_like(nd_s)
    acc_s[...] = jnp.zeros_like(acc_s)
    bh_s[...] = jnp.zeros_like(bh_s)
    bhn_s[...] = jnp.zeros_like(bhn_s)
    for par in range(2):
        r = lax.broadcasted_iota(jnp.int32, (VW, WIN), 0)
        l = lax.broadcasted_iota(jnp.int32, (VW, WIN), 1)
        free0 = _free0(par)
        hl = _fdiv18(l - 8 * par + DH) - 1
        he = jnp.where((r >= free0) & (r < free0 + 8), r - free0, _fdiv18(r - 8 * par + DH) - 1)
        ok = (he == hl) & (l >= 8 * par) & (l < 8 * par + GD)
        mmask_s[par] = jnp.where(ok, 1.0, 0.0).astype(f32)
    best_s[0] = jnp.float32(-jnp.inf)
    zero_s[0] = jnp.int32(0)
    best_s[1] = jnp.float32(0.0)

    def small_setup():
        beta = beta_ref[...].astype(f32)
        gsig = 1.0 / (1.0 + jnp.exp(-beta))
        fi = lax.broadcasted_iota(jnp.int32, (D, H), 0)
        hi = lax.broadcasted_iota(jnp.int32, (D, H), 1)
        gcol = jnp.sum(jnp.where(_fdiv18(fi) == hi, gsig, 0.0), axis=1, keepdims=True)
        g_s[...] = jnp.broadcast_to(gcol, (D, WIN))
        wr_s[...] = jnp.broadcast_to(wr_ref[...].astype(f32).reshape(1, D), (WIN, D)).T

    kq_r = lax.broadcasted_iota(jnp.int32, (WIN, G * WIN), 0)
    kq_c = lax.broadcasted_iota(jnp.int32, (WIN, G * WIN), 1) & (WIN - 1)
    r40 = lax.broadcasted_iota(jnp.int32, (VW // 2, WIN), 0)

    def ln1_tile(t, tie=None):
        cs = pl.ds(pl.multiple_of(t * WIN, WIN), WIN) if not isinstance(t, int) else slice(t * WIN, (t + 1) * WIN)
        first = (lambda r0, n: xl_s[r0:r0 + n, cs].astype(f32)) if tie is None else (
            lambda r0, n: xl_s[r0:r0 + n, cs].astype(f32) + tie)
        m = _colsum(first, 64) * (1.0 / D)

        def sq(r0, n):
            xc = xl_s[r0:r0 + n, cs].astype(f32) - m
            return xc * xc

        rstd = lax.rsqrt(_colsum(sq, 96) * (1.0 / D) + EPS)
        for r0 in range(0, D, 48):
            xn_s[t if isinstance(t, int) else 0, r0:r0 + 48, :] = ((xl_s[r0:r0 + 48, cs].astype(f32) - m) * rstd).astype(bf16)
        xnp_s[:, cs] = _as_u32(xn_s[t if isinstance(t, int) else 0])

    def proj(base, c):
        return jnp.dot(wT[pl.ds(base + c * MC, MC), :], _as_bf16(xnp_s[...]), preferred_element_type=f32)

    def proj_q(c0=0, c1=D // MC):
        for c in range(c0, c1):
            q = proj(0, c)
            qt_s[pl.ds(c * MC, MC), :] = (q * QSCALE).astype(bf16)
            pqt_s[pl.ds(c * MC, MC), :] = _phi(q).astype(bf16)

    def proj_k(c0=0, c1=D // MC):
        for c in range(c0, c1):
            k = proj(D, c)
            kt_s[pl.ds(c * MC, MC), :] = k.astype(bf16)
            pkt_s[pl.ds(c * MC, MC), :] = _phi(k).astype(bf16)

    def transpose_k():
        for g in range(NG):
            k_s[g, :, 0:VW] = kt_s[window(g // 2, g % 2), :].T

    def proj_v():
        for c in range(D // MC):
            vt_s[pl.ds(c * MC, MC), :] = proj(2 * D, c).astype(bf16)

    def mem_read():
        r80 = lax.broadcasted_iota(jnp.int32, (VW, L), 0)
        for g in range(NG):
            par = g % 2
            rows = window(g // 2, par)
            nd = jnp.dot(mext_s[g].astype(bf16), _pad_rows(pqt_s[rows, :], WIN), preferred_element_type=f32)
            rden = 1.0 / (nd[_free0(par):_free0(par) + 8] + 1e-6)
            scale = jnp.broadcast_to(rden[0:1], (VW, L))
            for a in range(1, G):
                scale = jnp.where(r80 >= 8 * par + a * DH, rden[a:a + 1], scale)
            nd_s[g] = nd * scale * jnp.concatenate([g_s[rows, :]] * (L // WIN), axis=1)

    def mem_update(g):
        free0 = _free0(g % 2) // 2
        rows = window(g // 2, g % 2)
        r = lax.broadcasted_iota(jnp.int32, (VW // 2, L), 0)
        lhs = _as_u32(vt_s[rows, :])
        lhs = _as_bf16(jnp.where((r >= free0) & (r < free0 + 4), u32(ONES2), lhs))
        upd = lax.dot_general(lhs, _pad_rows(pkt_s[rows, :], WIN), NT, preferred_element_type=f32)
        mext_s[g] += jnp.where(mmask_s[g % 2] > 0.5, upd, 0.0)

    def b_chunk(pr, par, st, mx, state, j, i):
        if i == 0:
            q = _as_u32(qt_s[window(pr, par), j * WIN:(j + 1) * WIN])
            lo = 4 * par
            state["rhs"] = jnp.concatenate(
                [_as_bf16(_pad_rows(jnp.where((r40 >= lo + 9 * a) & (r40 < lo + 9 * a + 9), q, u32(0)), WIN // 2))
                 for a in range(G)], axis=1)
        s = jnp.dot(k_s[2 * pr + par, i * WIN:(i + 1) * WIN, :], state["rhs"], preferred_element_type=f32)
        if i == j:
            s = s + jnp.where(kq_r > kq_c, MASKV, 0.0)
        m = jnp.max(s, axis=0, keepdims=True)
        state["m"] = m if i == 0 else jnp.maximum(state["m"], m)
        st[SOFF[j] + i * WIN:SOFF[j] + (i + 1) * WIN, :] = s
        if i == j:
            mx[j] = jnp.broadcast_to(state["m"], (8, G * WIN))

    def c_chunk(pr, par, st, mx, state, j, i):
        g = 2 * pr + par
        for a in range(G):
            row = par * GD + a * DH
            start = (row // 16) * 16
            off = row - start
            rows = pl.ds(pl.multiple_of(pr * (2 * GD) + start, 16), 32)
            one_row = ((off + DH) % 32) // 2
            r16 = lax.broadcasted_iota(jnp.int32, (16, WIN), 0)
            vt = _as_u32(vt_s[rows, i * WIN:(i + 1) * WIN])
            vt = _as_bf16(jnp.where(r16 == one_row, u32(ONES2), vt))
            hs = slice(a * WIN, (a + 1) * WIN)
            p = jnp.exp2(st[SOFF[j] + i * WIN:SOFF[j] + (i + 1) * WIN, hs] - mx[j, 0:1, hs]).astype(bf16)
            d = jnp.dot(vt, p, preferred_element_type=f32)
            acc = d if i == 0 else state[a] + d
            state[a] = acc
            if i == j:
                qs = slice(j * WIN, (j + 1) * WIN)
                lsum = acc[2 * one_row:2 * one_row + 1, :]
                ls = start - _woff(par)
                o = nd_s[g, ls:ls + 32, qs] + ((1.0 - g_s[rows, :]) * _recip(lsum)) * acc
                r32 = lax.broadcasted_iota(jnp.int32, (32, WIN), 0)
                keep = (r32 >= off) & (r32 < off + DH)
                pltpu.store(oT_s.at[rows, qs], o, mask=keep)

    bufs = ((stA, mxA), (stB, mxB))

    def b_all0():
        sb = {}
        for (j, i) in CHUNKS:
            b_chunk(0, 0, *bufs[0], sb, j, i)

    def step(pr, par):
        npr, npar = (pr, 1) if par == 0 else (pr + 1, 0)
        sb, sc = {}, {}
        for (j, i) in CHUNKS:
            b_chunk(npr, npar, *bufs[1 - par], sb, j, i)
            c_chunk(pr, par, *bufs[par], sc, j, i)

    def attention(update_memory):
        z = zero_s[0]
        for g in range(NG - 1):
            step(z + g // 2, g % 2)
        sc = {}
        for n, (j, i) in enumerate(CHUNKS):
            if n < NG and update_memory:
                mem_update(n)
            c_chunk(z + NG // 2 - 1, 1, *bufs[1], sc, j, i)

    def pack_ot():
        at_s[...] = oT_s[...].astype(bf16)
        otp_s[...] = _as_u32(at_s[...])

    def out_proj(nsplit=1, with_ln1=False):
        pack_ot()
        w = L // nsplit
        for p in range(nsplit):
            cs = slice(p * w, (p + 1) * w)
            for c in range(D // MC):
                a = jnp.dot(woT[pl.ds(c * MC, MC), :], _as_bf16(otp_s[:, cs]), preferred_element_type=f32)
                at_s[pl.ds(c * MC, MC), cs] = a.astype(bf16)
                if with_ln1 and c < L // WIN:
                    bits = pltpu.bitcast(a[0:8, c * WIN:(c + 1) * WIN], u32)
                    zero = pltpu.bitcast(lax.shift_right_logical(lax.shift_right_logical(bits, u32(16)), u32(16)), f32)
                    ln1_tile(c, zero[0:1, :])

    LW = 2 * WIN

    def ln2_strip(t, x_s, o_s):
        cs = slice(t * LW, (t + 1) * LW)
        for r0 in range(0, D, 32):
            h_s[r0:r0 + 32, cs] = (x_s[r0:r0 + 32, cs].astype(f32) + at_s[r0:r0 + 32, cs].astype(f32)).astype(bf16)
        m, rstd = _ln_stats(lambda r0, n: h_s[r0:r0 + n, cs].astype(f32))
        racc = None
        for r0 in range(0, D, 48):
            hf = h_s[r0:r0 + 48, cs].astype(f32)
            hn = ((hf - m) * rstd).astype(bf16)
            hn_s[r0:r0 + 48, cs] = hn
            hnf = hn.astype(f32)
            o_s[r0:r0 + 48, cs] = (hf + hnf).astype(bf16)
            wr = wr_s[r0:r0 + 48, :]
            p = _fold8(hnf * jnp.concatenate([wr] * (LW // WIN), axis=1))
            racc = p if racc is None else racc + p
        return jnp.sum(racc, axis=0, keepdims=True)

    def ln2(s, x_s, o_s, copy):
        rs = [ln2_strip(t, x_s, o_s) for t in range(L // LW)]
        copy.start()
        r = jnp.concatenate(rs, axis=1).astype(bf16).astype(f32)
        rmax = jnp.max(r)
        ridx = lax.broadcasted_iota(jnp.int32, (1, L), 1)
        amax = jnp.min(jnp.where(r == rmax, ridx, L))

        @pl.when(rmax > best_s[0])
        def _():
            best_s[0] = rmax
            best_s[1] = (amax + s * L).astype(f32)
            ts = pl.ds(pl.multiple_of((amax >> 7) << 7, WIN), WIN)
            bh_s[...] = h_s[:, ts]
            bhn_s[...] = hn_s[:, ts]

    xl_copy(0).wait()
    small_copy(0).start()
    small_copy(1).start()
    for t in range(L // WIN):
        ln1_tile(t)
    wq_copy(0).wait()
    w_copy(3).start()
    fence()
    xl_copy(1).start()
    fence()
    xr_copy(0).start()
    wT[pl.ds(0, WQA), :] = wraw[0, :, 0:WQA].T
    proj_q(0, 4)
    wq_copy(1).wait()
    w_copy(1).wait()
    wT[pl.ds(WQA, D - WQA), :] = wraw[0, :, WQA:D].T
    wT[pl.ds(D, D), :] = wraw[1].T
    proj_q(4, D // MC)
    proj_k(0, 4)
    w_copy(2).wait()
    w_copy(3).wait()
    small_copy(0).wait()
    small_copy(1).wait()
    wT[pl.ds(2 * D, D), :] = wraw[2].T
    woT[...] = wraw[3].T
    small_setup()
    proj_k(4, D // MC)
    transpose_k()
    proj_v()
    b_all0()

    def segment(s, carry):
        attention(True)

        @pl.when(s > 0)
        def _():
            out_copy(s - 1).wait()

        xr_copy(s).wait()
        xl_copy(s + 1).wait()
        fence()
        for i in range(3):
            @pl.when(s == i)
            def _():
                moe_copy(i).start()

        out_proj(1, True)
        proj_v()
        proj_k()
        transpose_k()
        proj_q()
        mem_read()
        b_all0()
        ln2(s, xr_s, out_s, out_copy(s))

        @pl.when(s + 2 < NSEG)
        def _():
            xr_copy(s + 1).start()
            xl_copy(s + 2).start()

        return carry

    lax.fori_loop(0, NSEG - 1, segment, 0)

    last_copy = pltpu.make_async_copy(out2_s, out_hbm.at[:, cols(NSEG - 1)], sem_o.at[1])
    attention(False)
    out_proj(2)
    ln2(NSEG - 1, xl_s, out2_s, last_copy)

    idx = best_s[1].astype(jnp.int32)
    tile = pl.ds(pl.multiple_of((idx >> 7) << 7, WIN), WIN)
    lane = idx & (WIN - 1)
    for i in range(3):
        moe_copy(i).wait()
    hn_t = bhn_s[...]
    onehot = (lax.broadcasted_iota(jnp.int32, (16, WIN), 1) == lane).astype(f32).astype(bf16)
    xs = lax.dot_general(onehot, hn_t, NT, preferred_element_type=f32).astype(bf16)
    FC = 4 * WIN
    RB = 64
    for c in range(F // FC):
        cs = slice(c * FC, (c + 1) * FC)
        gt = jnp.dot(xs, wg_v[:, cs], preferred_element_type=f32)[0:8].astype(bf16).astype(f32)
        up = jnp.dot(xs, wu_v[:, cs], preferred_element_type=f32)[0:8].astype(bf16).astype(f32)
        act = (gt * (1.0 / (1.0 + jnp.exp(-gt)))).astype(bf16).astype(f32) * up
        act = act.astype(bf16).astype(f32)
        for rb in range(D // RB):
            p = acc_s[rb * RB:(rb + 1) * RB, :]
            for t in range(0, FC // WIN, 2):
                w2 = wd_v[rb * RB:(rb + 1) * RB, c * FC + t * WIN:c * FC + (t + 2) * WIN].astype(f32)
                w2 = w2 * act[0:1, t * WIN:(t + 2) * WIN]
                p = p + w2[:, 0:WIN] + w2[:, WIN:2 * WIN]
            acc_s[rb * RB:(rb + 1) * RB, :] = p
    y = jnp.sum(acc_s[...], axis=1, keepdims=True)
    rsel = jnp.full((1, 1), best_s[0], f32)
    y = y.astype(bf16).astype(f32) * (1.0 / (1.0 + jnp.exp(-rsel)))
    lanes = lax.broadcasted_iota(jnp.int32, (D, WIN), 1)
    yt = jnp.where(lanes == lane, y.astype(bf16).astype(f32), 0.0)
    t = (hn_t.astype(f32) + yt).astype(bf16).astype(f32)
    out_copy(NSEG - 2).wait()
    last_copy.wait()
    fix_s[...] = (bh_s[...].astype(f32) + t).astype(bf16)
    fix = pltpu.make_async_copy(fix_s, out_hbm.at[:, tile], sem_o.at[0])
    fix.start()
    fix.wait()


@jax.jit
def pallas_sequential_preLN__memory_aug_infini_attn__moe_arch_mod__prompt_kernel(
    A_x: jax.Array,
    A_wq: jax.Array,
    A_wk: jax.Array,
    A_wv: jax.Array,
    A_wo: jax.Array,
    A_beta: jax.Array,
    B_x: jax.Array,
    B_w_r: jax.Array,
    B_w_gate: jax.Array,
    B_w_up: jax.Array,
    B_w_down: jax.Array,
):
    del B_x
    hbm = pl.BlockSpec(memory_space=pltpu.HBM)
    out_t = pl.pallas_call(
        _kernel,
        out_shape=jax.ShapeDtypeStruct((D, S), bf16),
        in_specs=[hbm] * 10,
        out_specs=hbm,
        scratch_shapes=[
            pltpu.VMEM((D, L), bf16),
            pltpu.VMEM((D, L), bf16),
            pltpu.VMEM((4, D, D), bf16),
            pltpu.VMEM((3 * D, D), bf16),
            pltpu.VMEM((D, D), bf16),
            pltpu.VMEM((D, F), bf16),
            pltpu.VMEM((D, F), bf16),
            pltpu.VMEM((D, F), bf16),
            pltpu.VMEM((4, D, WIN), bf16),
            pltpu.VMEM((D // 2, L), u32),
            pltpu.VMEM((D, L), bf16),
            pltpu.VMEM((D, L), bf16),
            pltpu.VMEM((D, L), bf16),
            pltpu.VMEM((NG, L, WIN), bf16),
            pltpu.VMEM((D, L), bf16),
            pltpu.VMEM((D, L), bf16),
            pltpu.VMEM((1280, G * WIN), f32),
            pltpu.VMEM((1280, G * WIN), f32),
            pltpu.VMEM((4, 8, G * WIN), f32),
            pltpu.VMEM((4, 8, G * WIN), f32),
            pltpu.VMEM((NG, VW, L), f32),
            pltpu.VMEM((NG, VW, WIN), f32),
            pltpu.VMEM((2, VW, WIN), f32),
            pltpu.VMEM((D, L), f32),
            pltpu.VMEM((D // 2, L), u32),
            pltpu.VMEM((D, L), bf16),
            pltpu.VMEM((D, WIN), f32),
            pltpu.VMEM((D, WIN), f32),
            pltpu.VMEM((D, L), bf16),
            pltpu.VMEM((D, L), bf16),
            pltpu.VMEM((D, L), bf16),
            pltpu.VMEM((D, L), bf16),
            pltpu.VMEM((D, WIN), bf16),
            pltpu.VMEM((D, WIN), bf16),
            pltpu.VMEM((D, WIN), bf16),
            pltpu.VMEM((D, WIN), f32),
            pltpu.VMEM((1, H), bf16),
            pltpu.VMEM((D,), bf16),
            pltpu.SMEM((2,), f32),
            pltpu.SMEM((1,), jnp.int32),
            pltpu.SemaphoreType.DMA((2,)),
            pltpu.SemaphoreType.DMA((5,)),
            pltpu.SemaphoreType.DMA((3,)),
            pltpu.SemaphoreType.DMA((2,)),
            pltpu.SemaphoreType.DMA((2,)),
            pltpu.SemaphoreType.REGULAR,
        ],
        compiler_params=pltpu.CompilerParams(vmem_limit_bytes=100 * 1024 * 1024),
    )(A_x.reshape(S, D).T, A_wq, A_wk, A_wv, A_wo, A_beta.reshape(1, H), B_w_r,
      B_w_gate, B_w_up, B_w_down.T)
    return out_t.T.reshape(1, S, D)
```

```python
import os
import jax
import jax.numpy as jnp
from jax import lax
import jax.experimental.pallas as pl
import jax.experimental.pallas.tpu as pltpu

S = 2048
D = 576
H = 32
DH = 18
NSEG = 4
L = 512
F = 4608
G = 4
NG = H // G
GD = G * DH
WIN = 128
VW = 80
RB1 = 64
RB2 = 96
PORDER = 'vqktmbl'
MC = 96
LOG2E = 1.4426950408889634
SCALE = 0.2353515625
QSCALE = SCALE * LOG2E
MASKV = -1e9 * LOG2E
EPS = 1e-5
SOFF = (0, 128, 384, 768)
CHUNKS = [(j, i) for j in (3, 2, 1, 0) for i in range(j + 1)]
f32 = jnp.float32
bf16 = jnp.bfloat16
u32 = jnp.uint32
NT = (((1,), (1,)), ((), ()))
ONES2 = 0x3F803F80


def _fdiv18(i):
    return jnp.floor((i.astype(f32) + 0.5) * (1.0 / DH)).astype(jnp.int32)


def _phi(t):
    return jnp.where(t > 0, t + 1.0, jnp.exp(t))


def _fold8(x):
    parts = [x[i:i + 8] for i in range(0, x.shape[0], 8)]
    while len(parts) > 1:
        parts = [parts[i] + parts[i + 1] if i + 1 < len(parts) else parts[i] for i in range(0, len(parts), 2)]
    return parts[0]


def _colsum(load, rb):
    acc = _fold8(load(0, rb))
    for r0 in range(rb, D, rb):
        acc = acc + _fold8(load(r0, rb))
    return jnp.sum(acc, axis=0, keepdims=True)


def _ln_stats(load):
    m = _colsum(load, RB1) * (1.0 / D)

    def sq(r0, n):
        xc = load(r0, n) - m
        return xc * xc

    v = _colsum(sq, RB2) * (1.0 / D)
    return m, lax.rsqrt(v + EPS)


def _recip(x):
    r = pl.reciprocal(x, approx=True)
    return r * (2.0 - x * r)


def _woff(par):
    return 16 * ((GD * par) // 16)


def _free0(par):
    return GD if par == 0 else 0


def _as_bf16(x):
    return pltpu.bitcast(x, bf16)


def _as_u32(x):
    return pltpu.bitcast(x, u32)


def _pad_rows(a, n):
    return jnp.concatenate([a, jnp.zeros((n - a.shape[0], a.shape[1]), a.dtype)], axis=0)


def _kernel(x_hbm, wq_hbm, wk_hbm, wv_hbm, wo_hbm, beta_hbm, wr_hbm, wg_hbm, wu_hbm, wd_hbm,
            out_hbm,
            xl_s, xr_s, wraw, wT, woT, wg_v, wu_v, wd_v,
            xn_s, xnp_s, qt_s, pqt_s, kt_s, k_s, pkt_s, vt_s, stA, stB, mxA, mxB, nd_s, mext_s, mmask_s,
            oT_s, otp_s, at_s, g_s, wr_s, h_s, hn_s, out_s, out2_s, bh_s, bhn_s, fix_s, acc_s, beta_ref, wr_ref, best_s, zero_s,
            sem_x, sem_w, sem_moe, sem_o, sem_s, sem_f):
    def cols(s):
        return pl.ds(pl.multiple_of(s * L, L), L)

    def window(pr, par):
        return pl.ds(pl.multiple_of(pr * (2 * GD) + _woff(par), 16), VW)

    def xl_copy(s):
        return pltpu.make_async_copy(x_hbm.at[:, cols(s)], xl_s, sem_x.at[0])

    def xr_copy(s):
        return pltpu.make_async_copy(x_hbm.at[:, cols(s)], xr_s, sem_x.at[1])

    def w_copy(i):
        src = (wq_hbm, wk_hbm, wv_hbm, wo_hbm)[i]
        return pltpu.make_async_copy(src, wraw.at[i], sem_w.at[i])

    WQA = 3 * WIN

    def wq_copy(part):
        cs = pl.ds(0, WQA) if part == 0 else pl.ds(WQA, D - WQA)
        return pltpu.make_async_copy(wq_hbm.at[:, cs], wraw.at[0, :, cs], sem_w.at[0 if part else 4])

    def moe_copy(i):
        src, dst = ((wg_hbm, wg_v), (wu_hbm, wu_v), (wd_hbm, wd_v))[i]
        return pltpu.make_async_copy(src, dst, sem_moe.at[i])

    def out_copy(s):
        return pltpu.make_async_copy(out_s, out_hbm.at[:, cols(s)], sem_o.at[0])

    def small_copy(i):
        src, dst = ((beta_hbm, beta_ref), (wr_hbm, wr_ref))[i]
        return pltpu.make_async_copy(src, dst, sem_s.at[i])

    def fence():
        pl.semaphore_signal(sem_f, 1)
        pl.semaphore_wait(sem_f, 1)

    xl_copy(0).start()
    fence()
    wq_copy(0).start()
    fence()
    wq_copy(1).start()
    fence()
    w_copy(1).start()
    fence()
    w_copy(2).start()

    mext_s[...] = jnp.zeros_like(mext_s)
    k_s[...] = jnp.zeros_like(k_s)
    nd_s[...] = jnp.zeros_like(nd_s)
    acc_s[...] = jnp.zeros_like(acc_s)
    bh_s[...] = jnp.zeros_like(bh_s)
    bhn_s[...] = jnp.zeros_like(bhn_s)
    for par in range(2):
        r = lax.broadcasted_iota(jnp.int32, (VW, WIN), 0)
        l = lax.broadcasted_iota(jnp.int32, (VW, WIN), 1)
        free0 = _free0(par)
        hl = _fdiv18(l - 8 * par + DH) - 1
        he = jnp.where((r >= free0) & (r < free0 + 8), r - free0, _fdiv18(r - 8 * par + DH) - 1)
        ok = (he == hl) & (l >= 8 * par) & (l < 8 * par + GD)
        mmask_s[par] = jnp.where(ok, 1.0, 0.0).astype(f32)
    best_s[0] = jnp.float32(-jnp.inf)
    zero_s[0] = jnp.int32(0)
    best_s[1] = jnp.float32(0.0)

    def small_setup():
        beta = beta_ref[...].astype(f32)
        gsig = 1.0 / (1.0 + jnp.exp(-beta))
        fi = lax.broadcasted_iota(jnp.int32, (D, H), 0)
        hi = lax.broadcasted_iota(jnp.int32, (D, H), 1)
        gcol = jnp.sum(jnp.where(_fdiv18(fi) == hi, gsig, 0.0), axis=1, keepdims=True)
        g_s[...] = jnp.broadcast_to(gcol, (D, WIN))
        wr_s[...] = jnp.broadcast_to(wr_ref[...].astype(f32).reshape(1, D), (WIN, D)).T

    kq_r = lax.broadcasted_iota(jnp.int32, (WIN, G * WIN), 0)
    kq_c = lax.broadcasted_iota(jnp.int32, (WIN, G * WIN), 1) & (WIN - 1)
    r40 = lax.broadcasted_iota(jnp.int32, (VW // 2, WIN), 0)

    def ln1_tile(t, tie=None):
        cs = pl.ds(pl.multiple_of(t * WIN, WIN), WIN) if not isinstance(t, int) else slice(t * WIN, (t + 1) * WIN)
        first = (lambda r0, n: xl_s[r0:r0 + n, cs].astype(f32)) if tie is None else (
            lambda r0, n: xl_s[r0:r0 + n, cs].astype(f32) + tie)
        m = _colsum(first, 64) * (1.0 / D)

        def sq(r0, n):
            xc = xl_s[r0:r0 + n, cs].astype(f32) - m
            return xc * xc

        rstd = lax.rsqrt(_colsum(sq, 96) * (1.0 / D) + EPS)
        for r0 in range(0, D, 48):
            xn_s[t if isinstance(t, int) else 0, r0:r0 + 48, :] = ((xl_s[r0:r0 + 48, cs].astype(f32) - m) * rstd).astype(bf16)
        xnp_s[:, cs] = _as_u32(xn_s[t if isinstance(t, int) else 0])

    def proj(base, c):
        return jnp.dot(wT[pl.ds(base + c * MC, MC), :], _as_bf16(xnp_s[...]), preferred_element_type=f32)

    def proj_q(c0=0, c1=D // MC):
        for c in range(c0, c1):
            q = proj(0, c)
            qt_s[pl.ds(c * MC, MC), :] = (q * QSCALE).astype(bf16)
            pqt_s[pl.ds(c * MC, MC), :] = _phi(q).astype(bf16)

    def proj_k(c0=0, c1=D // MC):
        for c in range(c0, c1):
            k = proj(D, c)
            kt_s[pl.ds(c * MC, MC), :] = k.astype(bf16)
            pkt_s[pl.ds(c * MC, MC), :] = _phi(k).astype(bf16)

    def transpose_k():
        for g in range(NG):
            k_s[g, :, 0:VW] = kt_s[window(g // 2, g % 2), :].T

    def proj_v():
        for c in range(D // MC):
            vt_s[pl.ds(c * MC, MC), :] = proj(2 * D, c).astype(bf16)

    def mem_read():
        r80 = lax.broadcasted_iota(jnp.int32, (VW, L), 0)
        for g in range(NG):
            par = g % 2
            rows = window(g // 2, par)
            nd = jnp.dot(mext_s[g].astype(bf16), _pad_rows(pqt_s[rows, :], WIN), preferred_element_type=f32)
            rden = 1.0 / (nd[_free0(par):_free0(par) + 8] + 1e-6)
            scale = jnp.broadcast_to(rden[0:1], (VW, L))
            for a in range(1, G):
                scale = jnp.where(r80 >= 8 * par + a * DH, rden[a:a + 1], scale)
            nd_s[g] = nd * scale * jnp.concatenate([g_s[rows, :]] * (L // WIN), axis=1)

    def mem_update(g):
        free0 = _free0(g % 2) // 2
        rows = window(g // 2, g % 2)
        r = lax.broadcasted_iota(jnp.int32, (VW // 2, L), 0)
        lhs = _as_u32(vt_s[rows, :])
        lhs = _as_bf16(jnp.where((r >= free0) & (r < free0 + 4), u32(ONES2), lhs))
        upd = lax.dot_general(lhs, _pad_rows(pkt_s[rows, :], WIN), NT, preferred_element_type=f32)
        mext_s[g] += jnp.where(mmask_s[g % 2] > 0.5, upd, 0.0)

    def b_chunk(pr, par, st, mx, state, j, i):
        if i == 0:
            q = _as_u32(qt_s[window(pr, par), j * WIN:(j + 1) * WIN])
            lo = 4 * par
            state["rhs"] = jnp.concatenate(
                [_as_bf16(_pad_rows(jnp.where((r40 >= lo + 9 * a) & (r40 < lo + 9 * a + 9), q, u32(0)), WIN // 2))
                 for a in range(G)], axis=1)
        s = jnp.dot(k_s[2 * pr + par, i * WIN:(i + 1) * WIN, :], state["rhs"], preferred_element_type=f32)
        if i == j:
            s = s + jnp.where(kq_r > kq_c, MASKV, 0.0)
        m = jnp.max(s, axis=0, keepdims=True)
        state["m"] = m if i == 0 else jnp.maximum(state["m"], m)
        st[SOFF[j] + i * WIN:SOFF[j] + (i + 1) * WIN, :] = s
        if i == j:
            mx[j] = jnp.broadcast_to(state["m"], (8, G * WIN))

    def c_chunk(pr, par, st, mx, state, j, i):
        g = 2 * pr + par
        for a in range(G):
            row = par * GD + a * DH
            start = (row // 16) * 16
            off = row - start
            rows = pl.ds(pl.multiple_of(pr * (2 * GD) + start, 16), 32)
            one_row = ((off + DH) % 32) // 2
            r16 = lax.broadcasted_iota(jnp.int32, (16, WIN), 0)
            vt = _as_u32(vt_s[rows, i * WIN:(i + 1) * WIN])
            vt = _as_bf16(jnp.where(r16 == one_row, u32(ONES2), vt))
            hs = slice(a * WIN, (a + 1) * WIN)
            p = jnp.exp2(st[SOFF[j] + i * WIN:SOFF[j] + (i + 1) * WIN, hs] - mx[j, 0:1, hs]).astype(bf16)
            d = jnp.dot(vt, p, preferred_element_type=f32)
            acc = d if i == 0 else state[a] + d
            state[a] = acc
            if i == j:
                qs = slice(j * WIN, (j + 1) * WIN)
                lsum = acc[2 * one_row:2 * one_row + 1, :]
                ls = start - _woff(par)
                o = nd_s[g, ls:ls + 32, qs] + ((1.0 - g_s[rows, :]) * _recip(lsum)) * acc
                r32 = lax.broadcasted_iota(jnp.int32, (32, WIN), 0)
                keep = (r32 >= off) & (r32 < off + DH)
                pltpu.store(oT_s.at[rows, qs], o, mask=keep)

    bufs = ((stA, mxA), (stB, mxB))

    def b_all0():
        sb = {}
        for (j, i) in CHUNKS:
            b_chunk(0, 0, *bufs[0], sb, j, i)

    def step(pr, par):
        npr, npar = (pr, 1) if par == 0 else (pr + 1, 0)
        sb, sc = {}, {}
        for (j, i) in CHUNKS:
            b_chunk(npr, npar, *bufs[1 - par], sb, j, i)
            c_chunk(pr, par, *bufs[par], sc, j, i)

    def attention(update_memory):
        z = zero_s[0]
        for g in range(NG - 1):
            step(z + g // 2, g % 2)
        sc = {}
        for n, (j, i) in enumerate(CHUNKS):
            if n < NG and update_memory:
                mem_update(n)
            c_chunk(z + NG // 2 - 1, 1, *bufs[1], sc, j, i)

    def pack_ot():
        at_s[...] = oT_s[...].astype(bf16)
        otp_s[...] = _as_u32(at_s[...])

    def out_proj(nsplit=1, with_ln1=False):
        pack_ot()
        w = L // nsplit
        for p in range(nsplit):
            cs = slice(p * w, (p + 1) * w)
            for c in range(D // MC):
                a = jnp.dot(woT[pl.ds(c * MC, MC), :], _as_bf16(otp_s[:, cs]), preferred_element_type=f32)
                at_s[pl.ds(c * MC, MC), cs] = a.astype(bf16)
                if with_ln1 and c < L // WIN:
                    bits = pltpu.bitcast(a[0:8, c * WIN:(c + 1) * WIN], u32)
                    zero = pltpu.bitcast(lax.shift_right_logical(lax.shift_right_logical(bits, u32(16)), u32(16)), f32)
                    ln1_tile(c, zero[0:1, :])

    LW = 2 * WIN

    def ln2_strip(t, x_s, o_s):
        cs = slice(t * LW, (t + 1) * LW)
        for r0 in range(0, D, 32):
            h_s[r0:r0 + 32, cs] = (x_s[r0:r0 + 32, cs].astype(f32) + at_s[r0:r0 + 32, cs].astype(f32)).astype(bf16)
        m, rstd = _ln_stats(lambda r0, n: h_s[r0:r0 + n, cs].astype(f32))
        racc = None
        for r0 in range(0, D, 48):
            hf = h_s[r0:r0 + 48, cs].astype(f32)
            hn = ((hf - m) * rstd).astype(bf16)
            hn_s[r0:r0 + 48, cs] = hn
            hnf = hn.astype(f32)
            o_s[r0:r0 + 48, cs] = (hf + hnf).astype(bf16)
            wr = wr_s[r0:r0 + 48, :]
            p = _fold8(hnf * jnp.concatenate([wr] * (LW // WIN), axis=1))
            racc = p if racc is None else racc + p
        return jnp.sum(racc, axis=0, keepdims=True)

    def ln2(s, x_s, o_s, copy):
        rs = [ln2_strip(t, x_s, o_s) for t in range(L // LW)]
        copy.start()
        r = jnp.concatenate(rs, axis=1).astype(bf16).astype(f32)
        rmax = jnp.max(r)
        ridx = lax.broadcasted_iota(jnp.int32, (1, L), 1)
        amax = jnp.min(jnp.where(r == rmax, ridx, L))

        @pl.when(rmax > best_s[0])
        def _():
            best_s[0] = rmax
            best_s[1] = (amax + s * L).astype(f32)
            ts = pl.ds(pl.multiple_of((amax >> 7) << 7, WIN), WIN)
            bh_s[...] = _as_u32(h_s[:, ts])
            bhn_s[...] = _as_u32(hn_s[:, ts])

    xl_copy(0).wait()
    small_copy(0).start()
    small_copy(1).start()
    for t in range(L // WIN):
        ln1_tile(t)
    wq_copy(0).wait()
    w_copy(3).start()
    fence()
    xl_copy(1).start()
    fence()
    xr_copy(0).start()
    wT[pl.ds(0, WQA), :] = wraw[0, :, 0:WQA].T
    proj_q(0, 4)
    wq_copy(1).wait()
    w_copy(1).wait()
    wT[pl.ds(WQA, D - WQA), :] = wraw[0, :, WQA:D].T
    wT[pl.ds(D, D), :] = wraw[1].T
    proj_q(4, D // MC)
    proj_k(0, 4)
    w_copy(2).wait()
    w_copy(3).wait()
    small_copy(0).wait()
    small_copy(1).wait()
    wT[pl.ds(2 * D, D), :] = wraw[2].T
    woT[...] = wraw[3].T
    small_setup()
    proj_k(4, D // MC)
    transpose_k()
    proj_v()
    b_all0()

    def segment(s, carry):
        attention(True)

        @pl.when(s > 0)
        def _():
            out_copy(s - 1).wait()

        xr_copy(s).wait()
        xl_copy(s + 1).wait()
        fence()
        for i in range(3):
            @pl.when(s == i)
            def _():
                moe_copy(i).start()

        out_proj(1, True)
        for ch in PORDER:
            if ch == 'l':
                ln2(s, xr_s, out_s, out_copy(s))
            else:
                {'v': proj_v, 'k': proj_k, 't': transpose_k, 'q': proj_q, 'm': mem_read, 'b': b_all0}[ch]()

        @pl.when(s + 2 < NSEG)
        def _():
            xr_copy(s + 1).start()
            xl_copy(s + 2).start()

        return carry

    lax.fori_loop(0, NSEG - 1, segment, 0)

    last_copy = pltpu.make_async_copy(out2_s, out_hbm.at[:, cols(NSEG - 1)], sem_o.at[1])
    attention(False)
    out_proj(2)
    ln2(NSEG - 1, xl_s, out2_s, last_copy)

    idx = best_s[1].astype(jnp.int32)
    tile = pl.ds(pl.multiple_of((idx >> 7) << 7, WIN), WIN)
    lane = idx & (WIN - 1)
    for i in range(3):
        moe_copy(i).wait()
    hn_t = _as_bf16(bhn_s[...])
    onehot = (lax.broadcasted_iota(jnp.int32, (16, WIN), 1) == lane).astype(f32).astype(bf16)
    xs = lax.dot_general(onehot, hn_t, NT, preferred_element_type=f32).astype(bf16)
    FC = 4 * WIN
    RB = 64
    for c in range(F // FC):
        cs = slice(c * FC, (c + 1) * FC)
        gt = jnp.dot(xs, wg_v[:, cs], preferred_element_type=f32)[0:8].astype(bf16).astype(f32)
        up = jnp.dot(xs, wu_v[:, cs], preferred_element_type=f32)[0:8].astype(bf16).astype(f32)
        act = (gt * (1.0 / (1.0 + jnp.exp(-gt)))).astype(bf16).astype(f32) * up
        act = act.astype(bf16).astype(f32)
        for rb in range(D // RB):
            p = acc_s[rb * RB:(rb + 1) * RB, :]
            for t in range(0, FC // WIN, 2):
                w2 = wd_v[rb * RB:(rb + 1) * RB, c * FC + t * WIN:c * FC + (t + 2) * WIN].astype(f32)
                w2 = w2 * act[0:1, t * WIN:(t + 2) * WIN]
                p = p + w2[:, 0:WIN] + w2[:, WIN:2 * WIN]
            acc_s[rb * RB:(rb + 1) * RB, :] = p
    y = jnp.sum(acc_s[...], axis=1, keepdims=True)
    rsel = jnp.full((1, 1), best_s[0], f32)
    y = y.astype(bf16).astype(f32) * (1.0 / (1.0 + jnp.exp(-rsel)))
    lanes = lax.broadcasted_iota(jnp.int32, (D, WIN), 1)
    yt = jnp.where(lanes == lane, y.astype(bf16).astype(f32), 0.0)
    t = (hn_t.astype(f32) + yt).astype(bf16).astype(f32)
    out_copy(NSEG - 2).wait()
    last_copy.wait()
    fix_s[...] = (_as_bf16(bh_s[...]).astype(f32) + t).astype(bf16)
    fix = pltpu.make_async_copy(fix_s, out_hbm.at[:, tile], sem_o.at[0])
    fix.start()
    fix.wait()


@jax.jit
def pallas_sequential_preLN__memory_aug_infini_attn__moe_arch_mod__prompt_kernel(
    A_x: jax.Array,
    A_wq: jax.Array,
    A_wk: jax.Array,
    A_wv: jax.Array,
    A_wo: jax.Array,
    A_beta: jax.Array,
    B_x: jax.Array,
    B_w_r: jax.Array,
    B_w_gate: jax.Array,
    B_w_up: jax.Array,
    B_w_down: jax.Array,
):
    del B_x
    hbm = pl.BlockSpec(memory_space=pltpu.HBM)
    out_t = pl.pallas_call(
        _kernel,
        out_shape=jax.ShapeDtypeStruct((D, S), bf16),
        in_specs=[hbm] * 10,
        out_specs=hbm,
        scratch_shapes=[
            pltpu.VMEM((D, L), bf16),
            pltpu.VMEM((D, L), bf16),
            pltpu.VMEM((4, D, D), bf16),
            pltpu.VMEM((3 * D, D), bf16),
            pltpu.VMEM((D, D), bf16),
            pltpu.VMEM((D, F), bf16),
            pltpu.VMEM((D, F), bf16),
            pltpu.VMEM((D, F), bf16),
            pltpu.VMEM((4, D, WIN), bf16),
            pltpu.VMEM((D // 2, L), u32),
            pltpu.VMEM((D, L), bf16),
            pltpu.VMEM((D, L), bf16),
            pltpu.VMEM((D, L), bf16),
            pltpu.VMEM((NG, L, WIN), bf16),
            pltpu.VMEM((D, L), bf16),
            pltpu.VMEM((D, L), bf16),
            pltpu.VMEM((1280, G * WIN), f32),
            pltpu.VMEM((1280, G * WIN), f32),
            pltpu.VMEM((4, 8, G * WIN), f32),
            pltpu.VMEM((4, 8, G * WIN), f32),
            pltpu.VMEM((NG, VW, L), f32),
            pltpu.VMEM((NG, VW, WIN), f32),
            pltpu.VMEM((2, VW, WIN), f32),
            pltpu.VMEM((D, L), f32),
            pltpu.VMEM((D // 2, L), u32),
            pltpu.VMEM((D, L), bf16),
            pltpu.VMEM((D, WIN), f32),
            pltpu.VMEM((D, WIN), f32),
            pltpu.VMEM((D, L), bf16),
            pltpu.VMEM((D, L), bf16),
            pltpu.VMEM((D, L), bf16),
            pltpu.VMEM((D, L), bf16),
            pltpu.VMEM((D // 2, WIN), u32),
            pltpu.VMEM((D // 2, WIN), u32),
            pltpu.VMEM((D, WIN), bf16),
            pltpu.VMEM((D, WIN), f32),
            pltpu.VMEM((1, H), bf16),
            pltpu.VMEM((D,), bf16),
            pltpu.SMEM((2,), f32),
            pltpu.SMEM((1,), jnp.int32),
            pltpu.SemaphoreType.DMA((2,)),
            pltpu.SemaphoreType.DMA((5,)),
            pltpu.SemaphoreType.DMA((3,)),
            pltpu.SemaphoreType.DMA((2,)),
            pltpu.SemaphoreType.DMA((2,)),
            pltpu.SemaphoreType.REGULAR,
        ],
        compiler_params=pltpu.CompilerParams(vmem_limit_bytes=100 * 1024 * 1024),
    )(A_x.reshape(S, D).T, A_wq, A_wk, A_wv, A_wo, A_beta.reshape(1, H), B_w_r,
      B_w_gate, B_w_up, B_w_down.T)
    return out_t.T.reshape(1, S, D)
```

```python
import os
import jax
import jax.numpy as jnp
from jax import lax
import jax.experimental.pallas as pl
import jax.experimental.pallas.tpu as pltpu

S = 2048
D = 576
H = 32
DH = 18
NSEG = 4
L = 512
F = 4608
G = 4
NG = H // G
GD = G * DH
WIN = 128
VW = 80
KTV = [[0], [], [1], [], [2], [3]]
KTQ = [[], [4], [5], [], [6], [7]]
MC = 96
LOG2E = 1.4426950408889634
SCALE = 0.2353515625
QSCALE = SCALE * LOG2E
MASKV = -1e9 * LOG2E
EPS = 1e-5
SOFF = (0, 128, 384, 768)
CHUNKS = [(j, i) for j in (3, 2, 1, 0) for i in range(j + 1)]
f32 = jnp.float32
bf16 = jnp.bfloat16
u32 = jnp.uint32
NT = (((1,), (1,)), ((), ()))
ONES2 = 0x3F803F80


def _fdiv18(i):
    return jnp.floor((i.astype(f32) + 0.5) * (1.0 / DH)).astype(jnp.int32)


def _phi(t):
    return jnp.where(t > 0, t + 1.0, jnp.exp(t))


def _fold8(x):
    parts = [x[i:i + 8] for i in range(0, x.shape[0], 8)]
    while len(parts) > 1:
        parts = [parts[i] + parts[i + 1] if i + 1 < len(parts) else parts[i] for i in range(0, len(parts), 2)]
    return parts[0]


def _colsum(load, rb):
    acc = _fold8(load(0, rb))
    for r0 in range(rb, D, rb):
        acc = acc + _fold8(load(r0, rb))
    return jnp.sum(acc, axis=0, keepdims=True)


def _ln_stats(load):
    m = _colsum(load, 64) * (1.0 / D)

    def sq(r0, n):
        xc = load(r0, n) - m
        return xc * xc

    v = _colsum(sq, 96) * (1.0 / D)
    return m, lax.rsqrt(v + EPS)


def _recip(x):
    r = pl.reciprocal(x, approx=True)
    return r * (2.0 - x * r)


def _zero_bits_after(a):
    bits = pltpu.bitcast(a[0:8, 0:WIN], u32)
    return lax.shift_right_logical(lax.shift_right_logical(bits, u32(16)), u32(16))[0:1]


def _woff(par):
    return 16 * ((GD * par) // 16)


def _free0(par):
    return GD if par == 0 else 0


def _as_bf16(x):
    return pltpu.bitcast(x, bf16)


def _as_u32(x):
    return pltpu.bitcast(x, u32)


def _pad_rows(a, n):
    return jnp.concatenate([a, jnp.zeros((n - a.shape[0], a.shape[1]), a.dtype)], axis=0)


def _kernel(x_hbm, wq_hbm, wk_hbm, wv_hbm, wo_hbm, beta_hbm, wr_hbm, wg_hbm, wu_hbm, wd_hbm,
            out_hbm,
            xl_s, xr_s, wraw, wT, woT, wg_v, wu_v, wd_v,
            xn_s, xnp_s, qt_s, pqt_s, kt_s, k_s, pkt_s, vt_s, stA, stB, mxA, mxB, nd_s, mext_s, mmask_s,
            oT_s, otp_s, at_s, g_s, wr_s, h_s, hn_s, out_s, out2_s, bh_s, bhn_s, fix_s, acc_s, beta_ref, wr_ref, best_s, zero_s,
            sem_x, sem_w, sem_moe, sem_o, sem_s, sem_f):
    def cols(s):
        return pl.ds(pl.multiple_of(s * L, L), L)

    def window(pr, par):
        return pl.ds(pl.multiple_of(pr * (2 * GD) + _woff(par), 16), VW)

    def xl_copy(s):
        return pltpu.make_async_copy(x_hbm.at[:, cols(s)], xl_s, sem_x.at[0])

    def xr_copy(s):
        return pltpu.make_async_copy(x_hbm.at[:, cols(s)], xr_s, sem_x.at[1])

    def w_copy(i):
        src = (wq_hbm, wk_hbm, wv_hbm, wo_hbm)[i]
        return pltpu.make_async_copy(src, wraw.at[i], sem_w.at[i])

    WQA = 3 * WIN

    def wq_copy(part):
        cs = pl.ds(0, WQA) if part == 0 else pl.ds(WQA, D - WQA)
        return pltpu.make_async_copy(wq_hbm.at[:, cs], wraw.at[0, :, cs], sem_w.at[0 if part else 4])

    def moe_copy(i):
        src, dst = ((wg_hbm, wg_v), (wu_hbm, wu_v), (wd_hbm, wd_v))[i]
        return pltpu.make_async_copy(src, dst, sem_moe.at[i])

    def out_copy(s):
        return pltpu.make_async_copy(out_s, out_hbm.at[:, cols(s)], sem_o.at[0])

    def small_copy(i):
        src, dst = ((beta_hbm, beta_ref), (wr_hbm, wr_ref))[i]
        return pltpu.make_async_copy(src, dst, sem_s.at[i])

    def fence():
        pl.semaphore_signal(sem_f, 1)
        pl.semaphore_wait(sem_f, 1)

    xl_copy(0).start()
    fence()
    wq_copy(0).start()
    fence()
    wq_copy(1).start()
    fence()
    w_copy(1).start()
    fence()
    w_copy(2).start()

    mext_s[...] = jnp.zeros_like(mext_s)
    k_s[...] = jnp.zeros_like(k_s)
    nd_s[...] = jnp.zeros_like(nd_s)
    acc_s[...] = jnp.zeros_like(acc_s)
    bh_s[...] = jnp.zeros_like(bh_s)
    bhn_s[...] = jnp.zeros_like(bhn_s)
    for par in range(2):
        r = lax.broadcasted_iota(jnp.int32, (VW, WIN), 0)
        l = lax.broadcasted_iota(jnp.int32, (VW, WIN), 1)
        free0 = _free0(par)
        hl = _fdiv18(l - 8 * par + DH) - 1
        he = jnp.where((r >= free0) & (r < free0 + 8), r - free0, _fdiv18(r - 8 * par + DH) - 1)
        ok = (he == hl) & (l >= 8 * par) & (l < 8 * par + GD)
        mmask_s[par] = jnp.where(ok, 1.0, 0.0).astype(f32)
    best_s[0] = jnp.float32(-jnp.inf)
    zero_s[0] = jnp.int32(0)
    best_s[1] = jnp.float32(0.0)

    def small_setup():
        beta = beta_ref[...].astype(f32)
        gsig = 1.0 / (1.0 + jnp.exp(-beta))
        fi = lax.broadcasted_iota(jnp.int32, (D, H), 0)
        hi = lax.broadcasted_iota(jnp.int32, (D, H), 1)
        gcol = jnp.sum(jnp.where(_fdiv18(fi) == hi, gsig, 0.0), axis=1, keepdims=True)
        g_s[...] = jnp.broadcast_to(gcol, (D, WIN))
        wr_s[...] = jnp.broadcast_to(wr_ref[...].astype(f32).reshape(1, D), (WIN, D)).T

    kq_r = lax.broadcasted_iota(jnp.int32, (WIN, G * WIN), 0)
    kq_c = lax.broadcasted_iota(jnp.int32, (WIN, G * WIN), 1) & (WIN - 1)
    r40 = lax.broadcasted_iota(jnp.int32, (VW // 2, WIN), 0)

    def ln1_tile(t, tie=None):
        cs = pl.ds(pl.multiple_of(t * WIN, WIN), WIN) if not isinstance(t, int) else slice(t * WIN, (t + 1) * WIN)
        first = (lambda r0, n: xl_s[r0:r0 + n, cs].astype(f32)) if tie is None else (
            lambda r0, n: xl_s[r0:r0 + n, cs].astype(f32) + tie)
        m = _colsum(first, 64) * (1.0 / D)

        def sq(r0, n):
            xc = xl_s[r0:r0 + n, cs].astype(f32) - m
            return xc * xc

        rstd = lax.rsqrt(_colsum(sq, 96) * (1.0 / D) + EPS)
        for r0 in range(0, D, 48):
            xn_s[t if isinstance(t, int) else 0, r0:r0 + 48, :] = ((xl_s[r0:r0 + 48, cs].astype(f32) - m) * rstd).astype(bf16)
        xnp_s[:, cs] = _as_u32(xn_s[t if isinstance(t, int) else 0])

    def proj(base, c):
        return jnp.dot(wT[pl.ds(base + c * MC, MC), :], _as_bf16(xnp_s[...]), preferred_element_type=f32)

    def transpose_k_tied(g, a):
        kw = _as_u32(kt_s[window(g // 2, g % 2), :]) | jnp.concatenate([_zero_bits_after(a)] * (L // WIN), axis=1)
        k_s[g, :, 0:VW] = _as_bf16(kw).T

    def proj_q(c0=0, c1=D // MC, kt=None):
        for c in range(c0, c1):
            q = proj(0, c)
            qt_s[pl.ds(c * MC, MC), :] = (q * QSCALE).astype(bf16)
            pqt_s[pl.ds(c * MC, MC), :] = _phi(q).astype(bf16)
            if kt is not None:
                for g in kt[c]:
                    transpose_k_tied(g, q)

    def proj_k(c0=0, c1=D // MC):
        for c in range(c0, c1):
            k = proj(D, c)
            kt_s[pl.ds(c * MC, MC), :] = k.astype(bf16)
            pkt_s[pl.ds(c * MC, MC), :] = _phi(k).astype(bf16)

    def transpose_k():
        for g in range(NG):
            k_s[g, :, 0:VW] = kt_s[window(g // 2, g % 2), :].T

    def proj_v(kt=None):
        for c in range(D // MC):
            v = proj(2 * D, c)
            vt_s[pl.ds(c * MC, MC), :] = v.astype(bf16)
            if kt is not None:
                for g in kt[c]:
                    transpose_k_tied(g, v)

    def mem_read():
        r80 = lax.broadcasted_iota(jnp.int32, (VW, L), 0)
        for g in range(NG):
            par = g % 2
            rows = window(g // 2, par)
            nd = jnp.dot(mext_s[g].astype(bf16), _pad_rows(pqt_s[rows, :], WIN), preferred_element_type=f32)
            rden = 1.0 / (nd[_free0(par):_free0(par) + 8] + 1e-6)
            scale = jnp.broadcast_to(rden[0:1], (VW, L))
            for a in range(1, G):
                scale = jnp.where(r80 >= 8 * par + a * DH, rden[a:a + 1], scale)
            nd_s[g] = nd * scale * jnp.concatenate([g_s[rows, :]] * (L // WIN), axis=1)

    def mem_update(g):
        free0 = _free0(g % 2) // 2
        rows = window(g // 2, g % 2)
        r = lax.broadcasted_iota(jnp.int32, (VW // 2, L), 0)
        lhs = _as_u32(vt_s[rows, :])
        lhs = _as_bf16(jnp.where((r >= free0) & (r < free0 + 4), u32(ONES2), lhs))
        upd = lax.dot_general(lhs, _pad_rows(pkt_s[rows, :], WIN), NT, preferred_element_type=f32)
        mext_s[g] += jnp.where(mmask_s[g % 2] > 0.5, upd, 0.0)

    def b_chunk(pr, par, st, mx, state, j, i):
        if i == 0:
            q = _as_u32(qt_s[window(pr, par), j * WIN:(j + 1) * WIN])
            lo = 4 * par
            state["rhs"] = jnp.concatenate(
                [_as_bf16(_pad_rows(jnp.where((r40 >= lo + 9 * a) & (r40 < lo + 9 * a + 9), q, u32(0)), WIN // 2))
                 for a in range(G)], axis=1)
        s = jnp.dot(k_s[2 * pr + par, i * WIN:(i + 1) * WIN, :], state["rhs"], preferred_element_type=f32)
        if i == j:
            s = s + jnp.where(kq_r > kq_c, MASKV, 0.0)
        m = jnp.max(s, axis=0, keepdims=True)
        state["m"] = m if i == 0 else jnp.maximum(state["m"], m)
        st[SOFF[j] + i * WIN:SOFF[j] + (i + 1) * WIN, :] = s
        if i == j:
            mx[j] = jnp.broadcast_to(state["m"], (8, G * WIN))

    def c_chunk(pr, par, st, mx, state, j, i):
        g = 2 * pr + par
        for a in range(G):
            row = par * GD + a * DH
            start = (row // 16) * 16
            off = row - start
            rows = pl.ds(pl.multiple_of(pr * (2 * GD) + start, 16), 32)
            one_row = ((off + DH) % 32) // 2
            r16 = lax.broadcasted_iota(jnp.int32, (16, WIN), 0)
            vt = _as_u32(vt_s[rows, i * WIN:(i + 1) * WIN])
            vt = _as_bf16(jnp.where(r16 == one_row, u32(ONES2), vt))
            hs = slice(a * WIN, (a + 1) * WIN)
            p = jnp.exp2(st[SOFF[j] + i * WIN:SOFF[j] + (i + 1) * WIN, hs] - mx[j, 0:1, hs]).astype(bf16)
            d = jnp.dot(vt, p, preferred_element_type=f32)
            acc = d if i == 0 else state[a] + d
            state[a] = acc
            if i == j:
                qs = slice(j * WIN, (j + 1) * WIN)
                lsum = acc[2 * one_row:2 * one_row + 1, :]
                ls = start - _woff(par)
                o = nd_s[g, ls:ls + 32, qs] + ((1.0 - g_s[rows, :]) * _recip(lsum)) * acc
                r32 = lax.broadcasted_iota(jnp.int32, (32, WIN), 0)
                keep = (r32 >= off) & (r32 < off + DH)
                pltpu.store(oT_s.at[rows, qs], o, mask=keep)

    bufs = ((stA, mxA), (stB, mxB))

    def b_all0():
        sb = {}
        for (j, i) in CHUNKS:
            b_chunk(0, 0, *bufs[0], sb, j, i)

    def step(pr, par):
        npr, npar = (pr, 1) if par == 0 else (pr + 1, 0)
        sb, sc = {}, {}
        for (j, i) in CHUNKS:
            b_chunk(npr, npar, *bufs[1 - par], sb, j, i)
            c_chunk(pr, par, *bufs[par], sc, j, i)

    def attention(update_memory):
        z = zero_s[0]
        for g in range(NG - 1):
            step(z + g // 2, g % 2)
        sc = {}
        for n, (j, i) in enumerate(CHUNKS):
            if n < NG and update_memory:
                mem_update(n)
            c_chunk(z + NG // 2 - 1, 1, *bufs[1], sc, j, i)

    def pack_ot():
        at_s[...] = oT_s[...].astype(bf16)
        otp_s[...] = _as_u32(at_s[...])

    def out_proj(nsplit=1, with_ln1=False):
        pack_ot()
        w = L // nsplit
        for p in range(nsplit):
            cs = slice(p * w, (p + 1) * w)
            for c in range(D // MC):
                a = jnp.dot(woT[pl.ds(c * MC, MC), :], _as_bf16(otp_s[:, cs]), preferred_element_type=f32)
                at_s[pl.ds(c * MC, MC), cs] = a.astype(bf16)
                if with_ln1 and c < L // WIN:
                    bits = pltpu.bitcast(a[0:8, c * WIN:(c + 1) * WIN], u32)
                    zero = pltpu.bitcast(lax.shift_right_logical(lax.shift_right_logical(bits, u32(16)), u32(16)), f32)
                    ln1_tile(c, zero[0:1, :])

    LW = 2 * WIN

    def ln2_strip(t, x_s, o_s):
        cs = slice(t * LW, (t + 1) * LW)
        for r0 in range(0, D, 32):
            h_s[r0:r0 + 32, cs] = (x_s[r0:r0 + 32, cs].astype(f32) + at_s[r0:r0 + 32, cs].astype(f32)).astype(bf16)
        m, rstd = _ln_stats(lambda r0, n: h_s[r0:r0 + n, cs].astype(f32))
        racc = None
        for r0 in range(0, D, 48):
            hf = h_s[r0:r0 + 48, cs].astype(f32)
            hn = ((hf - m) * rstd).astype(bf16)
            hn_s[r0:r0 + 48, cs] = hn
            hnf = hn.astype(f32)
            o_s[r0:r0 + 48, cs] = (hf + hnf).astype(bf16)
            wr = wr_s[r0:r0 + 48, :]
            p = _fold8(hnf * jnp.concatenate([wr] * (LW // WIN), axis=1))
            racc = p if racc is None else racc + p
        return jnp.sum(racc, axis=0, keepdims=True)

    def ln2(s, x_s, o_s, copy):
        rs = [ln2_strip(t, x_s, o_s) for t in range(L // LW)]
        copy.start()
        r = jnp.concatenate(rs, axis=1).astype(bf16).astype(f32)
        rmax = jnp.max(r)
        ridx = lax.broadcasted_iota(jnp.int32, (1, L), 1)
        amax = jnp.min(jnp.where(r == rmax, ridx, L))

        @pl.when(rmax > best_s[0])
        def _():
            best_s[0] = rmax
            best_s[1] = (amax + s * L).astype(f32)
            ts = pl.ds(pl.multiple_of((amax >> 7) << 7, WIN), WIN)
            bh_s[...] = _as_u32(h_s[:, ts])
            bhn_s[...] = _as_u32(hn_s[:, ts])

    xl_copy(0).wait()
    small_copy(0).start()
    small_copy(1).start()
    for t in range(L // WIN):
        ln1_tile(t)
    wq_copy(0).wait()
    w_copy(3).start()
    fence()
    xl_copy(1).start()
    fence()
    xr_copy(0).start()
    wT[pl.ds(0, WQA), :] = wraw[0, :, 0:WQA].T
    proj_q(0, 4)
    wq_copy(1).wait()
    w_copy(1).wait()
    wT[pl.ds(WQA, D - WQA), :] = wraw[0, :, WQA:D].T
    wT[pl.ds(D, D), :] = wraw[1].T
    proj_q(4, D // MC)
    proj_k(0, 4)
    w_copy(2).wait()
    w_copy(3).wait()
    small_copy(0).wait()
    small_copy(1).wait()
    wT[pl.ds(2 * D, D), :] = wraw[2].T
    woT[...] = wraw[3].T
    small_setup()
    proj_k(4, D // MC)
    transpose_k()
    proj_v()
    b_all0()

    def segment(s, carry):
        attention(True)

        @pl.when(s > 0)
        def _():
            out_copy(s - 1).wait()

        xr_copy(s).wait()
        xl_copy(s + 1).wait()
        fence()
        for i in range(3):
            @pl.when(s == i)
            def _():
                moe_copy(i).start()

        out_proj(1, True)
        proj_k()
        proj_v(KTV)
        proj_q(kt=KTQ)
        mem_read()
        b_all0()
        ln2(s, xr_s, out_s, out_copy(s))

        @pl.when(s + 2 < NSEG)
        def _():
            xr_copy(s + 1).start()
            xl_copy(s + 2).start()

        return carry

    lax.fori_loop(0, NSEG - 1, segment, 0)

    last_copy = pltpu.make_async_copy(out2_s, out_hbm.at[:, cols(NSEG - 1)], sem_o.at[1])
    attention(False)
    out_proj(2)
    ln2(NSEG - 1, xl_s, out2_s, last_copy)

    idx = best_s[1].astype(jnp.int32)
    tile = pl.ds(pl.multiple_of((idx >> 7) << 7, WIN), WIN)
    lane = idx & (WIN - 1)
    for i in range(3):
        moe_copy(i).wait()
    hn_t = _as_bf16(bhn_s[...])
    onehot = (lax.broadcasted_iota(jnp.int32, (16, WIN), 1) == lane).astype(f32).astype(bf16)
    xs = lax.dot_general(onehot, hn_t, NT, preferred_element_type=f32).astype(bf16)
    FC = 4 * WIN
    RB = 64
    for c in range(F // FC):
        cs = slice(c * FC, (c + 1) * FC)
        gt = jnp.dot(xs, wg_v[:, cs], preferred_element_type=f32)[0:8].astype(bf16).astype(f32)
        up = jnp.dot(xs, wu_v[:, cs], preferred_element_type=f32)[0:8].astype(bf16).astype(f32)
        act = (gt * (1.0 / (1.0 + jnp.exp(-gt)))).astype(bf16).astype(f32) * up
        act = act.astype(bf16).astype(f32)
        for rb in range(D // RB):
            p = acc_s[rb * RB:(rb + 1) * RB, :]
            for t in range(0, FC // WIN, 2):
                w2 = wd_v[rb * RB:(rb + 1) * RB, c * FC + t * WIN:c * FC + (t + 2) * WIN].astype(f32)
                w2 = w2 * act[0:1, t * WIN:(t + 2) * WIN]
                p = p + w2[:, 0:WIN] + w2[:, WIN:2 * WIN]
            acc_s[rb * RB:(rb + 1) * RB, :] = p
    y = jnp.sum(acc_s[...], axis=1, keepdims=True)
    rsel = jnp.full((1, 1), best_s[0], f32)
    y = y.astype(bf16).astype(f32) * (1.0 / (1.0 + jnp.exp(-rsel)))
    lanes = lax.broadcasted_iota(jnp.int32, (D, WIN), 1)
    yt = jnp.where(lanes == lane, y.astype(bf16).astype(f32), 0.0)
    t = (hn_t.astype(f32) + yt).astype(bf16).astype(f32)
    out_copy(NSEG - 2).wait()
    last_copy.wait()
    fix_s[...] = (_as_bf16(bh_s[...]).astype(f32) + t).astype(bf16)
    fix = pltpu.make_async_copy(fix_s, out_hbm.at[:, tile], sem_o.at[0])
    fix.start()
    fix.wait()


@jax.jit
def pallas_sequential_preLN__memory_aug_infini_attn__moe_arch_mod__prompt_kernel(
    A_x: jax.Array,
    A_wq: jax.Array,
    A_wk: jax.Array,
    A_wv: jax.Array,
    A_wo: jax.Array,
    A_beta: jax.Array,
    B_x: jax.Array,
    B_w_r: jax.Array,
    B_w_gate: jax.Array,
    B_w_up: jax.Array,
    B_w_down: jax.Array,
):
    del B_x
    hbm = pl.BlockSpec(memory_space=pltpu.HBM)
    out_t = pl.pallas_call(
        _kernel,
        out_shape=jax.ShapeDtypeStruct((D, S), bf16),
        in_specs=[hbm] * 10,
        out_specs=hbm,
        scratch_shapes=[
            pltpu.VMEM((D, L), bf16),
            pltpu.VMEM((D, L), bf16),
            pltpu.VMEM((4, D, D), bf16),
            pltpu.VMEM((3 * D, D), bf16),
            pltpu.VMEM((D, D), bf16),
            pltpu.VMEM((D, F), bf16),
            pltpu.VMEM((D, F), bf16),
            pltpu.VMEM((D, F), bf16),
            pltpu.VMEM((4, D, WIN), bf16),
            pltpu.VMEM((D // 2, L), u32),
            pltpu.VMEM((D, L), bf16),
            pltpu.VMEM((D, L), bf16),
            pltpu.VMEM((D, L), bf16),
            pltpu.VMEM((NG, L, WIN), bf16),
            pltpu.VMEM((D, L), bf16),
            pltpu.VMEM((D, L), bf16),
            pltpu.VMEM((1280, G * WIN), f32),
            pltpu.VMEM((1280, G * WIN), f32),
            pltpu.VMEM((4, 8, G * WIN), f32),
            pltpu.VMEM((4, 8, G * WIN), f32),
            pltpu.VMEM((NG, VW, L), f32),
            pltpu.VMEM((NG, VW, WIN), f32),
            pltpu.VMEM((2, VW, WIN), f32),
            pltpu.VMEM((D, L), f32),
            pltpu.VMEM((D // 2, L), u32),
            pltpu.VMEM((D, L), bf16),
            pltpu.VMEM((D, WIN), f32),
            pltpu.VMEM((D, WIN), f32),
            pltpu.VMEM((D, L), bf16),
            pltpu.VMEM((D, L), bf16),
            pltpu.VMEM((D, L), bf16),
            pltpu.VMEM((D, L), bf16),
            pltpu.VMEM((D // 2, WIN), u32),
            pltpu.VMEM((D // 2, WIN), u32),
            pltpu.VMEM((D, WIN), bf16),
            pltpu.VMEM((D, WIN), f32),
            pltpu.VMEM((1, H), bf16),
            pltpu.VMEM((D,), bf16),
            pltpu.SMEM((2,), f32),
            pltpu.SMEM((1,), jnp.int32),
            pltpu.SemaphoreType.DMA((2,)),
            pltpu.SemaphoreType.DMA((5,)),
            pltpu.SemaphoreType.DMA((3,)),
            pltpu.SemaphoreType.DMA((2,)),
            pltpu.SemaphoreType.DMA((2,)),
            pltpu.SemaphoreType.REGULAR,
        ],
        compiler_params=pltpu.CompilerParams(vmem_limit_bytes=100 * 1024 * 1024),
    )(A_x.reshape(S, D).T, A_wq, A_wk, A_wv, A_wo, A_beta.reshape(1, H), B_w_r,
      B_w_gate, B_w_up, B_w_down.T)
    return out_t.T.reshape(1, S, D)
```

```python
import os
import jax
import jax.numpy as jnp
from jax import lax
import jax.experimental.pallas as pl
import jax.experimental.pallas.tpu as pltpu

S = 2048
D = 576
H = 32
DH = 18
NSEG = 4
L = 512
F = 4608
G = 4
NG = H // G
GD = G * DH
WIN = 128
VW = 80
KTV = [[0], [], [1], [], [2], [3]]
KTQ = [[], [4], [5], [], [6], [7]]
MC = 96
LOG2E = 1.4426950408889634
SCALE = 0.2353515625
QSCALE = SCALE * LOG2E
MASKV = -1e9 * LOG2E
EPS = 1e-5
SOFF = (0, 128, 384, 768)
CHUNKS = [(j, i) for j in (3, 2, 1, 0) for i in range(j + 1)]
f32 = jnp.float32
bf16 = jnp.bfloat16
u32 = jnp.uint32
NT = (((1,), (1,)), ((), ()))
ONES2 = 0x3F803F80


def _fdiv18(i):
    return jnp.floor((i.astype(f32) + 0.5) * (1.0 / DH)).astype(jnp.int32)


def _phi(t):
    return jnp.where(t > 0, t + 1.0, jnp.exp(t))


def _fold8(x):
    parts = [x[i:i + 8] for i in range(0, x.shape[0], 8)]
    while len(parts) > 1:
        parts = [parts[i] + parts[i + 1] if i + 1 < len(parts) else parts[i] for i in range(0, len(parts), 2)]
    return parts[0]


def _fold8max(x):
    parts = [x[i:i + 8] for i in range(0, x.shape[0], 8)]
    while len(parts) > 1:
        parts = [jnp.maximum(parts[i], parts[i + 1]) if i + 1 < len(parts) else parts[i]
                 for i in range(0, len(parts), 2)]
    return parts[0]


def _colsum(load, rb):
    acc = _fold8(load(0, rb))
    for r0 in range(rb, D, rb):
        acc = acc + _fold8(load(r0, rb))
    return jnp.sum(acc, axis=0, keepdims=True)


def _ln_stats(load):
    m = _colsum(load, 64) * (1.0 / D)

    def sq(r0, n):
        xc = load(r0, n) - m
        return xc * xc

    v = _colsum(sq, 96) * (1.0 / D)
    return m, lax.rsqrt(v + EPS)


def _recip(x):
    r = pl.reciprocal(x, approx=True)
    return r * (2.0 - x * r)


def _zero_bits_after(a):
    bits = pltpu.bitcast(a[0:8, 0:WIN], u32)
    return lax.shift_right_logical(lax.shift_right_logical(bits, u32(16)), u32(16))[0:1]


def _woff(par):
    return 16 * ((GD * par) // 16)


def _free0(par):
    return GD if par == 0 else 0


def _as_bf16(x):
    return pltpu.bitcast(x, bf16)


def _as_u32(x):
    return pltpu.bitcast(x, u32)


def _pad_rows(a, n):
    return jnp.concatenate([a, jnp.zeros((n - a.shape[0], a.shape[1]), a.dtype)], axis=0)


def _kernel(x_hbm, wq_hbm, wk_hbm, wv_hbm, wo_hbm, beta_hbm, wr_hbm, wg_hbm, wu_hbm, wd_hbm,
            out_hbm,
            xl_s, xr_s, wraw, wT, woT, wg_v, wu_v, wd_v,
            xn_s, xnp_s, qt_s, pqt_s, kt_s, k_s, pkt_s, vt_s, stA, stB, mxA, mxB, nd_s, mext_s, mmask_s,
            oT_s, otp_s, at_s, g_s, wr_s, h_s, hn_s, out_s, out2_s, bh_s, bhn_s, fix_s, acc_s, beta_ref, wr_ref, best_s, zero_s,
            sem_x, sem_w, sem_moe, sem_o, sem_s, sem_f):
    def cols(s):
        return pl.ds(pl.multiple_of(s * L, L), L)

    def window(pr, par):
        return pl.ds(pl.multiple_of(pr * (2 * GD) + _woff(par), 16), VW)

    def xl_copy(s):
        return pltpu.make_async_copy(x_hbm.at[:, cols(s)], xl_s, sem_x.at[0])

    def xr_copy(s):
        return pltpu.make_async_copy(x_hbm.at[:, cols(s)], xr_s, sem_x.at[1])

    def w_copy(i):
        src = (wq_hbm, wk_hbm, wv_hbm, wo_hbm)[i]
        return pltpu.make_async_copy(src, wraw.at[i], sem_w.at[i])

    WQA = 3 * WIN

    def wq_copy(part):
        cs = pl.ds(0, WQA) if part == 0 else pl.ds(WQA, D - WQA)
        return pltpu.make_async_copy(wq_hbm.at[:, cs], wraw.at[0, :, cs], sem_w.at[0 if part else 4])

    def moe_copy(i):
        src, dst = ((wg_hbm, wg_v), (wu_hbm, wu_v), (wd_hbm, wd_v))[i]
        return pltpu.make_async_copy(src, dst, sem_moe.at[i])

    def out_copy(s):
        return pltpu.make_async_copy(out_s, out_hbm.at[:, cols(s)], sem_o.at[0])

    def small_copy(i):
        src, dst = ((beta_hbm, beta_ref), (wr_hbm, wr_ref))[i]
        return pltpu.make_async_copy(src, dst, sem_s.at[i])

    def fence():
        pl.semaphore_signal(sem_f, 1)
        pl.semaphore_wait(sem_f, 1)

    xl_copy(0).start()
    fence()
    wq_copy(0).start()
    fence()
    wq_copy(1).start()
    fence()
    w_copy(1).start()
    fence()
    w_copy(2).start()

    mext_s[...] = jnp.zeros_like(mext_s)
    k_s[...] = jnp.zeros_like(k_s)
    nd_s[...] = jnp.zeros_like(nd_s)
    acc_s[...] = jnp.zeros_like(acc_s)
    bh_s[...] = jnp.zeros_like(bh_s)
    bhn_s[...] = jnp.zeros_like(bhn_s)
    for par in range(2):
        r = lax.broadcasted_iota(jnp.int32, (VW, WIN), 0)
        l = lax.broadcasted_iota(jnp.int32, (VW, WIN), 1)
        free0 = _free0(par)
        hl = _fdiv18(l - 8 * par + DH) - 1
        he = jnp.where((r >= free0) & (r < free0 + 8), r - free0, _fdiv18(r - 8 * par + DH) - 1)
        ok = (he == hl) & (l >= 8 * par) & (l < 8 * par + GD)
        mmask_s[par] = jnp.where(ok, 1.0, 0.0).astype(f32)
    best_s[0] = jnp.float32(-jnp.inf)
    zero_s[0] = jnp.int32(0)
    best_s[1] = jnp.float32(0.0)

    def small_setup():
        beta = beta_ref[...].astype(f32)
        gsig = 1.0 / (1.0 + jnp.exp(-beta))
        fi = lax.broadcasted_iota(jnp.int32, (D, H), 0)
        hi = lax.broadcasted_iota(jnp.int32, (D, H), 1)
        gcol = jnp.sum(jnp.where(_fdiv18(fi) == hi, gsig, 0.0), axis=1, keepdims=True)
        g_s[...] = jnp.broadcast_to(gcol, (D, WIN))
        wr_s[...] = jnp.broadcast_to(wr_ref[...].astype(f32).reshape(1, D), (WIN, D)).T

    QW = WIN // G

    def lane_quarter(rows):
        return lax.broadcasted_iota(jnp.int32, (rows, WIN), 1) >> 5

    def by_quarter(vals, qq, rows):
        lq = lane_quarter(rows)
        out = vals[(G - 1 - qq) % G]
        for lane_q in range(G - 1):
            out = jnp.where(lq == lane_q, vals[(lane_q - qq) % G], out)
        return out

    def diag_bias(query, key0):
        k = lax.broadcasted_iota(jnp.int32, query.shape, 0) + key0
        return jnp.where(k > query, MASKV, 0.0)

    lane_q32 = lax.broadcasted_iota(jnp.int32, (QW, WIN), 1)
    bias0 = jnp.concatenate([diag_bias((lane_q32 - QW * a) & (WIN - 1), 0) for a in range(G)], axis=1)
    bias_q = diag_bias(lane_q32 & (QW - 1), 0)
    r40 = lax.broadcasted_iota(jnp.int32, (VW // 2, WIN), 0)

    def ln1_tile(t, tie=None):
        cs = pl.ds(pl.multiple_of(t * WIN, WIN), WIN) if not isinstance(t, int) else slice(t * WIN, (t + 1) * WIN)
        first = (lambda r0, n: xl_s[r0:r0 + n, cs].astype(f32)) if tie is None else (
            lambda r0, n: xl_s[r0:r0 + n, cs].astype(f32) + tie)
        m = _colsum(first, 64) * (1.0 / D)

        def sq(r0, n):
            xc = xl_s[r0:r0 + n, cs].astype(f32) - m
            return xc * xc

        rstd = lax.rsqrt(_colsum(sq, 96) * (1.0 / D) + EPS)
        for r0 in range(0, D, 48):
            xn_s[t if isinstance(t, int) else 0, r0:r0 + 48, :] = ((xl_s[r0:r0 + 48, cs].astype(f32) - m) * rstd).astype(bf16)
        xnp_s[:, cs] = _as_u32(xn_s[t if isinstance(t, int) else 0])

    def proj(base, c):
        return jnp.dot(wT[pl.ds(base + c * MC, MC), :], _as_bf16(xnp_s[...]), preferred_element_type=f32)

    def transpose_k_tied(g, a):
        kw = _as_u32(kt_s[window(g // 2, g % 2), :]) | jnp.concatenate([_zero_bits_after(a)] * (L // WIN), axis=1)
        k_s[g, :, 0:VW] = _as_bf16(kw).T

    def proj_q(c0=0, c1=D // MC, kt=None):
        for c in range(c0, c1):
            q = proj(0, c)
            qt_s[pl.ds(c * MC, MC), :] = (q * QSCALE).astype(bf16)
            pqt_s[pl.ds(c * MC, MC), :] = _phi(q).astype(bf16)
            if kt is not None:
                for g in kt[c]:
                    transpose_k_tied(g, q)

    def proj_k(c0=0, c1=D // MC):
        for c in range(c0, c1):
            k = proj(D, c)
            kt_s[pl.ds(c * MC, MC), :] = k.astype(bf16)
            pkt_s[pl.ds(c * MC, MC), :] = _phi(k).astype(bf16)

    def transpose_k():
        for g in range(NG):
            k_s[g, :, 0:VW] = kt_s[window(g // 2, g % 2), :].T

    def proj_v(kt=None):
        for c in range(D // MC):
            v = proj(2 * D, c)
            vt_s[pl.ds(c * MC, MC), :] = v.astype(bf16)
            if kt is not None:
                for g in kt[c]:
                    transpose_k_tied(g, v)

    def mem_read():
        r80 = lax.broadcasted_iota(jnp.int32, (VW, L), 0)
        for g in range(NG):
            par = g % 2
            rows = window(g // 2, par)
            nd = jnp.dot(mext_s[g].astype(bf16), _pad_rows(pqt_s[rows, :], WIN), preferred_element_type=f32)
            rden = 1.0 / (nd[_free0(par):_free0(par) + 8] + 1e-6)
            scale = jnp.broadcast_to(rden[0:1], (VW, L))
            for a in range(1, G):
                scale = jnp.where(r80 >= 8 * par + a * DH, rden[a:a + 1], scale)
            nd_s[g] = nd * scale * jnp.concatenate([g_s[rows, :]] * (L // WIN), axis=1)

    def mem_update(g):
        free0 = _free0(g % 2) // 2
        rows = window(g // 2, g % 2)
        r = lax.broadcasted_iota(jnp.int32, (VW // 2, L), 0)
        lhs = _as_u32(vt_s[rows, :])
        lhs = _as_bf16(jnp.where((r >= free0) & (r < free0 + 4), u32(ONES2), lhs))
        upd = lax.dot_general(lhs, _pad_rows(pkt_s[rows, :], WIN), NT, preferred_element_type=f32)
        mext_s[g] += jnp.where(mmask_s[g % 2] > 0.5, upd, 0.0)

    def b_chunk(pr, par, st, mx, state, j, i):
        if i == 0:
            q = _as_u32(qt_s[window(pr, par), j * WIN:(j + 1) * WIN])
            lo = 4 * par
            state["tiles"] = [
                _pad_rows(jnp.where((r40 >= lo + 9 * a) & (r40 < lo + 9 * a + 9),
                                    pltpu.roll(q, QW * a, 1) if a else q, u32(0)), WIN // 2)
                for a in range(G)]
            state["rhs"] = jnp.concatenate([_as_bf16(t) for t in state["tiles"]], axis=1)
        g = 2 * pr + par
        r0 = SOFF[j] + i * WIN
        k0 = i * WIN
        if i < j:
            s = jnp.dot(k_s[g, k0:k0 + WIN, :], state["rhs"], preferred_element_type=f32)
            m = _fold8max(s)
            st[r0:r0 + WIN, :] = s
        else:
            wq = [_as_bf16(by_quarter(state["tiles"], qq, WIN // 2)) for qq in range(1, G)]
            s = jnp.dot(k_s[g, k0:k0 + QW, :], state["rhs"], preferred_element_type=f32) + bias0
            st[r0:r0 + QW, :] = s
            m = _fold8max(s)
            mq = [None] * G
            for kq in range(1, G):
                rhs = jnp.concatenate(wq[kq - 1:], axis=1) if kq < G - 1 else wq[G - 2]
                sk = jnp.dot(k_s[g, k0 + kq * QW:k0 + (kq + 1) * QW, :], rhs, preferred_element_type=f32)
                for qq in range(kq, G):
                    t = sk[:, (qq - kq) * WIN:(qq - kq + 1) * WIN]
                    if qq == kq:
                        t = t + bias_q
                    st[r0 + kq * QW:r0 + (kq + 1) * QW, (qq - 1) * WIN:qq * WIN] = t
                    tm = _fold8max(t)
                    mq[qq] = tm if mq[qq] is None else jnp.maximum(mq[qq], tm)
            lq = lane_quarter(8)
            extra = []
            for a in range(G):
                e = jnp.full((8, WIN), -jnp.inf, f32)
                for qq in range(1, G):
                    e = jnp.where(lq == (qq + a) % G, mq[qq], e)
                extra.append(e)
            m = jnp.maximum(m, jnp.concatenate(extra, axis=1))
        state["m"] = m if i == 0 else jnp.maximum(state["m"], m)
        if i == j:
            mx[j] = jnp.broadcast_to(jnp.max(state["m"], axis=0, keepdims=True), (8, G * WIN))

    def c_chunk(pr, par, st, mx, state, j, i):
        g = 2 * pr + par
        r0 = SOFF[j] + i * WIN
        if i == j:
            ms = [mx[j, 0:1, a * WIN:(a + 1) * WIN] for a in range(G)]
            mw = [None] + [by_quarter(ms, qq, 1) for qq in range(1, G)]
            ew = {(kq, qq): jnp.exp2(st[r0 + kq * QW:r0 + (kq + 1) * QW, (qq - 1) * WIN:qq * WIN] - mw[qq])
                  for kq in range(1, G) for qq in range(kq, G)}
        for a in range(G):
            row = par * GD + a * DH
            start = (row // 16) * 16
            off = row - start
            rows = pl.ds(pl.multiple_of(pr * (2 * GD) + start, 16), 32)
            one_row = ((off + DH) % 32) // 2
            r16 = lax.broadcasted_iota(jnp.int32, (16, WIN), 0)
            vt = _as_u32(vt_s[rows, i * WIN:(i + 1) * WIN])
            vt = _as_bf16(jnp.where(r16 == one_row, u32(ONES2), vt))
            hs = slice(a * WIN, (a + 1) * WIN)
            if i < j:
                p = jnp.exp2(st[r0:r0 + WIN, hs] - mx[j, 0:1, hs]).astype(bf16)
            else:
                lq = lane_quarter(QW)
                parts = [jnp.exp2(st[r0:r0 + QW, hs] - ms[a])]
                for kq in range(1, G):
                    e = jnp.zeros((QW, WIN), f32)
                    for qq in range(kq, G):
                        e = jnp.where(lq == (qq + a) % G, ew[(kq, qq)], e)
                    parts.append(e)
                p = jnp.concatenate(parts, axis=0).astype(bf16)
            d = jnp.dot(vt, p, preferred_element_type=f32)
            acc = d if i == 0 else state[a] + d
            state[a] = acc
            if i == j:
                qs = slice(j * WIN, (j + 1) * WIN)
                lsum = acc[2 * one_row:2 * one_row + 1, :]
                an = acc * _recip(lsum)
                if a:
                    an = pltpu.roll(an, WIN - QW * a, 1)
                ls = start - _woff(par)
                o = nd_s[g, ls:ls + 32, qs] + (1.0 - g_s[rows, :]) * an
                r32 = lax.broadcasted_iota(jnp.int32, (32, WIN), 0)
                keep = (r32 >= off) & (r32 < off + DH)
                pltpu.store(oT_s.at[rows, qs], o, mask=keep)

    bufs = ((stA, mxA), (stB, mxB))

    def b_all0():
        sb = {}
        for (j, i) in CHUNKS:
            b_chunk(0, 0, *bufs[0], sb, j, i)

    def step(pr, par):
        npr, npar = (pr, 1) if par == 0 else (pr + 1, 0)
        sb, sc = {}, {}
        for (j, i) in CHUNKS:
            c_chunk(pr, par, *bufs[par], sc, j, i)
            b_chunk(npr, npar, *bufs[1 - par], sb, j, i)

    def attention(update_memory):
        z = zero_s[0]
        for g in range(NG - 1):
            step(z + g // 2, g % 2)
        sc = {}
        for n, (j, i) in enumerate(CHUNKS):
            if n < NG and update_memory:
                mem_update(n)
            c_chunk(z + NG // 2 - 1, 1, *bufs[1], sc, j, i)

    def pack_ot():
        at_s[...] = oT_s[...].astype(bf16)
        otp_s[...] = _as_u32(at_s[...])

    def out_proj(nsplit=1, with_ln1=False):
        pack_ot()
        w = L // nsplit
        for p in range(nsplit):
            cs = slice(p * w, (p + 1) * w)
            for c in range(D // MC):
                a = jnp.dot(woT[pl.ds(c * MC, MC), :], _as_bf16(otp_s[:, cs]), preferred_element_type=f32)
                at_s[pl.ds(c * MC, MC), cs] = a.astype(bf16)
                if with_ln1 and c < L // WIN:
                    bits = pltpu.bitcast(a[0:8, c * WIN:(c + 1) * WIN], u32)
                    zero = pltpu.bitcast(lax.shift_right_logical(lax.shift_right_logical(bits, u32(16)), u32(16)), f32)
                    ln1_tile(c, zero[0:1, :])

    LW = 2 * WIN

    def ln2_strip(t, x_s, o_s):
        cs = slice(t * LW, (t + 1) * LW)
        for r0 in range(0, D, 32):
            h_s[r0:r0 + 32, cs] = (x_s[r0:r0 + 32, cs].astype(f32) + at_s[r0:r0 + 32, cs].astype(f32)).astype(bf16)
        m, rstd = _ln_stats(lambda r0, n: h_s[r0:r0 + n, cs].astype(f32))
        racc = None
        for r0 in range(0, D, 48):
            hf = h_s[r0:r0 + 48, cs].astype(f32)
            hn = ((hf - m) * rstd).astype(bf16)
            hn_s[r0:r0 + 48, cs] = hn
            hnf = hn.astype(f32)
            o_s[r0:r0 + 48, cs] = (hf + hnf).astype(bf16)
            wr = wr_s[r0:r0 + 48, :]
            p = _fold8(hnf * jnp.concatenate([wr] * (LW // WIN), axis=1))
            racc = p if racc is None else racc + p
        return jnp.sum(racc, axis=0, keepdims=True)

    def ln2(s, x_s, o_s, copy):
        rs = [ln2_strip(t, x_s, o_s) for t in range(L // LW)]
        copy.start()
        r = jnp.concatenate(rs, axis=1).astype(bf16).astype(f32)
        rmax = jnp.max(r)
        ridx = lax.broadcasted_iota(jnp.int32, (1, L), 1)
        amax = jnp.min(jnp.where(r == rmax, ridx, L))

        @pl.when(rmax > best_s[0])
        def _():
            best_s[0] = rmax
            best_s[1] = (amax + s * L).astype(f32)
            ts = pl.ds(pl.multiple_of((amax >> 7) << 7, WIN), WIN)
            bh_s[...] = _as_u32(h_s[:, ts])
            bhn_s[...] = _as_u32(hn_s[:, ts])

    xl_copy(0).wait()
    small_copy(0).start()
    small_copy(1).start()
    for t in range(L // WIN):
        ln1_tile(t)
    wq_copy(0).wait()
    w_copy(3).start()
    fence()
    xl_copy(1).start()
    fence()
    xr_copy(0).start()
    wT[pl.ds(0, WQA), :] = wraw[0, :, 0:WQA].T
    proj_q(0, 4)
    wq_copy(1).wait()
    w_copy(1).wait()
    wT[pl.ds(WQA, D - WQA), :] = wraw[0, :, WQA:D].T
    wT[pl.ds(D, D), :] = wraw[1].T
    proj_q(4, D // MC)
    proj_k(0, 4)
    w_copy(2).wait()
    w_copy(3).wait()
    small_copy(0).wait()
    small_copy(1).wait()
    wT[pl.ds(2 * D, D), :] = wraw[2].T
    woT[...] = wraw[3].T
    small_setup()
    proj_k(4, D // MC)
    transpose_k()
    proj_v()
    b_all0()

    def segment(s, carry):
        attention(True)

        @pl.when(s > 0)
        def _():
            out_copy(s - 1).wait()

        xr_copy(s).wait()
        xl_copy(s + 1).wait()
        fence()
        for i in range(3):
            @pl.when(s == i)
            def _():
                moe_copy(i).start()

        out_proj(1, True)
        proj_k()
        proj_v(KTV)
        proj_q(kt=KTQ)
        mem_read()
        b_all0()
        ln2(s, xr_s, out_s, out_copy(s))

        @pl.when(s + 2 < NSEG)
        def _():
            xr_copy(s + 1).start()
            xl_copy(s + 2).start()

        return carry

    lax.fori_loop(0, NSEG - 1, segment, 0)

    last_copy = pltpu.make_async_copy(out2_s, out_hbm.at[:, cols(NSEG - 1)], sem_o.at[1])
    attention(False)
    out_proj(2)
    ln2(NSEG - 1, xl_s, out2_s, last_copy)

    idx = best_s[1].astype(jnp.int32)
    tile = pl.ds(pl.multiple_of((idx >> 7) << 7, WIN), WIN)
    lane = idx & (WIN - 1)
    for i in range(3):
        moe_copy(i).wait()
    hn_t = _as_bf16(bhn_s[...])
    onehot = (lax.broadcasted_iota(jnp.int32, (16, WIN), 1) == lane).astype(f32).astype(bf16)
    xs = lax.dot_general(onehot, hn_t, NT, preferred_element_type=f32).astype(bf16)
    FC = 4 * WIN
    RB = 64
    for c in range(F // FC):
        cs = slice(c * FC, (c + 1) * FC)
        gt = jnp.dot(xs, wg_v[:, cs], preferred_element_type=f32)[0:8].astype(bf16).astype(f32)
        up = jnp.dot(xs, wu_v[:, cs], preferred_element_type=f32)[0:8].astype(bf16).astype(f32)
        act = (gt * (1.0 / (1.0 + jnp.exp(-gt)))).astype(bf16).astype(f32) * up
        act = act.astype(bf16).astype(f32)
        for rb in range(D // RB):
            p = acc_s[rb * RB:(rb + 1) * RB, :]
            for t in range(0, FC // WIN, 2):
                w2 = wd_v[rb * RB:(rb + 1) * RB, c * FC + t * WIN:c * FC + (t + 2) * WIN].astype(f32)
                w2 = w2 * act[0:1, t * WIN:(t + 2) * WIN]
                p = p + w2[:, 0:WIN] + w2[:, WIN:2 * WIN]
            acc_s[rb * RB:(rb + 1) * RB, :] = p
    y = jnp.sum(acc_s[...], axis=1, keepdims=True)
    rsel = jnp.full((1, 1), best_s[0], f32)
    y = y.astype(bf16).astype(f32) * (1.0 / (1.0 + jnp.exp(-rsel)))
    lanes = lax.broadcasted_iota(jnp.int32, (D, WIN), 1)
    yt = jnp.where(lanes == lane, y.astype(bf16).astype(f32), 0.0)
    t = (hn_t.astype(f32) + yt).astype(bf16).astype(f32)
    out_copy(NSEG - 2).wait()
    last_copy.wait()
    fix_s[...] = (_as_bf16(bh_s[...]).astype(f32) + t).astype(bf16)
    fix = pltpu.make_async_copy(fix_s, out_hbm.at[:, tile], sem_o.at[0])
    fix.start()
    fix.wait()


@jax.jit
def pallas_sequential_preLN__memory_aug_infini_attn__moe_arch_mod__prompt_kernel(
    A_x: jax.Array,
    A_wq: jax.Array,
    A_wk: jax.Array,
    A_wv: jax.Array,
    A_wo: jax.Array,
    A_beta: jax.Array,
    B_x: jax.Array,
    B_w_r: jax.Array,
    B_w_gate: jax.Array,
    B_w_up: jax.Array,
    B_w_down: jax.Array,
):
    del B_x
    hbm = pl.BlockSpec(memory_space=pltpu.HBM)
    out_t = pl.pallas_call(
        _kernel,
        out_shape=jax.ShapeDtypeStruct((D, S), bf16),
        in_specs=[hbm] * 10,
        out_specs=hbm,
        scratch_shapes=[
            pltpu.VMEM((D, L), bf16),
            pltpu.VMEM((D, L), bf16),
            pltpu.VMEM((4, D, D), bf16),
            pltpu.VMEM((3 * D, D), bf16),
            pltpu.VMEM((D, D), bf16),
            pltpu.VMEM((D, F), bf16),
            pltpu.VMEM((D, F), bf16),
            pltpu.VMEM((D, F), bf16),
            pltpu.VMEM((4, D, WIN), bf16),
            pltpu.VMEM((D // 2, L), u32),
            pltpu.VMEM((D, L), bf16),
            pltpu.VMEM((D, L), bf16),
            pltpu.VMEM((D, L), bf16),
            pltpu.VMEM((NG, L, WIN), bf16),
            pltpu.VMEM((D, L), bf16),
            pltpu.VMEM((D, L), bf16),
            pltpu.VMEM((1280, G * WIN), f32),
            pltpu.VMEM((1280, G * WIN), f32),
            pltpu.VMEM((4, 8, G * WIN), f32),
            pltpu.VMEM((4, 8, G * WIN), f32),
            pltpu.VMEM((NG, VW, L), f32),
            pltpu.VMEM((NG, VW, WIN), f32),
            pltpu.VMEM((2, VW, WIN), f32),
            pltpu.VMEM((D, L), f32),
            pltpu.VMEM((D // 2, L), u32),
            pltpu.VMEM((D, L), bf16),
            pltpu.VMEM((D, WIN), f32),
            pltpu.VMEM((D, WIN), f32),
            pltpu.VMEM((D, L), bf16),
            pltpu.VMEM((D, L), bf16),
            pltpu.VMEM((D, L), bf16),
            pltpu.VMEM((D, L), bf16),
            pltpu.VMEM((D // 2, WIN), u32),
            pltpu.VMEM((D // 2, WIN), u32),
            pltpu.VMEM((D, WIN), bf16),
            pltpu.VMEM((D, WIN), f32),
            pltpu.VMEM((1, H), bf16),
            pltpu.VMEM((D,), bf16),
            pltpu.SMEM((2,), f32),
            pltpu.SMEM((1,), jnp.int32),
            pltpu.SemaphoreType.DMA((2,)),
            pltpu.SemaphoreType.DMA((5,)),
            pltpu.SemaphoreType.DMA((3,)),
            pltpu.SemaphoreType.DMA((2,)),
            pltpu.SemaphoreType.DMA((2,)),
            pltpu.SemaphoreType.REGULAR,
        ],
        compiler_params=pltpu.CompilerParams(vmem_limit_bytes=100 * 1024 * 1024),
    )(A_x.reshape(S, D).T, A_wq, A_wk, A_wv, A_wo, A_beta.reshape(1, H), B_w_r,
      B_w_gate, B_w_up, B_w_down.T)
    return out_t.T.reshape(1, S, D)
```

```python
import os
import jax
import jax.numpy as jnp
from jax import lax
import jax.experimental.pallas as pl
import jax.experimental.pallas.tpu as pltpu

S = 2048
D = 576
H = 32
DH = 18
NSEG = 4
L = 512
F = 4608
G = 4
NG = H // G
GD = G * DH
WIN = 128
VW = 80
KTV = [[0], [], [1], [], [2], [3]]
KTQ = [[], [4], [5], [], [6], [7]]
MC = 96
LOG2E = 1.4426950408889634
SCALE = 0.2353515625
QSCALE = SCALE * LOG2E
MASKV = -1e9 * LOG2E
EPS = 1e-5
SOFF = (0, 128, 384, 768)
CHUNKS = [(j, i) for j in (3, 2, 1, 0) for i in range(j + 1)]
f32 = jnp.float32
bf16 = jnp.bfloat16
u32 = jnp.uint32
NT = (((1,), (1,)), ((), ()))
ONES2 = 0x3F803F80


def _fdiv18(i):
    return jnp.floor((i.astype(f32) + 0.5) * (1.0 / DH)).astype(jnp.int32)


def _phi(t):
    return jnp.where(t > 0, t + 1.0, jnp.exp(t))


def _fold8(x):
    parts = [x[i:i + 8] for i in range(0, x.shape[0], 8)]
    while len(parts) > 1:
        parts = [parts[i] + parts[i + 1] if i + 1 < len(parts) else parts[i] for i in range(0, len(parts), 2)]
    return parts[0]


def _fold8max(x):
    parts = [x[i:i + 8] for i in range(0, x.shape[0], 8)]
    while len(parts) > 1:
        parts = [jnp.maximum(parts[i], parts[i + 1]) if i + 1 < len(parts) else parts[i]
                 for i in range(0, len(parts), 2)]
    return parts[0]


def _colsum(load, rb):
    acc = _fold8(load(0, rb))
    for r0 in range(rb, D, rb):
        acc = acc + _fold8(load(r0, rb))
    return jnp.sum(acc, axis=0, keepdims=True)


def _ln_stats(load):
    m = _colsum(load, 64) * (1.0 / D)

    def sq(r0, n):
        xc = load(r0, n) - m
        return xc * xc

    v = _colsum(sq, 96) * (1.0 / D)
    return m, lax.rsqrt(v + EPS)


def _recip(x):
    r = pl.reciprocal(x, approx=True)
    return r * (2.0 - x * r)


def _zero_bits_after(a):
    bits = pltpu.bitcast(a[0:8, 0:WIN], u32)
    return lax.shift_right_logical(lax.shift_right_logical(bits, u32(16)), u32(16))[0:1]


def _woff(par):
    return 16 * ((GD * par) // 16)


def _free0(par):
    return GD if par == 0 else 0


def _as_bf16(x):
    return pltpu.bitcast(x, bf16)


def _as_u32(x):
    return pltpu.bitcast(x, u32)


def _pad_rows(a, n):
    return jnp.concatenate([a, jnp.zeros((n - a.shape[0], a.shape[1]), a.dtype)], axis=0)


def _kernel(x_hbm, wq_hbm, wk_hbm, wv_hbm, wo_hbm, beta_hbm, wr_hbm, wg_hbm, wu_hbm, wd_hbm,
            out_hbm,
            xl_s, xr_s, wraw, wT, woT, wg_v, wu_v, wd_v,
            xn_s, xnp_s, qt_s, pqt_s, kt_s, k_s, pkt_s, vt_s, stA, stB, mxA, mxB, nd_s, mext_s, mmask_s,
            oT_s, otp_s, at_s, g_s, wr_s, h_s, hn_s, out_s, out2_s, bh_s, bhn_s, fix_s, acc_s, beta_ref, wr_ref, best_s, zero_s,
            sem_x, sem_w, sem_moe, sem_o, sem_s, sem_f):
    def cols(s):
        return pl.ds(pl.multiple_of(s * L, L), L)

    def window(pr, par):
        return pl.ds(pl.multiple_of(pr * (2 * GD) + _woff(par), 16), VW)

    def xl_copy(s):
        return pltpu.make_async_copy(x_hbm.at[:, cols(s)], xl_s, sem_x.at[0])

    def xr_copy(s):
        return pltpu.make_async_copy(x_hbm.at[:, cols(s)], xr_s, sem_x.at[1])

    def w_copy(i):
        src = (wq_hbm, wk_hbm, wv_hbm, wo_hbm)[i]
        return pltpu.make_async_copy(src, wraw.at[i], sem_w.at[i])

    WQA = 3 * WIN

    def wq_copy(part):
        cs = pl.ds(0, WQA) if part == 0 else pl.ds(WQA, D - WQA)
        return pltpu.make_async_copy(wq_hbm.at[:, cs], wraw.at[0, :, cs], sem_w.at[0 if part else 4])

    def moe_copy(i):
        src, dst = ((wg_hbm, wg_v), (wu_hbm, wu_v), (wd_hbm, wd_v))[i]
        return pltpu.make_async_copy(src, dst, sem_moe.at[i])

    def out_copy(s):
        return pltpu.make_async_copy(out_s, out_hbm.at[:, cols(s)], sem_o.at[0])

    def small_copy(i):
        src, dst = ((beta_hbm, beta_ref), (wr_hbm, wr_ref))[i]
        return pltpu.make_async_copy(src, dst, sem_s.at[i])

    def fence():
        pl.semaphore_signal(sem_f, 1)
        pl.semaphore_wait(sem_f, 1)

    xl_copy(0).start()
    fence()
    wq_copy(0).start()
    fence()
    wq_copy(1).start()
    fence()
    w_copy(1).start()
    fence()
    w_copy(2).start()

    mext_s[...] = jnp.zeros_like(mext_s)
    k_s[...] = jnp.zeros_like(k_s)
    nd_s[...] = jnp.zeros_like(nd_s)
    acc_s[...] = jnp.zeros_like(acc_s)
    bh_s[...] = jnp.zeros_like(bh_s)
    bhn_s[...] = jnp.zeros_like(bhn_s)
    for par in range(2):
        r = lax.broadcasted_iota(jnp.int32, (VW, WIN), 0)
        l = lax.broadcasted_iota(jnp.int32, (VW, WIN), 1)
        free0 = _free0(par)
        hl = _fdiv18(l - 8 * par + DH) - 1
        he = jnp.where((r >= free0) & (r < free0 + 8), r - free0, _fdiv18(r - 8 * par + DH) - 1)
        ok = (he == hl) & (l >= 8 * par) & (l < 8 * par + GD)
        mmask_s[par] = jnp.where(ok, 1.0, 0.0).astype(f32)
    best_s[0] = jnp.float32(-jnp.inf)
    zero_s[0] = jnp.int32(0)
    best_s[1] = jnp.float32(0.0)

    def small_setup():
        beta = beta_ref[...].astype(f32)
        gsig = 1.0 / (1.0 + jnp.exp(-beta))
        fi = lax.broadcasted_iota(jnp.int32, (D, H), 0)
        hi = lax.broadcasted_iota(jnp.int32, (D, H), 1)
        gcol = jnp.sum(jnp.where(_fdiv18(fi) == hi, gsig, 0.0), axis=1, keepdims=True)
        g_s[...] = jnp.broadcast_to(gcol, (D, WIN))
        wr_s[...] = jnp.broadcast_to(wr_ref[...].astype(f32).reshape(1, D), (WIN, D)).T

    QW = WIN // G

    def lane_quarter(rows):
        return lax.broadcasted_iota(jnp.int32, (rows, WIN), 1) >> 5

    def by_quarter(vals, qq, rows):
        lq = lane_quarter(rows)
        out = vals[(G - 1 - qq) % G]
        for lane_q in range(G - 1):
            out = jnp.where(lq == lane_q, vals[(lane_q - qq) % G], out)
        return out

    def diag_bias(query, key0):
        k = lax.broadcasted_iota(jnp.int32, query.shape, 0) + key0
        return jnp.where(k > query, MASKV, 0.0)

    lane_q32 = lax.broadcasted_iota(jnp.int32, (QW, WIN), 1)
    bias0 = jnp.concatenate([diag_bias((lane_q32 - QW * a) & (WIN - 1), 0) for a in range(G)], axis=1)
    bias_q = diag_bias(lane_q32 & (QW - 1), 0)
    r40 = lax.broadcasted_iota(jnp.int32, (VW // 2, WIN), 0)

    def ln1_tile(t, tie=None):
        cs = pl.ds(pl.multiple_of(t * WIN, WIN), WIN) if not isinstance(t, int) else slice(t * WIN, (t + 1) * WIN)
        first = (lambda r0, n: xl_s[r0:r0 + n, cs].astype(f32)) if tie is None else (
            lambda r0, n: xl_s[r0:r0 + n, cs].astype(f32) + tie)
        m = _colsum(first, 64) * (1.0 / D)

        def sq(r0, n):
            xc = xl_s[r0:r0 + n, cs].astype(f32) - m
            return xc * xc

        rstd = lax.rsqrt(_colsum(sq, 96) * (1.0 / D) + EPS)
        for r0 in range(0, D, 48):
            xn_s[t if isinstance(t, int) else 0, r0:r0 + 48, :] = ((xl_s[r0:r0 + 48, cs].astype(f32) - m) * rstd).astype(bf16)
        xnp_s[:, cs] = _as_u32(xn_s[t if isinstance(t, int) else 0])

    def proj(base, c):
        return jnp.dot(_as_bf16(wT[pl.ds((base + c * MC) // 2, MC // 2), :]), _as_bf16(xnp_s[...]), preferred_element_type=f32)

    def transpose_k_tied(g, a):
        kw = _as_u32(kt_s[window(g // 2, g % 2), :]) | jnp.concatenate([_zero_bits_after(a)] * (L // WIN), axis=1)
        k_s[g, :, 0:VW] = _as_u32(_as_bf16(kw).T)

    def proj_q(c0=0, c1=D // MC, kt=None):
        for c in range(c0, c1):
            q = proj(0, c)
            qt_s[pl.ds(c * MC, MC), :] = (q * QSCALE).astype(bf16)
            pqt_s[pl.ds(c * MC, MC), :] = _phi(q).astype(bf16)
            if kt is not None:
                for g in kt[c]:
                    transpose_k_tied(g, q)

    def proj_k(c0=0, c1=D // MC):
        for c in range(c0, c1):
            k = proj(D, c)
            kt_s[pl.ds(c * MC, MC), :] = k.astype(bf16)
            pkt_s[pl.ds(c * MC, MC), :] = _phi(k).astype(bf16)

    def transpose_k():
        for g in range(NG):
            k_s[g, :, 0:VW] = _as_u32(kt_s[window(g // 2, g % 2), :].T)

    def proj_v(kt=None):
        for c in range(D // MC):
            v = proj(2 * D, c)
            vt_s[pl.ds(c * MC, MC), :] = v.astype(bf16)
            if kt is not None:
                for g in kt[c]:
                    transpose_k_tied(g, v)

    def mem_read():
        r80 = lax.broadcasted_iota(jnp.int32, (VW, L), 0)
        for g in range(NG):
            par = g % 2
            rows = window(g // 2, par)
            nd = jnp.dot(mext_s[g].astype(bf16), _pad_rows(pqt_s[rows, :], WIN), preferred_element_type=f32)
            rden = 1.0 / (nd[_free0(par):_free0(par) + 8] + 1e-6)
            scale = jnp.broadcast_to(rden[0:1], (VW, L))
            for a in range(1, G):
                scale = jnp.where(r80 >= 8 * par + a * DH, rden[a:a + 1], scale)
            nd_s[g] = nd * scale * jnp.concatenate([g_s[rows, :]] * (L // WIN), axis=1)

    def mem_update(g):
        free0 = _free0(g % 2) // 2
        rows = window(g // 2, g % 2)
        r = lax.broadcasted_iota(jnp.int32, (VW // 2, L), 0)
        lhs = _as_u32(vt_s[rows, :])
        lhs = _as_bf16(jnp.where((r >= free0) & (r < free0 + 4), u32(ONES2), lhs))
        upd = lax.dot_general(lhs, _pad_rows(pkt_s[rows, :], WIN), NT, preferred_element_type=f32)
        mext_s[g] += jnp.where(mmask_s[g % 2] > 0.5, upd, 0.0)

    def b_chunk(pr, par, st, mx, state, j, i):
        if i == 0:
            q = _as_u32(qt_s[window(pr, par), j * WIN:(j + 1) * WIN])
            lo = 4 * par
            state["tiles"] = [
                _pad_rows(jnp.where((r40 >= lo + 9 * a) & (r40 < lo + 9 * a + 9),
                                    pltpu.roll(q, QW * a, 1) if a else q, u32(0)), WIN // 2)
                for a in range(G)]
            state["rhs"] = jnp.concatenate([_as_bf16(t) for t in state["tiles"]], axis=1)
        g = 2 * pr + par
        r0 = SOFF[j] + i * WIN
        k0 = i * WIN
        if i < j:
            s = jnp.dot(_as_bf16(k_s[g, k0 // 2:(k0 + WIN) // 2, :]), state["rhs"], preferred_element_type=f32)
            m = _fold8max(s)
            st[r0:r0 + WIN, :] = s
        else:
            wq = [_as_bf16(by_quarter(state["tiles"], qq, WIN // 2)) for qq in range(1, G)]
            s = jnp.dot(_as_bf16(k_s[g, k0 // 2:(k0 + QW) // 2, :]), state["rhs"], preferred_element_type=f32) + bias0
            st[r0:r0 + QW, :] = s
            m = _fold8max(s)
            mq = [None] * G
            for kq in range(1, G):
                rhs = jnp.concatenate(wq[kq - 1:], axis=1) if kq < G - 1 else wq[G - 2]
                sk = jnp.dot(_as_bf16(k_s[g, (k0 + kq * QW) // 2:(k0 + (kq + 1) * QW) // 2, :]), rhs, preferred_element_type=f32)
                for qq in range(kq, G):
                    t = sk[:, (qq - kq) * WIN:(qq - kq + 1) * WIN]
                    if qq == kq:
                        t = t + bias_q
                    st[r0 + kq * QW:r0 + (kq + 1) * QW, (qq - 1) * WIN:qq * WIN] = t
                    tm = _fold8max(t)
                    mq[qq] = tm if mq[qq] is None else jnp.maximum(mq[qq], tm)
            lq = lane_quarter(8)
            extra = []
            for a in range(G):
                e = jnp.full((8, WIN), -jnp.inf, f32)
                for qq in range(1, G):
                    e = jnp.where(lq == (qq + a) % G, mq[qq], e)
                extra.append(e)
            m = jnp.maximum(m, jnp.concatenate(extra, axis=1))
        state["m"] = m if i == 0 else jnp.maximum(state["m"], m)
        if i == j:
            mx[j] = jnp.broadcast_to(jnp.max(state["m"], axis=0, keepdims=True), (8, G * WIN))

    def c_chunk(pr, par, st, mx, state, j, i):
        g = 2 * pr + par
        r0 = SOFF[j] + i * WIN
        if i == j:
            ms = [mx[j, 0:1, a * WIN:(a + 1) * WIN] for a in range(G)]
            mw = [None] + [by_quarter(ms, qq, 1) for qq in range(1, G)]
            ew = {(kq, qq): jnp.exp2(st[r0 + kq * QW:r0 + (kq + 1) * QW, (qq - 1) * WIN:qq * WIN] - mw[qq])
                  for kq in range(1, G) for qq in range(kq, G)}
        for a in range(G):
            row = par * GD + a * DH
            start = (row // 16) * 16
            off = row - start
            rows = pl.ds(pl.multiple_of(pr * (2 * GD) + start, 16), 32)
            one_row = ((off + DH) % 32) // 2
            r16 = lax.broadcasted_iota(jnp.int32, (16, WIN), 0)
            vt = _as_u32(vt_s[rows, i * WIN:(i + 1) * WIN])
            vt = _as_bf16(jnp.where(r16 == one_row, u32(ONES2), vt))
            hs = slice(a * WIN, (a + 1) * WIN)
            if i < j:
                p = jnp.exp2(st[r0:r0 + WIN, hs] - mx[j, 0:1, hs]).astype(bf16)
            else:
                lq = lane_quarter(QW)
                parts = [jnp.exp2(st[r0:r0 + QW, hs] - ms[a])]
                for kq in range(1, G):
                    e = jnp.zeros((QW, WIN), f32)
                    for qq in range(kq, G):
                        e = jnp.where(lq == (qq + a) % G, ew[(kq, qq)], e)
                    parts.append(e)
                p = jnp.concatenate(parts, axis=0).astype(bf16)
            d = jnp.dot(vt, p, preferred_element_type=f32)
            acc = d if i == 0 else state[a] + d
            state[a] = acc
            if i == j:
                qs = slice(j * WIN, (j + 1) * WIN)
                lsum = acc[2 * one_row:2 * one_row + 1, :]
                an = acc * _recip(lsum)
                if a:
                    an = pltpu.roll(an, WIN - QW * a, 1)
                ls = start - _woff(par)
                o = nd_s[g, ls:ls + 32, qs] + (1.0 - g_s[rows, :]) * an
                r32 = lax.broadcasted_iota(jnp.int32, (32, WIN), 0)
                keep = (r32 >= off) & (r32 < off + DH)
                pltpu.store(oT_s.at[rows, qs], o, mask=keep)

    bufs = ((stA, mxA), (stB, mxB))

    def b_all0():
        sb = {}
        for (j, i) in CHUNKS:
            b_chunk(0, 0, *bufs[0], sb, j, i)

    def step(pr, par):
        npr, npar = (pr, 1) if par == 0 else (pr + 1, 0)
        sb, sc = {}, {}
        for (j, i) in CHUNKS:
            c_chunk(pr, par, *bufs[par], sc, j, i)
            b_chunk(npr, npar, *bufs[1 - par], sb, j, i)

    def attention(update_memory):
        z = zero_s[0]
        for g in range(NG - 1):
            step(z + g // 2, g % 2)
        sc = {}
        for n, (j, i) in enumerate(CHUNKS):
            if n < NG and update_memory:
                mem_update(n)
            c_chunk(z + NG // 2 - 1, 1, *bufs[1], sc, j, i)

    def pack_ot():
        at_s[...] = oT_s[...].astype(bf16)
        otp_s[...] = _as_u32(at_s[...])

    def out_proj(nsplit=1, with_ln1=False):
        pack_ot()
        w = L // nsplit
        for p in range(nsplit):
            cs = slice(p * w, (p + 1) * w)
            for c in range(D // MC):
                a = jnp.dot(_as_bf16(woT[pl.ds(c * MC // 2, MC // 2), :]), _as_bf16(otp_s[:, cs]), preferred_element_type=f32)
                at_s[pl.ds(c * MC, MC), cs] = a.astype(bf16)
                if with_ln1 and c < L // WIN:
                    bits = pltpu.bitcast(a[0:8, c * WIN:(c + 1) * WIN], u32)
                    zero = pltpu.bitcast(lax.shift_right_logical(lax.shift_right_logical(bits, u32(16)), u32(16)), f32)
                    ln1_tile(c, zero[0:1, :])

    LW = 2 * WIN

    def ln2_strip(t, x_s, o_s):
        cs = slice(t * LW, (t + 1) * LW)
        for r0 in range(0, D, 32):
            h_s[r0:r0 + 32, cs] = (x_s[r0:r0 + 32, cs].astype(f32) + at_s[r0:r0 + 32, cs].astype(f32)).astype(bf16)
        m, rstd = _ln_stats(lambda r0, n: h_s[r0:r0 + n, cs].astype(f32))
        racc = None
        for r0 in range(0, D, 48):
            hf = h_s[r0:r0 + 48, cs].astype(f32)
            hn = ((hf - m) * rstd).astype(bf16)
            hn_s[r0:r0 + 48, cs] = hn
            hnf = hn.astype(f32)
            o_s[r0:r0 + 48, cs] = (hf + hnf).astype(bf16)
            wr = wr_s[r0:r0 + 48, :]
            p = _fold8(hnf * jnp.concatenate([wr] * (LW // WIN), axis=1))
            racc = p if racc is None else racc + p
        return jnp.sum(racc, axis=0, keepdims=True)

    def ln2(s, x_s, o_s, copy):
        rs = [ln2_strip(t, x_s, o_s) for t in range(L // LW)]
        copy.start()
        r = jnp.concatenate(rs, axis=1).astype(bf16).astype(f32)
        rmax = jnp.max(r)
        ridx = lax.broadcasted_iota(jnp.int32, (1, L), 1)
        amax = jnp.min(jnp.where(r == rmax, ridx, L))

        @pl.when(rmax > best_s[0])
        def _():
            best_s[0] = rmax
            best_s[1] = (amax + s * L).astype(f32)
            ts = pl.ds(pl.multiple_of((amax >> 7) << 7, WIN), WIN)
            bh_s[...] = _as_u32(h_s[:, ts])
            bhn_s[...] = _as_u32(hn_s[:, ts])

    xl_copy(0).wait()
    small_copy(0).start()
    small_copy(1).start()
    for t in range(L // WIN):
        ln1_tile(t)
    wq_copy(0).wait()
    w_copy(3).start()
    fence()
    xl_copy(1).start()
    fence()
    xr_copy(0).start()
    wT[pl.ds(0, WQA // 2), :] = _as_u32(wraw[0, :, 0:WQA].T)
    proj_q(0, 4)
    wq_copy(1).wait()
    w_copy(1).wait()
    wT[pl.ds(WQA // 2, (D - WQA) // 2), :] = _as_u32(wraw[0, :, WQA:D].T)
    wT[pl.ds(D // 2, D // 2), :] = _as_u32(wraw[1].T)
    proj_q(4, D // MC)
    proj_k(0, 4)
    w_copy(2).wait()
    w_copy(3).wait()
    small_copy(0).wait()
    small_copy(1).wait()
    wT[pl.ds(D, D // 2), :] = _as_u32(wraw[2].T)
    woT[...] = _as_u32(wraw[3].T)
    small_setup()
    proj_k(4, D // MC)
    transpose_k()
    proj_v()
    b_all0()

    def segment(s, carry):
        attention(True)

        @pl.when(s > 0)
        def _():
            out_copy(s - 1).wait()

        xr_copy(s).wait()
        xl_copy(s + 1).wait()
        fence()
        for i in range(3):
            @pl.when(s == i)
            def _():
                moe_copy(i).start()

        out_proj(1, True)
        proj_k()
        proj_v(KTV)
        proj_q(kt=KTQ)
        mem_read()
        b_all0()
        ln2(s, xr_s, out_s, out_copy(s))

        @pl.when(s + 2 < NSEG)
        def _():
            xr_copy(s + 1).start()
            xl_copy(s + 2).start()

        return carry

    lax.fori_loop(0, NSEG - 1, segment, 0)

    last_copy = pltpu.make_async_copy(out2_s, out_hbm.at[:, cols(NSEG - 1)], sem_o.at[1])
    attention(False)
    out_proj(2)
    ln2(NSEG - 1, xl_s, out2_s, last_copy)

    idx = best_s[1].astype(jnp.int32)
    tile = pl.ds(pl.multiple_of((idx >> 7) << 7, WIN), WIN)
    lane = idx & (WIN - 1)
    for i in range(3):
        moe_copy(i).wait()
    hn_t = _as_bf16(bhn_s[...])
    onehot = (lax.broadcasted_iota(jnp.int32, (16, WIN), 1) == lane).astype(f32).astype(bf16)
    xs = lax.dot_general(onehot, hn_t, NT, preferred_element_type=f32).astype(bf16)
    FC = 4 * WIN
    RB = 64
    for c in range(F // FC):
        cs = slice(c * FC, (c + 1) * FC)
        gt = jnp.dot(xs, wg_v[:, cs], preferred_element_type=f32)[0:8].astype(bf16).astype(f32)
        up = jnp.dot(xs, wu_v[:, cs], preferred_element_type=f32)[0:8].astype(bf16).astype(f32)
        act = (gt * (1.0 / (1.0 + jnp.exp(-gt)))).astype(bf16).astype(f32) * up
        act = act.astype(bf16).astype(f32)
        for rb in range(D // RB):
            p = acc_s[rb * RB:(rb + 1) * RB, :]
            for t in range(0, FC // WIN, 2):
                w2 = wd_v[rb * RB:(rb + 1) * RB, c * FC + t * WIN:c * FC + (t + 2) * WIN].astype(f32)
                w2 = w2 * act[0:1, t * WIN:(t + 2) * WIN]
                p = p + w2[:, 0:WIN] + w2[:, WIN:2 * WIN]
            acc_s[rb * RB:(rb + 1) * RB, :] = p
    y = jnp.sum(acc_s[...], axis=1, keepdims=True)
    rsel = jnp.full((1, 1), best_s[0], f32)
    y = y.astype(bf16).astype(f32) * (1.0 / (1.0 + jnp.exp(-rsel)))
    lanes = lax.broadcasted_iota(jnp.int32, (D, WIN), 1)
    yt = jnp.where(lanes == lane, y.astype(bf16).astype(f32), 0.0)
    t = (hn_t.astype(f32) + yt).astype(bf16).astype(f32)
    out_copy(NSEG - 2).wait()
    last_copy.wait()
    fix_s[...] = (_as_bf16(bh_s[...]).astype(f32) + t).astype(bf16)
    fix = pltpu.make_async_copy(fix_s, out_hbm.at[:, tile], sem_o.at[0])
    fix.start()
    fix.wait()


@jax.jit
def pallas_sequential_preLN__memory_aug_infini_attn__moe_arch_mod__prompt_kernel(
    A_x: jax.Array,
    A_wq: jax.Array,
    A_wk: jax.Array,
    A_wv: jax.Array,
    A_wo: jax.Array,
    A_beta: jax.Array,
    B_x: jax.Array,
    B_w_r: jax.Array,
    B_w_gate: jax.Array,
    B_w_up: jax.Array,
    B_w_down: jax.Array,
):
    del B_x
    hbm = pl.BlockSpec(memory_space=pltpu.HBM)
    out_t = pl.pallas_call(
        _kernel,
        out_shape=jax.ShapeDtypeStruct((D, S), bf16),
        in_specs=[hbm] * 10,
        out_specs=hbm,
        scratch_shapes=[
            pltpu.VMEM((D, L), bf16),
            pltpu.VMEM((D, L), bf16),
            pltpu.VMEM((4, D, D), bf16),
            pltpu.VMEM((3 * D // 2, D), u32),
            pltpu.VMEM((D // 2, D), u32),
            pltpu.VMEM((D, F), bf16),
            pltpu.VMEM((D, F), bf16),
            pltpu.VMEM((D, F), bf16),
            pltpu.VMEM((4, D, WIN), bf16),
            pltpu.VMEM((D // 2, L), u32),
            pltpu.VMEM((D, L), bf16),
            pltpu.VMEM((D, L), bf16),
            pltpu.VMEM((D, L), bf16),
            pltpu.VMEM((NG, L // 2, WIN), u32),
            pltpu.VMEM((D, L), bf16),
            pltpu.VMEM((D, L), bf16),
            pltpu.VMEM((1280, G * WIN), f32),
            pltpu.VMEM((1280, G * WIN), f32),
            pltpu.VMEM((4, 8, G * WIN), f32),
            pltpu.VMEM((4, 8, G * WIN), f32),
            pltpu.VMEM((NG, VW, L), f32),
            pltpu.VMEM((NG, VW, WIN), f32),
            pltpu.VMEM((2, VW, WIN), f32),
            pltpu.VMEM((D, L), f32),
            pltpu.VMEM((D // 2, L), u32),
            pltpu.VMEM((D, L), bf16),
            pltpu.VMEM((D, WIN), f32),
            pltpu.VMEM((D, WIN), f32),
            pltpu.VMEM((D, L), bf16),
            pltpu.VMEM((D, L), bf16),
            pltpu.VMEM((D, L), bf16),
            pltpu.VMEM((D, L), bf16),
            pltpu.VMEM((D // 2, WIN), u32),
            pltpu.VMEM((D // 2, WIN), u32),
            pltpu.VMEM((D, WIN), bf16),
            pltpu.VMEM((D, WIN), f32),
            pltpu.VMEM((1, H), bf16),
            pltpu.VMEM((D,), bf16),
            pltpu.SMEM((2,), f32),
            pltpu.SMEM((1,), jnp.int32),
            pltpu.SemaphoreType.DMA((2,)),
            pltpu.SemaphoreType.DMA((5,)),
            pltpu.SemaphoreType.DMA((3,)),
            pltpu.SemaphoreType.DMA((2,)),
            pltpu.SemaphoreType.DMA((2,)),
            pltpu.SemaphoreType.REGULAR,
        ],
        compiler_params=pltpu.CompilerParams(vmem_limit_bytes=100 * 1024 * 1024),
    )(A_x.reshape(S, D).T, A_wq, A_wk, A_wv, A_wo, A_beta.reshape(1, H), B_w_r,
      B_w_gate, B_w_up, B_w_down.T)
    return out_t.T.reshape(1, S, D)
```
